```python
import jax
import jax.numpy as jnp

def _softmax(x, axis=-1):
    return jax.nn.softmax(x, axis=axis)

def _gelu(x):
    return jax.nn.gelu(x, approximate=True)

def _silu(x):
    return jax.nn.silu(x)

def _sigmoid(x):
    return jax.nn.sigmoid(x)

def _layernorm(x, axis=-1, eps=1e-05):
    m = jnp.mean(x, axis=axis, keepdims=True)
    v = jnp.var(x, axis=axis, keepdims=True)
    return (x - m) / jnp.sqrt(v + eps)

def _scatter_add(tgt, idx, src, axis=0):
    return tgt.at[idx].add(src)

def _segment_sum(src, seg, n):
    return jax.ops.segment_sum(src, seg, n)

class _Rng:

    def __init__(self, key):
        self._k = key

    def _next(self):
        self._k, sub = jax.random.split(self._k)
        return sub

    def normal(self, shape):
        return jax.random.normal(self._next(), shape, dtype=jnp.bfloat16)

    def randint(self, lo, hi, shape):
        return jax.random.randint(self._next(), shape, lo, hi, dtype=jnp.int32)

    def uniform(self, shape, lo=0.0, hi=1.0):
        return jax.random.uniform(self._next(), shape, jnp.bfloat16, lo, hi)

    def permutation(self, n):
        return jax.random.permutation(self._next(), n)
kernel_name = 'adaLN_cond__sliding_local_dilated__glu_gated_bilinear__prompt'

def setup_inputs():
    _rng = _Rng(jax.random.key(int.from_bytes(__import__("os").urandom(4), "little")))
    _w = lambda a: (lambda t: t.astype(jnp.bfloat16) if jnp.issubdtype(t.dtype, jnp.floating) else t)(jnp.asarray(a))

    def _A_setup():
        B, S, D = (1, 2048, 576)
        return {'x': _w((lambda *s: _rng.normal(s) * 0.05)(B, S, D)), 'wqkv': _w((lambda *s: _rng.normal(s) * 0.05)(D, 3 * D)), 'wo': _w((lambda *s: _rng.normal(s) * 0.05)(D, D))}
    _A_in = _A_setup()

    def _B_setup():
        B, S, D, F = (1, 2048, 576, 4608)
        return {'x': _w((lambda *s: _rng.normal(s) * 0.05)(B, S, D)), 'w_gate': _w((lambda *s: _rng.normal(s) * 0.05)(D, F) * D ** (-0.5)), 'w_up': _w((lambda *s: _rng.normal(s) * 0.05)(D, F) * D ** (-0.5)), 'w_down': _w((lambda *s: _rng.normal(s) * 0.05)(F, D) * F ** (-0.5))}
    _B_in = _B_setup()
    return {'A_x': _A_in['x'], 'A_wqkv': _A_in['wqkv'], 'A_wo': _A_in['wo'], 'B_x': _B_in['x'], 'B_w_gate': _B_in['w_gate'], 'B_w_up': _B_in['w_up'], 'B_w_down': _B_in['w_down'], 'c': _w((lambda *s: _rng.normal(s) * 0.05)(1, 576)), 'w_mod': _w((lambda *s: _rng.normal(s) * 0.05)(576, 6 * 576) * 576 ** (-0.5))}

def reference(A_x, A_wqkv, A_wo, B_x, B_w_gate, B_w_up, B_w_down, c, w_mod):

    def _A_ref(x, wqkv, wo):
        B, S, D = x.shape
        H = 32
        Dh = D // H
        W, dil = (8, 2)
        qkv = (lambda x, *d: x.transpose(*d))((x @ wqkv).reshape(B, S, 3, H, Dh), 2, 0, 3, 1, 4)
        q, k, v = (qkv[0], qkv[1], qkv[2])
        scale = Dh ** (-0.5)
        pos = jnp.arange(S)
        off = jnp.arange(W) * dil
        idx = pos[:, None] - off[None, :]
        mask = idx >= 0
        idx_c = jnp.where(mask, idx, 0).reshape(-1)
        kg = k[:, :, idx_c, :].reshape(B, H, S, W, Dh)
        vg = v[:, :, idx_c, :].reshape(B, H, S, W, Dh)
        logits = jnp.einsum('bhsd,bhswd->bhsw', q, kg) * scale
        logits = jnp.where(mask[None, None, :, :], logits, -1000000000.0)
        attn = _softmax(logits, axis=-1)
        o = jnp.einsum('bhsw,bhswd->bhsd', attn, vg)
        return (lambda x, *d: x.transpose(*d))(o, 0, 2, 1, 3).reshape(B, S, D) @ wo

    def _B_ref(x, w_gate, w_up, w_down):
        g = jnp.einsum('bsd,df->bsf', x, w_gate)
        u = jnp.einsum('bsd,df->bsf', x, w_up)
        h = g * u
        return jnp.einsum('bsf,fd->bsd', h, w_down)
    x = A_x
    mod = (_silu(c) @ w_mod).reshape(c.shape[0], 6, 1, -1)
    sa, ca, ga, sb, cb, gb = (mod[:, 0].copy(), mod[:, 1].copy(), mod[:, 2].copy(), mod[:, 3].copy(), mod[:, 4].copy(), mod[:, 5].copy())
    h = _layernorm(x, axis=-1) * (1 + ca) + sa
    x = x + ga * _A_ref(h, A_wqkv, A_wo)
    h = _layernorm(x, axis=-1) * (1 + cb) + sb
    x = x + gb * _B_ref(h, B_w_gate, B_w_up, B_w_down)
    return x
```

```python
import functools

import jax
import jax.numpy as jnp
from jax import lax
import jax.experimental.pallas as pl
import jax.experimental.pallas.tpu as pltpu

N_HEADS = 32
WINDOW = 8
DILATION = 2
LN_EPS = 1e-5
MASK_VALUE = -1000000000.0
LANES = 128

T1 = 256
T2 = 256
FC = 512

F32 = jnp.float32
BF16 = jnp.bfloat16
_TN = (((0,), (0,)), ((), ()))


def _dot_tn(a, b):
  return lax.dot_general(a, b, _TN, preferred_element_type=F32)


def _tile_lanes(col, n):
  return col if n == 1 else jnp.concatenate([col] * n, axis=1)


def _ln_modulate(x, scale1p, shift):
  inv_d = 1.0 / x.shape[0]
  mean = jnp.sum(x, axis=0, keepdims=True) * inv_d
  xc = x - mean
  var = jnp.sum(xc * xc, axis=0, keepdims=True) * inv_d
  return xc * lax.rsqrt(var + LN_EPS) * scale1p + shift


def _attention_block(qkv_ref, cur, prev, o_ref, o_idx, pos0, d_model):
  dh = d_model // N_HEADS
  lane = lax.broadcasted_iota(jnp.int32, (N_HEADS, LANES), 1)

  def head_rows(blk, part, d):
    return qkv_ref[blk, pl.ds(part * d_model + d, N_HEADS, stride=dh), :]

  def shifted(c, p, w):
    if w == 0:
      return c
    s = w * DILATION
    return pltpu.roll(jnp.where(lane < LANES - s, c, p), s, 1)

  logits = [None] * WINDOW
  for d in range(dh):
    q = head_rows(cur, 0, d)
    kc, kp = head_rows(cur, 1, d), head_rows(prev, 1, d)
    for w in range(WINDOW):
      t = q * shifted(kc, kp, w)
      logits[w] = t if d == 0 else logits[w] + t
  scale = dh ** -0.5
  for w in range(WINDOW):
    logits[w] = logits[w] * scale
    if w:
      logits[w] = jnp.where(lane + pos0 >= w * DILATION, logits[w], MASK_VALUE)
  m = functools.reduce(jnp.maximum, logits)
  e = [jnp.exp(l - m) for l in logits]
  inv = 1.0 / functools.reduce(jnp.add, e)
  p = [x * inv for x in e]
  for d in range(dh):
    vc, vp = head_rows(cur, 2, d), head_rows(prev, 2, d)
    o = p[0] * vc
    for w in range(1, WINDOW):
      o = o + p[w] * shifted(vc, vp, w)
    o_ref[o_idx, pl.ds(d, N_HEADS, stride=dh), :] = o


def _kernel(xt_hbm, wqkv_hbm, wo_hbm, wg_hbm, wu_hbm, wdt_hbm, c_hbm, wmod_hbm,
            out_hbm,
            xt_v, wqkv_v, wo_v, wg_v, wu_v, wdt_v, c_v, wmod_v,
            mod_v, qkv_v, o_v, x1_v, h2_v, out_v, in_sem, out_sem):
  d_model, seq = xt_hbm.shape
  d_ff = wg_hbm.shape[1]
  n1, n2 = seq // T1, seq // T2
  nb = T1 // LANES

  c_cp = pltpu.make_async_copy(c_hbm, c_v, in_sem.at[0])
  wmod_cp = pltpu.make_async_copy(wmod_hbm, wmod_v, in_sem.at[1])
  wqkv_cp = pltpu.make_async_copy(wqkv_hbm, wqkv_v, in_sem.at[2])
  wo_cp = pltpu.make_async_copy(wo_hbm, wo_v, in_sem.at[3])
  wg_cp = pltpu.make_async_copy(wg_hbm, wg_v, in_sem.at[4])
  wu_cp = pltpu.make_async_copy(wu_hbm, wu_v, in_sem.at[5])
  wdt_cp = pltpu.make_async_copy(wdt_hbm, wdt_v, in_sem.at[6])
  x_cps = [
      pltpu.make_async_copy(xt_hbm.at[:, pl.ds(i * T1, T1)], xt_v.at[i],
                            in_sem.at[7 + i]) for i in range(n1)
  ]
  for cp in (c_cp, wmod_cp, *x_cps, wqkv_cp, wo_cp):
    cp.start()
  c_cp.wait()
  wmod_cp.wait()
  for cp in (wg_cp, wu_cp, wdt_cp):
    cp.start()

  cv = c_v[...].astype(F32)
  sc = cv * jax.nn.sigmoid(cv)
  sc_col = jnp.broadcast_to(sc, (LANES, d_model)).T
  for j in range(6 * d_model // LANES):
    cols = pl.ds(j * LANES, LANES)
    row = jnp.sum(wmod_v[:, cols].astype(F32) * sc_col, axis=0, keepdims=True)
    mod_v[cols, :] = jnp.broadcast_to(row, (LANES, LANES)).T
  for part in (1, 4):
    rows = pl.ds(part * d_model, d_model)
    mod_v[rows, :] = mod_v[rows, :] + 1.0

  def mod(part, n):
    return _tile_lanes(mod_v[pl.ds(part * d_model, d_model), :], n)

  for cp in (*x_cps, wqkv_cp, wo_cp):
    cp.wait()

  qkv_v[0] = jnp.zeros(qkv_v.shape[1:], F32)

  @pl.loop(0, n1)
  def _(i):
    x = xt_v[i].astype(F32)
    h1 = _ln_modulate(x, mod(1, nb), mod(0, nb)).astype(BF16)
    qkv = _dot_tn(wqkv_v[...], h1)
    for b in range(nb):
      qkv_v[b + 1] = qkv[:, b * LANES:(b + 1) * LANES]
    for b in range(nb):
      _attention_block(qkv_v, b + 1, b, o_v, b, i * T1 + b * LANES, d_model)
    qkv_v[0] = qkv_v[nb]
    o = jnp.concatenate([o_v[b] for b in range(nb)], axis=1).astype(BF16)
    x1 = x + mod(2, nb) * _dot_tn(wo_v[...], o)
    x1_v[i] = x1
    h2_v[i] = _ln_modulate(x1, mod(4, nb), mod(3, nb)).astype(BF16)

  for cp in (wg_cp, wu_cp, wdt_cp):
    cp.wait()

  def out_copy(i, slot):
    cols = pl.ds(pl.multiple_of(i * T2, T2), T2)
    return pltpu.make_async_copy(out_v.at[slot], out_hbm.at[:, cols],
                                 out_sem.at[slot])

  @pl.loop(0, n2)
  def _(i):
    slot = i % 2

    @pl.when(i >= 2)
    def _():
      out_copy(i - 2, slot).wait()

    h2 = h2_v[i]
    acc = None
    for f in range(d_ff // FC):
      cols = pl.ds(f * FC, FC)
      g = _dot_tn(wg_v[:, cols], h2)
      u = _dot_tn(wu_v[:, cols], h2)
      part = jnp.dot(wdt_v[:, cols], (g * u).astype(BF16),
                     preferred_element_type=F32)
      acc = part if acc is None else acc + part
    out_v[slot] = (x1_v[i] + mod(5, T2 // LANES) * acc).astype(out_v.dtype)
    out_copy(i, slot).start()

  for i in range(n2 - 2, n2):
    out_copy(i, i % 2).wait()


@jax.jit
def pallas_adaLN_cond__sliding_local_dilated__glu_gated_bilinear__prompt_kernel(
    A_x: jax.Array,
    A_wqkv: jax.Array,
    A_wo: jax.Array,
    B_x: jax.Array,
    B_w_gate: jax.Array,
    B_w_up: jax.Array,
    B_w_down: jax.Array,
    c: jax.Array,
    w_mod: jax.Array,
):
  del B_x
  batch, seq, d_model = A_x.shape
  d_ff = B_w_gate.shape[1]
  assert batch == 1 and T1 == T2 and seq % T1 == 0 and d_ff % FC == 0
  n1 = seq // T1
  hbm = pl.BlockSpec(memory_space=pltpu.HBM)
  operands = (A_x.reshape(seq, d_model).T, A_wqkv, A_wo, B_w_gate, B_w_up,
              B_w_down.T, c, w_mod)
  like = lambda a: pltpu.VMEM(a.shape, a.dtype)
  out_t = pl.pallas_call(
      _kernel,
      in_specs=[hbm] * len(operands),
      out_specs=hbm,
      out_shape=jax.ShapeDtypeStruct((d_model, seq), A_x.dtype),
      scratch_shapes=[
          pltpu.VMEM((n1, d_model, T1), A_x.dtype),
          *map(like, operands[1:]),
          pltpu.VMEM((6 * d_model, LANES), F32),
          pltpu.VMEM((T1 // LANES + 1, 3 * d_model, LANES), F32),
          pltpu.VMEM((T1 // LANES, d_model, LANES), F32),
          pltpu.VMEM((n1, d_model, T1), F32),
          pltpu.VMEM((n1, d_model, T1), BF16),
          pltpu.VMEM((2, d_model, T2), A_x.dtype),
          pltpu.SemaphoreType.DMA((7 + n1,)),
          pltpu.SemaphoreType.DMA((2,)),
      ],
      compiler_params=pltpu.CompilerParams(vmem_limit_bytes=100 * 2**20),
      name="adaln_window_attn_glu",
  )(*operands)
  return out_t.T.reshape(batch, seq, d_model)
```

```python
import functools

import jax
import jax.numpy as jnp
from jax import lax
import jax.experimental.pallas as pl
import jax.experimental.pallas.tpu as pltpu

N_HEADS = 32
WINDOW = 8
DILATION = 2
LN_EPS = 1e-5
MASK_VALUE = -1000000000.0
LANES = 128
NB = LANES // N_HEADS
TILE = NB * LANES
HALO = 16

NC = 3
FS = 1536
PACKED = False

F32 = jnp.float32
BF16 = jnp.bfloat16
_TN = (((0,), (0,)), ((), ()))


def _dot_tn(a, b):
  return lax.dot_general(a, b, _TN, preferred_element_type=F32)


def _dot(a, b):
  return jnp.dot(a, b, preferred_element_type=F32)


def _tile_lanes(col, n):
  return col if n == 1 else jnp.concatenate([col] * n, axis=1)


def _ln_modulate(x, scale1p, shift):
  inv_d = 1.0 / x.shape[0]
  mean = jnp.sum(x, axis=0, keepdims=True) * inv_d
  xc = x - mean
  var = jnp.sum(xc * xc, axis=0, keepdims=True) * inv_d
  return xc * lax.rsqrt(var + LN_EPS) * scale1p + shift


def _strassen_lhs(a11, a12, a21, a22):
  f11, f12, f21, f22 = (a.astype(F32) for a in (a11, a12, a21, a22))
  c = lambda a: a.astype(BF16)
  return (c(f11 + f22), c(f21 + f22), a11, a22, c(f11 + f12), c(f21 - f11),
          c(f12 - f22))


def _strassen_rhs(b11, b12, b21, b22):
  c = lambda b: b.astype(BF16)
  return (c(b11 + b22), c(b11), c(b12 - b22), c(b21 - b11), c(b22),
          c(b11 + b12), c(b21 + b22))


def _strassen_out(m1, m2, m3, m4, m5, m6, m7):
  return m1 + m4 - m5 + m7, m3 + m5, m2 + m4, m1 - m2 + m3 + m6


_ORDER = (2, 3, 0, 4, 6, 1, 5)


def _kernel(xt_hbm, wqkv_hbm, wo_hbm, wg_hbm, wu_hbm, wdt_hbm, c_hbm, wmod_hbm,
            out_hbm,
            xt_v, wqkv_v, wo_v, wg_v, wu_v, wdt_v, c_v, wmod_v,
            mod_v, qkv_v, qt_v, kvt_v, ot_v, o_v, x1_v, hb_v, hr_v, acc_v, out_v,
            in_sem, out_sem):
  d_model, seq = xt_hbm.shape
  d_ff = wg_hbm.shape[1]
  dh = d_model // N_HEADS
  n_tiles = seq // TILE
  fc = d_ff // NC
  fh = FS // 2
  kh = 256
  mh = d_model // 2

  sems = iter(range(in_sem.shape[0]))
  copy = lambda src, dst: pltpu.make_async_copy(src, dst, in_sem.at[next(sems)])
  c_cp = copy(c_hbm, c_v)
  wmod_cp = copy(wmod_hbm, wmod_v)
  wqkv_cp = copy(wqkv_hbm, wqkv_v)
  wo_cp = copy(wo_hbm, wo_v)
  x_cps = [copy(xt_hbm.at[:, pl.ds(i * TILE, TILE)], xt_v.at[i])
           for i in range(n_tiles)]
  ff_cps = [copy(w_hbm.at[:, pl.ds(j * fc, fc)], w_v.at[j])
            for j in range(NC)
            for w_hbm, w_v in ((wg_hbm, wg_v), (wu_hbm, wu_v), (wdt_hbm, wdt_v))]
  for cp in (c_cp, wmod_cp, *x_cps, wqkv_cp, wo_cp):
    cp.start()
  c_cp.wait()
  wmod_cp.wait()
  for cp in ff_cps:
    cp.start()

  cv = c_v[...].astype(F32)
  sc = cv * jax.nn.sigmoid(cv)
  sc_col = jnp.broadcast_to(sc, (LANES, d_model)).T
  for j in range(6 * d_model // LANES):
    cols = pl.ds(j * LANES, LANES)
    row = jnp.sum(wmod_v[:, cols].astype(F32) * sc_col, axis=0, keepdims=True)
    mod_v[cols, :] = jnp.broadcast_to(row, (LANES, LANES)).T
  for part in (1, 4):
    rows = pl.ds(part * d_model, d_model)
    mod_v[rows, :] = mod_v[rows, :] + 1.0

  def mod(part, n=1):
    return _tile_lanes(mod_v[pl.ds(part * d_model, d_model), :], n)

  for cp in (*x_cps, wqkv_cp, wo_cp):
    cp.wait()

  kvt_v[:, pl.ds(LANES, HALO), :] = jnp.zeros((2 * dh, HALO, LANES), F32)
  lane = lax.broadcasted_iota(jnp.int32, (HALO, LANES), 1)

  @pl.loop(0, n_tiles)
  def _(i):
    x = xt_v[i].astype(F32)
    h1 = _ln_modulate(x, mod(1, NB), mod(0, NB)).astype(BF16)
    qkv = _dot_tn(wqkv_v[...], h1)
    for b in range(NB):
      qkv_v[b] = qkv[:, b * LANES:(b + 1) * LANES]

    for part in range(3):
      for d in range(dh):
        rows = pl.ds(part * d_model + d, N_HEADS, stride=dh)
        t = jnp.concatenate([qkv_v[b, rows, :] for b in range(NB)], axis=0).T
        if part == 0:
          qt_v[d] = t
        else:
          j = (part - 1) * dh + d
          prev = kvt_v[j, pl.ds(LANES, HALO), :]
          tail = jnp.where(lane < LANES - N_HEADS, t[LANES - HALO:], prev)
          kvt_v[j, pl.ds(0, HALO), :] = pltpu.roll(tail, N_HEADS, 1)
          kvt_v[j, pl.ds(HALO, LANES), :] = t

    scale = dh ** -0.5
    pos = (lax.broadcasted_iota(jnp.int32, (8, LANES), 0) + i * TILE
           + lax.broadcasted_iota(jnp.int32, (8, LANES), 1) // N_HEADS * LANES)
    for g in range(LANES // 8):
      logits = [None] * WINDOW
      for d in range(dh):
        q = qt_v[d, pl.ds(8 * g, 8), :]
        for w in range(WINDOW):
          t = q * kvt_v[d, pl.ds(HALO + 8 * g - DILATION * w, 8), :]
          logits[w] = t if d == 0 else logits[w] + t
      for w in range(WINDOW):
        logits[w] = logits[w] * scale
        if 8 * g < DILATION * w:
          logits[w] = jnp.where(pos + 8 * g >= DILATION * w, logits[w], MASK_VALUE)
      m = functools.reduce(jnp.maximum, logits)
      e = [jnp.exp(l - m) for l in logits]
      inv = 1.0 / functools.reduce(jnp.add, e)
      p = [x_ * inv for x_ in e]
      for d in range(dh):
        o = None
        for w in range(WINDOW):
          t = p[w] * kvt_v[dh + d, pl.ds(HALO + 8 * g - DILATION * w, 8), :]
          o = t if o is None else o + t
        ot_v[d, pl.ds(8 * g, 8), :] = o

    for d in range(dh):
      t = ot_v[d].T
      for b in range(NB):
        o_v[b, pl.ds(d, N_HEADS, stride=dh), :] = t[b * N_HEADS:(b + 1) * N_HEADS]

    o = jnp.concatenate([o_v[b] for b in range(NB)], axis=1).astype(BF16)
    x1 = x + mod(2, NB) * _dot_tn(wo_v[...], o)
    x1_v[i] = x1
    h2 = _ln_modulate(x1, mod(4, NB), mod(3, NB))
    half = TILE // 2
    bs = _strassen_rhs(h2[:kh, :half], h2[:kh, half:], h2[kh:2 * kh, :half],
                       h2[kh:2 * kh, half:])
    for j in range(7):
      hb_v[i, j] = bs[j]
    hr_v[i] = h2[2 * kh:].astype(BF16)

  for cp in ff_cps:
    cp.wait()

  def out_copy(i):
    cols = pl.ds(pl.multiple_of(i * TILE, TILE), TILE)
    return pltpu.make_async_copy(out_v.at[i], out_hbm.at[:, cols], out_sem.at[i])

  @pl.loop(0, n_tiles)
  def _(i):
    half = TILE // 2

    def step(j):
      def project(w_v, c0):
        r = _dot_tn(w_v[j, pl.ds(2 * kh, d_model - 2 * kh), pl.ds(c0, FS)], hr_v[i])
        a = _strassen_lhs(w_v[j, pl.ds(0, kh), pl.ds(c0, fh)],
                          w_v[j, pl.ds(kh, kh), pl.ds(c0, fh)],
                          w_v[j, pl.ds(0, kh), pl.ds(c0 + fh, fh)],
                          w_v[j, pl.ds(kh, kh), pl.ds(c0 + fh, fh)])
        m = {k: _dot_tn(a[k], hb_v[i, k]) for k in _ORDER}
        c11, c12, c21, c22 = _strassen_out(*(m[k] for k in range(7)))
        return (c11 + r[:fh, :half], c12 + r[:fh, half:],
                c21 + r[fh:, :half], c22 + r[fh:, half:])

      acc = None
      for c0 in range(0, fc, FS):
        g = project(wg_v, c0)
        u = project(wu_v, c0)
        b = _strassen_rhs(*(gg * uu for gg, uu in zip(g, u)))
        a = _strassen_lhs(wdt_v[j, pl.ds(0, mh), pl.ds(c0, fh)],
                          wdt_v[j, pl.ds(0, mh), pl.ds(c0 + fh, fh)],
                          wdt_v[j, pl.ds(mh, mh), pl.ds(c0, fh)],
                          wdt_v[j, pl.ds(mh, mh), pl.ds(c0 + fh, fh)])
        m = {k: _dot(a[k], b[k]) for k in _ORDER}
        acc = m if acc is None else {k: acc[k] + m[k] for k in _ORDER}
      return acc

    if NC == 1:
      acc = step(0)
      acc = [acc[k] for k in range(7)]
    else:
      @pl.loop(0, NC)
      def _(j):
        acc = step(j)
        for k in _ORDER:
          acc_v[k] = jnp.where(j > 0, acc_v[k], 0.0) + acc[k]
      acc = [acc_v[k] for k in range(7)]
    c11, c12, c21, c22 = _strassen_out(*acc)
    y = jnp.concatenate([jnp.concatenate([c11, c12], axis=1),
                         jnp.concatenate([c21, c22], axis=1)], axis=0)
    out_v[i] = (x1_v[i] + mod(5, NB) * y).astype(out_v.dtype)
    out_copy(i).start()

  for i in range(n_tiles):
    out_copy(i).wait()


@jax.jit
def pallas_adaLN_cond__sliding_local_dilated__glu_gated_bilinear__prompt_kernel(
    A_x, A_wqkv, A_wo, B_x, B_w_gate, B_w_up, B_w_down, c, w_mod):
  del B_x
  batch, seq, d_model = A_x.shape
  d_ff = B_w_gate.shape[1]
  dh = d_model // N_HEADS
  n_tiles = seq // TILE
  fc = d_ff // NC
  assert batch == 1 and seq % TILE == 0 and fc % FS == 0 and FS % 256 == 0
  hbm = pl.BlockSpec(memory_space=pltpu.HBM)
  operands = (A_x.reshape(seq, d_model).T, A_wqkv, A_wo, B_w_gate, B_w_up,
              B_w_down.T, c, w_mod)
  like = lambda a: pltpu.VMEM(a.shape, a.dtype)
  out_t = pl.pallas_call(
      _kernel,
      in_specs=[hbm] * len(operands),
      out_specs=hbm,
      out_shape=jax.ShapeDtypeStruct((d_model, seq), A_x.dtype),
      scratch_shapes=[
          pltpu.VMEM((n_tiles, d_model, TILE), A_x.dtype),
          like(A_wqkv), like(A_wo),
          *[pltpu.VMEM((NC, d_model, fc), BF16)] * 3,
          like(c), like(w_mod),
          pltpu.VMEM((6 * d_model, LANES), F32),
          pltpu.VMEM((NB, 3 * d_model, LANES), F32),
          pltpu.VMEM((dh, LANES, LANES), F32),
          pltpu.VMEM((2 * dh, HALO + LANES, LANES), F32),
          pltpu.VMEM((dh, LANES, LANES), F32),
          pltpu.VMEM((NB, d_model, LANES), F32),
          pltpu.VMEM((n_tiles, d_model, TILE), F32),
          pltpu.VMEM((n_tiles, 7, 256, TILE // 2), BF16),
          pltpu.VMEM((n_tiles, d_model - 512, TILE), BF16),
          pltpu.VMEM((7, d_model // 2, TILE // 2), F32),
          pltpu.VMEM((n_tiles, d_model, TILE), A_x.dtype),
          pltpu.SemaphoreType.DMA((4 + n_tiles + 3 * NC,)),
          pltpu.SemaphoreType.DMA((n_tiles,)),
      ],
      compiler_params=pltpu.CompilerParams(vmem_limit_bytes=110 * 2**20),
      name="adaln_window_attn_glu",
  )(*operands)
  return out_t.T.reshape(batch, seq, d_model)
```

```python
import functools

import jax
import jax.numpy as jnp
from jax import lax
import jax.experimental.pallas as pl
import jax.experimental.pallas.tpu as pltpu

N_HEADS = 32
WINDOW = 8
DILATION = 2
LN_EPS = 1e-5
MASK_VALUE = -1000000000.0
LANES = 128
NB = LANES // N_HEADS
TILE = NB * LANES
HALO = 16

NC = 3
FS = 1536
QC = 64
FLAGS = None
NT = 3
LINK = 0
MR = 64
PACK_T = True
ANCHOR_L = True
ANCHOR_ST = False
TAIL = "SPUKWMm"
PRO_T = True
ANCHOR_T = True
ANCHOR_S = False
GATE_ROW = 0
WC = 64
SKIP_FFN = False
G = 1
BODY = "Q0,S0,P0,Q1,S1,P1,Q2,S2,P2,Q3,S3,P3,Q4,S4,P4,Q5,S5,P5,Q6,S6,P6,Q7,S7,P7,Q8,S8,P8,Q9,S9,P9,Q10,S10,P10,Q11,S11,P11,Q12,S12,P12,Q13,S13,P13,Q14,S14,P14,Q15,S15,P15,Q16,U0,m0,m2,Q17,U1,M0,Q18,U2,M1,Q19,M2,Q20,M3,Q21,m1,m3,Q22,M4,Q23,M5,Q24,M6,Q25,M7,Q26|W0,Tq0,l0,W1,Tq1,L0,W2,Tq2,l1,W3,Tk0,L1,W4,Tk1,l2,W5,Tk2,L2,W6,Tv0,l3,W7,Tv1,L3,W8,Tv2"

F32 = jnp.float32
BF16 = jnp.bfloat16
_TN = (((0,), (0,)), ((), ()))


def _dot_tn(a, b):
  return lax.dot_general(a, b, _TN, preferred_element_type=F32)


def _dot(a, b):
  return jnp.dot(a, b, preferred_element_type=F32)


def _words(x):
  return pltpu.bitcast(x, jnp.int32)


def _halves(x):
  return pltpu.bitcast(x, BF16)


def _tile_lanes(col, n):
  return col if n == 1 else jnp.concatenate([col] * n, axis=1)


def _ln_modulate(x, scale1p, shift):
  inv_d = 1.0 / x.shape[0]
  mean = jnp.sum(x, axis=0, keepdims=True) * inv_d
  xc = x - mean
  var = jnp.sum(xc * xc, axis=0, keepdims=True) * inv_d
  return xc * lax.rsqrt(var + LN_EPS) * scale1p + shift


def _strassen_lhs(a11, a12, a21, a22):
  f11, f12, f21, f22 = (a.astype(F32) for a in (a11, a12, a21, a22))
  c = lambda a: a.astype(BF16)
  return (c(f11 + f22), c(f21 + f22), a11, a22, c(f11 + f12), c(f21 - f11),
          c(f12 - f22))


def _strassen_rhs(b11, b12, b21, b22):
  c = lambda b: b.astype(BF16)
  return (c(b11 + b22), c(b11), c(b12 - b22), c(b21 - b11), c(b22),
          c(b11 + b12), c(b21 + b22))


def _strassen_out(m1, m2, m3, m4, m5, m6, m7):
  return m1 + m4 - m5 + m7, m3 + m5, m2 + m4, m1 - m2 + m3 + m6


_ORDER = (2, 3, 0, 4, 6, 1, 5)


def _kernel(xt_hbm, wqkv_hbm, wo_hbm, wg_hbm, wu_hbm, wdt_hbm, c_hbm, wmod_hbm,
            out_hbm,
            xt_v, wqkv_v, wo_v, wg_v, wu_v, wdt_v, c_v, wmod_v,
            mod_v, wqkvt_v, wot_v, h1_v, ob_v, qkv_v, edge_v, qt_v, kt_v, vt_v, ot_v, x1_v,
            hb_v, hr_v, acc_v, out_v, in_sem, out_sem):
  d_model, seq = xt_hbm.shape
  d_ff = wg_hbm.shape[1]
  dh = d_model // N_HEADS
  n_tiles = seq // TILE
  fc = d_ff // NC
  fh = FS // 2
  kh = 256
  mh = d_model // 2
  half = TILE // 2

  sems = iter(range(in_sem.shape[0]))
  copy = lambda src, dst: pltpu.make_async_copy(src, dst, in_sem.at[next(sems)])
  cols_copy = lambda src, dst, a, b: copy(src.at[:, pl.ds(a, b - a)],
                                          dst.at[:, pl.ds(a, b - a)])
  c_cp = copy(c_hbm, c_v)
  wmod_cps = [cols_copy(wmod_hbm, wmod_v, 0, 2 * d_model),
              cols_copy(wmod_hbm, wmod_v, 2 * d_model, 6 * d_model)]
  qkv_cuts = (0, 640, 1152, 3 * d_model)
  wqkv_cps = [cols_copy(wqkv_hbm, wqkv_v, a, b)
              for a, b in zip(qkv_cuts, qkv_cuts[1:])]
  wo_cp = copy(wo_hbm, wo_v)
  x_cps = [copy(xt_hbm.at[:, pl.ds(i * TILE, TILE)], xt_v.at[i])
           for i in range(n_tiles)]
  ff_cps = [copy(w_hbm.at[:, pl.ds(j * fc, fc)], w_v.at[j])
            for j in range(NC)
            for w_hbm, w_v in ((wg_hbm, wg_v), (wu_hbm, wu_v), (wdt_hbm, wdt_v))]
  for cp in (c_cp, x_cps[0], wmod_cps[0], *wqkv_cps, x_cps[1], wo_cp,
             wmod_cps[1], *x_cps[2:], *ff_cps):
    cp.start()

  c_cp.wait()
  cv = c_v[...].astype(F32)
  sc = cv * jax.nn.sigmoid(cv)
  sc_col = jnp.broadcast_to(sc, (LANES, d_model)).T

  def modulation(lo, hi):
    for j in range(lo * d_model // LANES, hi * d_model // LANES):
      cols = pl.ds(j * LANES, LANES)
      row = jnp.sum(wmod_v[:, cols].astype(F32) * sc_col, axis=0, keepdims=True)
      mod_v[cols, :] = jnp.broadcast_to(row, (LANES, LANES)).T
    for part in (1, 4):
      if lo <= part < hi:
        rows = pl.ds(part * d_model, d_model)
        mod_v[rows, :] = mod_v[rows, :] + 1.0

  def mod(part, n=1, lo=0, size=d_model):
    return _tile_lanes(mod_v[pl.ds(part * d_model + lo, size), :], n)

  lane = lax.broadcasted_iota(jnp.int32, (HALO, LANES), 1)

  target = [None]

  def anchor(vals, link=0):
    regs = []
    for v in vals:
      v = pltpu.bitcast(v, jnp.int32)
      regs += [v[i:i + 8] for i in range(0, v.shape[0], 8)]
    v = regs[0]
    for r in regs[1:]:
      v = v | r
      for _ in range(link):
        v = v ^ lax.shift_right_logical(v, 1)
    if target[0] is not None:
      if target[0] is ob_v:
        ob_v[1, 0, pl.ds(0, 8), :] = v
      else:
        h1_v[1, pl.ds(0, 8), pl.ds(0, LANES)] = v

  def opaque_zero(s, k):
    return lax.shift_right_logical(s + k, 16)

  stats = {}

  def moments(load, key):
    inv_d = 1.0 / d_model
    mean = jnp.sum(load(0), axis=0, keepdims=True) * inv_d
    xc = load(1) - mean
    var = jnp.sum(xc * xc, axis=0, keepdims=True) * inv_d
    rstd = lax.rsqrt(var + LN_EPS)
    stats[key] = (mean, rstd)
    if ANCHOR_ST:
      anchor([jnp.broadcast_to(rstd, (8, LANES))])

  def normalize(x, key, part, lo, size):
    mean, rstd = stats[key]
    return (x - mean) * rstd * mod(part + 1, 1, lo, size) + mod(part, 1, lo, size)

  def norm1_stats(s, b):
    cols = pl.ds(b * LANES, LANES)
    moments(lambda k: xt_v[s + opaque_zero(s, 32 + k), :, cols].astype(F32), (1, b))

  def norm1(s, b):
    cols = pl.ds(b * LANES, LANES)
    x = xt_v[s + opaque_zero(s, 34), :, cols].astype(F32)
    h1_v[0, :, cols] = h = _words(normalize(x, (1, b), 0, 0, d_model).astype(BF16))
    if ANCHOR_L:
      anchor([h])

  def project_qkv(z, r):
    qkv = _dot(_halves(wqkvt_v[pl.ds(r * QC // 2, QC // 2), :]), _halves(h1_v[z]))
    if PACK_T:
      qkv = _words(qkv.astype(BF16))
    size = qkv.shape[0]
    for b in range(NB):
      qkv_v[b, pl.ds(r * size, size), :] = qkv[:, b * LANES:(b + 1) * LANES]

  def to_token_major(z, part, i, n):
    buf = (qt_v, kt_v, vt_v)[part]
    m = dh // 2 if PACK_T else dh
    for j in range(i * m // n, (i + 1) * m // n):
      rows = pl.ds(part * m * N_HEADS + j, N_HEADS, stride=m)
      t = jnp.concatenate([qkv_v[b, rows, :] for b in range(NB)], axis=0).T
      if part:
        tail = jnp.where(lane < LANES - N_HEADS, t[LANES - HALO:], edge_v[part - 1, j])
        edge_v[part - 1, j] = t[LANES - HALO:]
        t = jnp.concatenate([pltpu.roll(tail, N_HEADS, 1), t], axis=0)
      if PACK_T:
        buf[2 * j] = pltpu.bitcast(t << 16, F32)
        buf[2 * j + 1] = pltpu.bitcast(t & -65536, F32)
      else:
        buf[j] = t

  probs = {}

  def scores(s, zz, a):
    rows = 8 * G
    r0 = a * rows
    z = lax.shift_right_logical(s + a, 16)
    scale = dh ** -0.5
    logits = [None] * WINDOW
    for d in range(dh):
      q = qt_v[z + d, pl.ds(r0, rows), :]
      for w in range(WINDOW):
        t = q * kt_v[z + d, pl.ds(HALO + r0 - DILATION * w, rows), :]
        logits[w] = t if d == 0 else logits[w] + t
    for w in range(WINDOW):
      logits[w] = logits[w] * scale
      if r0 < DILATION * w:
        pos = (lax.broadcasted_iota(jnp.int32, (rows, LANES), 0) + s * TILE + r0
               + lax.broadcasted_iota(jnp.int32, (rows, LANES), 1)
               // N_HEADS * LANES)
        logits[w] = jnp.where(pos >= DILATION * w, logits[w], MASK_VALUE)
    m = functools.reduce(jnp.maximum, logits)
    e = [jnp.exp(l - m) for l in logits]
    inv = 1.0 / functools.reduce(jnp.add, e)
    probs[a] = [x_ * inv for x_ in e]
    if ANCHOR_S:
      anchor([inv])

  def mix(s, zz, a):
    rows = 8 * G
    r0 = a * rows
    z = lax.shift_right_logical(s + a, 16)
    p = probs.pop(a)
    outs = []
    for d in range(dh):
      o = None
      for w in range(WINDOW):
        t = p[w] * vt_v[z + d, pl.ds(HALO + r0 - DILATION * w, rows), :]
        o = t if o is None else o + t
      ot_v[d // 2, pl.ds(2 * r0 + d % 2, rows, stride=2), :] = o
      outs.append(o)
    anchor(outs, LINK)

  def to_feature_major(z, i, n):
    pairs = dh // 2
    for d in range(i * pairs // n, (i + 1) * pairs // n):
      t = _words(ot_v[z + d].astype(BF16)).T
      for b in range(NB):
        ob_v[0, b, pl.ds(d, N_HEADS, stride=pairs), :] = t[b * N_HEADS:(b + 1) * N_HEADS]

  def project_out(s, z, r):
    rows = pl.ds(r * WC, WC)
    x1_v[s, rows, :] = (xt_v[s, rows, :].astype(F32)
                        + mod(2, NB, r * WC, WC) * _dot(_halves(wot_v[pl.ds(r * WC // 2, WC // 2), :]), jnp.concatenate([_halves(ob_v[z, b]) for b in range(NB)], axis=1)))

  def norm2_stats(s, b):
    cols = pl.ds(b * LANES, LANES)
    moments(lambda k: x1_v[s + opaque_zero(s, 40 + k), :, cols], (2, b))

  def norm2(s, b, i):
    lo, hi = pl.ds(b * LANES, LANES), pl.ds(half + b * LANES, LANES)
    t = s + opaque_zero(s, 42)

    def h2(col, row, size):
      cols = (lo, hi)[col]
      return normalize(x1_v[t, pl.ds(row, size), cols], (2, b + col * NB // 2), 3, row, size)

    r = i * MR
    bs = _strassen_rhs(h2(0, r, MR), h2(1, r, MR), h2(0, kh + r, MR), h2(1, kh + r, MR))
    for j in range(7):
      hb_v[s, j, pl.ds(r // 2, MR // 2), lo] = _words(bs[j])
    outs = list(bs)
    if r == 0:
      for col in range(2):
        rest = h2(col, 2 * kh, d_model - 2 * kh).astype(BF16)
        hr_v[s, :, (lo, hi)[col]] = _words(rest)
        outs.append(rest)
    anchor(outs)

  def run(order, s, s_prev, s_next2):
    first, *rest = order.split("|")
    run_block(first, s, s_prev, s_next2)
    for part in rest:
      pl.when(opaque_zero(s, 50) == 0)(functools.partial(run_block, part, s, s_prev, s_next2))

  def run_block(order, s, s_prev, s_next2):
    z = lax.shift_right_logical(s + 17, 16)
    pending = []
    names = order.split(",")
    for n, name in enumerate(names):
      nxt = [x[0] for x in names[n + 1:] if x[0] in "QW"]
      target[0] = None if not nxt else h1_v if nxt[0] == "Q" else ob_v
      kind = name.rstrip("0123456789")
      i = int(name[len(kind):])
      if kind == "L": norm1(s_next2, i)
      elif kind == "l": norm1_stats(s_next2, i)
      elif kind == "m": norm2_stats(s_prev, i)
      elif kind == "M": norm2(s_prev, *divmod(i, kh // MR))
      elif kind == "U": to_feature_major(z, i, NT)
      elif kind in "QW":
        project_qkv(z, i) if kind == "Q" else project_out(s, z, i)
      elif kind == "S": scores(s, z, i)
      elif kind == "P": mix(s, z, i)
      elif kind[0] == "T": to_token_major(z, "qkv".index(kind[1]), i, NT)
      else: raise ValueError(name)
    target[0] = None

  edge_v[...] = jnp.zeros(edge_v.shape, edge_v.dtype)
  x1_v[0] = jnp.zeros(x1_v.shape[1:], F32)
  x_cps[0].wait()
  wmod_cps[0].wait()
  modulation(0, 2)
  for b in range(NB):
    norm1_stats(jnp.int32(0), b)
    norm1(jnp.int32(0), b)
  done = 0
  for cp, a, b in zip(wqkv_cps, qkv_cuts, qkv_cuts[1:]):
    cp.wait()
    wqkvt_v[pl.ds(a // 2, (b - a) // 2), :] = _words(wqkv_v[:, pl.ds(a, b - a)].T)
    while (done + 1) * QC <= b:
      project_qkv(0, done)
      done += 1
  if PRO_T:
    for part in range(3):
      to_token_major(0, part, 0, 1)
  x_cps[1].wait()
  for b in range(NB):
    norm1_stats(jnp.int32(1), b)
    norm1(jnp.int32(1), b)
  wo_cp.wait()
  wot_v[...] = _words(wo_v[...].T)
  wmod_cps[1].wait()
  modulation(2, 6)
  for cp in x_cps[2:]:
    cp.wait()

  @pl.loop(0, n_tiles - 1)
  def _(s):
    run(BODY, s, jnp.maximum(s - 1, 0), jnp.minimum(s + 2, n_tiles - 1))

  last = n_tiles - 1
  tail = [n for n in BODY.replace("|", ",").split(",") if n[0] in TAIL]
  if tail:
    run(",".join(tail), jnp.int32(last), jnp.int32(last - 1), None)
  for b in range(NB):
    norm2_stats(jnp.int32(last), b)
  for i in range(2 * kh // MR):
    norm2(jnp.int32(last), *divmod(i, kh // MR))

  for cp in ff_cps:
    cp.wait()

  def out_copy(i):
    cols = pl.ds(pl.multiple_of(i * TILE, TILE), TILE)
    return pltpu.make_async_copy(out_v.at[i], out_hbm.at[:, cols], out_sem.at[i])

  @pl.loop(0, n_tiles)
  def _(i):
    if SKIP_FFN:
      out_v[i] = (x1_v[i] + hb_v[i, 0, 0:8, 0:128].astype(F32)[0:1, 0:1] + hr_v[i, 0:8, 0:128].astype(F32)[0:1, 0:1]).astype(BF16)
      out_copy(i).start()
      return
    def step(j):
      def project(w_v, c0):
        r = _dot_tn(w_v[j, pl.ds(2 * kh, d_model - 2 * kh), pl.ds(c0, FS)], _halves(hr_v[i]))
        a = _strassen_lhs(w_v[j, pl.ds(0, kh), pl.ds(c0, fh)],
                          w_v[j, pl.ds(kh, kh), pl.ds(c0, fh)],
                          w_v[j, pl.ds(0, kh), pl.ds(c0 + fh, fh)],
                          w_v[j, pl.ds(kh, kh), pl.ds(c0 + fh, fh)])
        m = {k: _dot_tn(a[k], _halves(hb_v[i, k])) for k in _ORDER}
        c11, c12, c21, c22 = _strassen_out(*(m[k] for k in range(7)))
        return (c11 + r[:fh, :half], c12 + r[:fh, half:],
                c21 + r[fh:, :half], c22 + r[fh:, half:])

      acc = None
      for c0 in range(0, fc, FS):
        g = project(wg_v, c0)
        u = project(wu_v, c0)
        b = _strassen_rhs(*(gg * uu for gg, uu in zip(g, u)))
        a = _strassen_lhs(wdt_v[j, pl.ds(0, mh), pl.ds(c0, fh)],
                          wdt_v[j, pl.ds(0, mh), pl.ds(c0 + fh, fh)],
                          wdt_v[j, pl.ds(mh, mh), pl.ds(c0, fh)],
                          wdt_v[j, pl.ds(mh, mh), pl.ds(c0 + fh, fh)])
        m = {k: _dot(a[k], b[k]) for k in _ORDER}
        acc = m if acc is None else {k: acc[k] + m[k] for k in _ORDER}
      return acc

    @pl.loop(0, NC)
    def _(j):
      acc = step(j)
      for k in _ORDER:
        acc_v[k] = jnp.where(j > 0, acc_v[k], 0.0) + acc[k]
    c11, c12, c21, c22 = _strassen_out(*(acc_v[k] for k in range(7)))
    y = jnp.concatenate([jnp.concatenate([c11, c12], axis=1),
                         jnp.concatenate([c21, c22], axis=1)], axis=0)
    out_v[i] = (x1_v[i] + mod(5, NB) * y).astype(out_v.dtype)
    out_copy(i).start()

  for i in range(n_tiles):
    out_copy(i).wait()


@jax.jit
def pallas_adaLN_cond__sliding_local_dilated__glu_gated_bilinear__prompt_kernel(
    A_x, A_wqkv, A_wo, B_x, B_w_gate, B_w_up, B_w_down, c, w_mod):
  del B_x
  batch, seq, d_model = A_x.shape
  d_ff = B_w_gate.shape[1]
  dh = d_model // N_HEADS
  n_tiles = seq // TILE
  fc = d_ff // NC
  assert batch == 1 and seq % TILE == 0 and fc % FS == 0 and FS % 256 == 0
  hbm = pl.BlockSpec(memory_space=pltpu.HBM)
  operands = (A_x.reshape(seq, d_model).T, A_wqkv, A_wo, B_w_gate, B_w_up,
              B_w_down.T, c, w_mod)
  like = lambda a: pltpu.VMEM(a.shape, a.dtype)
  out_t = pl.pallas_call(
      _kernel,
      in_specs=[hbm] * len(operands),
      out_specs=hbm,
      out_shape=jax.ShapeDtypeStruct((d_model, seq), A_x.dtype),
      scratch_shapes=[
          pltpu.VMEM((n_tiles, d_model, TILE), A_x.dtype),
          like(A_wqkv), like(A_wo),
          *[pltpu.VMEM((NC, d_model, fc), BF16)] * 3,
          like(c), like(w_mod),
          pltpu.VMEM((6 * d_model, LANES), F32),
          pltpu.VMEM((3 * d_model // 2, d_model), jnp.int32),
          pltpu.VMEM((d_model // 2, d_model), jnp.int32),
          pltpu.VMEM((2, d_model // 2, TILE), jnp.int32),
          pltpu.VMEM((2, NB, d_model // 2, LANES), jnp.int32),
          (pltpu.VMEM((NB, 3 * d_model // 2, LANES), jnp.int32) if PACK_T else pltpu.VMEM((NB, 3 * d_model, LANES), F32)),
          (pltpu.VMEM((2, dh // 2, HALO, LANES), jnp.int32) if PACK_T else pltpu.VMEM((2, dh, HALO, LANES), F32)),
          pltpu.VMEM((dh + 1, LANES, LANES), F32),
          pltpu.VMEM((dh + 1, HALO + LANES, LANES), F32),
          pltpu.VMEM((dh + 1, HALO + LANES, LANES), F32),
          pltpu.VMEM((dh // 2, 2 * LANES, LANES), F32),
          pltpu.VMEM((n_tiles, d_model, TILE), F32),
          pltpu.VMEM((n_tiles, 7, 128, TILE // 2), jnp.int32),
          pltpu.VMEM((n_tiles, (d_model - 512) // 2, TILE), jnp.int32),
          pltpu.VMEM((7, d_model // 2, TILE // 2), F32),
          pltpu.VMEM((n_tiles, d_model, TILE), A_x.dtype),
          pltpu.SemaphoreType.DMA((7 + n_tiles + 3 * NC,)),
          pltpu.SemaphoreType.DMA((n_tiles,)),
      ],
      compiler_params=pltpu.CompilerParams(vmem_limit_bytes=110 * 2**20, flags=FLAGS),
      name="adaln_window_attn_glu",
  )(*operands)
  return out_t.T.reshape(batch, seq, d_model)
```

```python
import functools

import jax
import jax.numpy as jnp
from jax import lax
import jax.experimental.pallas as pl
import jax.experimental.pallas.tpu as pltpu

N_HEADS = 32
WINDOW = 8
DILATION = 2
LN_EPS = 1e-5
MASK_VALUE = -1000000000.0
LANES = 128
SUBLANES = 8
NB = LANES // N_HEADS
TILE = NB * LANES
HALO = 16

NC = 3
FS = 1536
QC = 64
MR = 64
CHAINS = ((2, 2), (2, 2))
TAIL_WAYS = (8, 9)
TAIL_CHAINS = 3
WAY_S = 2
GATE = 2
GATE_M = True
WAY_P = 3
KH = 256
DMA_CUTS = (0, 512, 1728)
Q0_CUTS = (0, 512, 1280, 1728)
X_ORDER = (("a", 1, 17), ("u", 17, 18), ("l", 18, 22), ("m", 22, 26))
Y_ORDER = (("t", 0, 9), ("L4", 0, 8))
ONLY_LOOP = False
ANCHOR_ST = True
TAIL_ORDER = None
PRO_ORDER = None
ANCHOR_L = False
SKIP_FFN = False
FLAGS = None

F32 = jnp.float32
BF16 = jnp.bfloat16
I32 = jnp.int32
_TN = (((0,), (0,)), ((), ()))


def _dot_tn(a, b):
  return lax.dot_general(a, b, _TN, preferred_element_type=F32)


def _dot(a, b):
  return jnp.dot(a, b, preferred_element_type=F32)


def _load_bf16(ref, lead, lo, size):
  words = ref.bitcast(I32)[(*lead, pl.ds(lo // 2, size // 2), slice(None))]
  return pltpu.bitcast(words, BF16)


def _lane_blocks(ref, lead, lo, size):
  n = ref.shape[len(lead)]
  return jnp.concatenate(
      [_load_bf16(ref, (*lead, b), lo, size) for b in range(n)], axis=1)


def _column_sum(x, chains=2):
  size = chains * SUBLANES
  acc = functools.reduce(jnp.add, [x[i:i + size] for i in range(0, x.shape[0], size)])
  return jnp.sum(acc, axis=0, keepdims=True)


def _after(x, earlier, zero):
  if earlier is None:
    return x
  return pltpu.bitcast(
      pltpu.bitcast(x, I32) | (pltpu.bitcast(earlier, I32) & zero), F32)


def _strassen_lhs(a11, a12, a21, a22):
  f11, f12, f21, f22 = (a.astype(F32) for a in (a11, a12, a21, a22))
  c = lambda a: a.astype(BF16)
  return (c(f11 + f22), c(f21 + f22), a11, a22, c(f11 + f12), c(f21 - f11),
          c(f12 - f22))


def _strassen_rhs(b11, b12, b21, b22):
  c = lambda b: b.astype(BF16)
  return (c(b11 + b22), c(b11), c(b12 - b22), c(b21 - b11), c(b22),
          c(b11 + b12), c(b21 + b22))


def _strassen_out(m1, m2, m3, m4, m5, m6, m7):
  return m1 + m4 - m5 + m7, m3 + m5, m2 + m4, m1 - m2 + m3 + m6


_ORDER = (2, 3, 0, 4, 6, 1, 5)


def _interleave(matmuls, *placed):
  slots = [[m] for m in matmuls]
  for pieces, lo, hi in placed:
    for k, p in enumerate(pieces):
      slots[lo + k * (hi - lo) // len(pieces)].append(p)
  return [p for slot in slots for p in slot]


def _kernel(xt_hbm, wqkv_hbm, wo_hbm, wg_hbm, wu_hbm, wdt_hbm, c_hbm, wmod_hbm,
            out_hbm,
            xt_v, wqkv_v, wo_v, wg_v, wu_v, wdt_v, c_v, wmod_v,
            sc_v, mod_v, stat_v, wqkvt_v, wot_v, h1_v, ob_v, qkv_v, edge_v, qt_v, kt_v,
            vt_v, ot_v, op_v, x1_v, hb_v, hr_v, acc_v, out_v, in_sem, out_sem):
  d_model, seq = xt_hbm.shape
  d_ff = wg_hbm.shape[1]
  dh = d_model // N_HEADS
  pairs = dh // 2
  n_tiles = seq // TILE
  last = n_tiles - 1
  fc = d_ff // NC
  fh = FS // 2
  mh = d_model // 2
  half = TILE // 2

  sems = iter(range(in_sem.shape[0]))
  copy = lambda src, dst: pltpu.make_async_copy(src, dst, in_sem.at[next(sems)])

  def col_copies(src, dst, cuts):
    return [copy(src.at[:, pl.ds(a, b - a)], dst.at[:, pl.ds(a, b - a)])
            for a, b in zip(cuts, cuts[1:])]

  mod_cuts = (0, 3, 6, 9, 14, 6 * d_model // LANES)
  c_cp = copy(c_hbm, c_v)
  wmod_cps = col_copies(wmod_hbm, wmod_v, [j * LANES for j in mod_cuts])
  wqkv_cps = col_copies(wqkv_hbm, wqkv_v, DMA_CUTS)
  wo_cp = copy(wo_hbm, wo_v)
  x_cps = [copy(xt_hbm.at[:, pl.ds(i * TILE, TILE)], xt_v.at[i])
           for i in range(n_tiles)]
  ff_cps = [copy(w_hbm.at[:, pl.ds(j * fc, fc)], w_v.at[j])
            for j in range(NC)
            for w_hbm, w_v in ((wg_hbm, wg_v), (wu_hbm, wu_v), (wdt_hbm, wdt_v))]
  for cp in (c_cp, x_cps[0], *wmod_cps[:3], *wqkv_cps, x_cps[1], wo_cp,
             wmod_cps[3], *x_cps[2:], wmod_cps[4], *ff_cps):
    cp.start()

  def opaque_zero(s, k):
    return lax.shift_right_logical(s + k, 16)

  target = [None]
  results = []

  def anchor(vals):
    if target[0] is None:
      return
    regs = []
    for v in vals:
      v = pltpu.bitcast(v, I32)
      regs += [v[i:i + SUBLANES] for i in range(0, v.shape[0], SUBLANES)]
    target[0].bitcast(I32)[1, 0, pl.ds(0, SUBLANES), :] = functools.reduce(
        jnp.bitwise_or, regs)

  def modulation(s, j, chains=1):
    if len(results) >= GATE:
      sc_v[1, pl.ds(0, SUBLANES), :] = results[-GATE]
    cols = pl.ds(j * LANES, LANES)
    row = _column_sum(wmod_v[:, cols].astype(F32) * sc_v[opaque_zero(s, 60)],
                      chains)
    anchor([jnp.broadcast_to(row, (SUBLANES, LANES))])
    store_modulation(j, row)

  def store_modulation(j, row):
    part = (j * LANES + lax.broadcasted_iota(I32, (1, LANES), 1)) // d_model
    row = jnp.where((part == 1) | (part == 4), row + 1.0, row)
    mod_v[pl.ds(j * LANES, LANES), :] = jnp.broadcast_to(row, (LANES, LANES)).T

  def modulation_mxu(lo, hi):
    cv = c_v[...].astype(F32)
    sc = jnp.broadcast_to(cv * jax.nn.sigmoid(cv), (2 * SUBLANES, d_model))
    rows = _dot(sc.astype(BF16), wmod_v[:, pl.ds(lo * LANES, (hi - lo) * LANES)])
    for j in range(lo, hi):
      store_modulation(j, rows[:1, (j - lo) * LANES:(j - lo + 1) * LANES])

  def mod(part, lo, size, n=1):
    col = mod_v[pl.ds(part * d_model + lo, size), :]
    return col if n == 1 else jnp.concatenate([col] * n, axis=1)

  def moments(load, which, s, b, chains):
    inv_d = 1.0 / d_model
    mean = _column_sum(load(0), chains) * inv_d
    xc = load(1) - mean
    var = _column_sum(xc * xc, chains) * inv_d
    for k, v in enumerate((mean, lax.rsqrt(var + LN_EPS))):
      stat_v[which, s, k, b] = v = jnp.broadcast_to(v, (SUBLANES, LANES))
    if ANCHOR_ST is True or ANCHOR_ST == which:
      anchor([v])

  def normalize(x, which, s, b, lo):
    size = x.shape[0]
    mean, rstd = (jnp.tile(stat_v[which, s, k, b], (size // SUBLANES, 1))
                  for k in range(2))
    return ((x - mean) * rstd * mod(3 * which + 1, lo, size)
            + mod(3 * which, lo, size))

  def norm1_stats(s, b):
    if len(results) >= GATE:
      xt_v[n_tiles, pl.ds(0, 2 * SUBLANES), pl.ds(0, LANES)] = pltpu.bitcast(
          results[-GATE], BF16)
    cols = pl.ds(b * LANES, LANES)
    moments(lambda k: xt_v[s + opaque_zero(s, 32 + k), :, cols].astype(F32),
            0, s, b, 2)

  def hold_x():
    xt_v[n_tiles, pl.ds(0, 2 * SUBLANES), pl.ds(0, LANES)] = pltpu.bitcast(
        results[-1], BF16)

  def norm1(s, b, i=0, n=1):
    size = d_model // n
    rows = pl.ds(i * size, size)
    x = xt_v[s + opaque_zero(s, 34), rows, pl.ds(b * LANES, LANES)]
    h1_v[0, b, rows, :] = normalize(x.astype(F32), 0, s, b, i * size).astype(BF16)
    if ANCHOR_L:
      anchor([h1_v.bitcast(I32)[opaque_zero(s, 35), b, pl.ds(0, SUBLANES), :]])

  def project_qkv(s, lo, size=QC):
    qkv = _dot(_lane_blocks(wqkvt_v, (), lo, size)[:, :d_model],
               _lane_blocks(h1_v, (opaque_zero(s, 17),), 0, d_model))
    results.append(qkv[:SUBLANES, :LANES])
    for b in range(NB):
      qkv_v[b, pl.ds(lo, size), :] = qkv[:, b * LANES:(b + 1) * LANES].astype(BF16)

  def to_token_major(part, i, n=3):
    buf = (qt_v, kt_v, vt_v)[part]
    for j in range(i * pairs // n, (i + 1) * pairs // n):
      rows = pl.ds(part * mh + j, N_HEADS, stride=pairs)
      t = jnp.concatenate(
          [qkv_v.bitcast(I32)[b, rows, :] for b in range(NB)], axis=0).T
      if part:
        tail = jnp.where(
            lax.broadcasted_iota(I32, (HALO, LANES), 1) < LANES - N_HEADS,
            t[LANES - HALO:], edge_v[part - 1, j])
        edge_v[part - 1, j] = t[LANES - HALO:]
        t = jnp.concatenate([pltpu.roll(tail, N_HEADS, 1), t], axis=0)
      buf[2 * j] = pltpu.bitcast(t << 16, F32)
      buf[2 * j + 1] = pltpu.bitcast(t & -65536, F32)

  def attend(s, g, way_s, way_p):
    r0 = g * SUBLANES
    z = opaque_zero(s, g)
    window = lambda w: pl.ds(HALO + r0 - DILATION * w, SUBLANES)

    q = [qt_v[z + d, pl.ds(r0, SUBLANES), :] for d in range(dh)]
    logits = []
    for w in range(WINDOW):
      acc = None
      for d in range(dh):
        qd = q[d] if d else _after(q[d], logits[w - way_s] if w >= way_s else None, z)
        t = qd * kt_v[z + d, window(w), :]
        acc = t if d == 0 else acc + t
      logits.append(acc)
    for w in range(WINDOW):
      logits[w] = logits[w] * dh ** -0.5
      if r0 < DILATION * w:
        shape = (SUBLANES, LANES)
        pos = (s * TILE + r0 + lax.broadcasted_iota(I32, shape, 0)
               + lax.broadcasted_iota(I32, shape, 1) // N_HEADS * LANES)
        logits[w] = jnp.where(pos >= DILATION * w, logits[w], MASK_VALUE)
    m = functools.reduce(jnp.maximum, logits)
    e = [jnp.exp(l - m) for l in logits]
    inv = 1.0 / functools.reduce(jnp.add, e)
    p = [x * inv for x in e]
    outs = []
    for d in range(dh):
      o = None
      for w in range(WINDOW):
        pw = p[w] if w else _after(p[w], outs[d - way_p] if d >= way_p else None, z)
        t = pw * vt_v[z + d, window(w), :]
        o = t if o is None else o + t
      ot_v[d // 2, pl.ds(2 * r0 + d % 2, SUBLANES, stride=2), :] = o
      outs.append(o)
    if way_p < dh:
      anchor(outs[-way_p:])

  def to_feature_major(s, i, n=3):
    for j in range(i * pairs // n, (i + 1) * pairs // n):
      op_v[j] = ot_v[opaque_zero(s, 18) + j].astype(BF16)
      t = op_v.bitcast(I32)[j].T
      for b in range(NB):
        ob_v.bitcast(I32)[0, b, pl.ds(j, N_HEADS, stride=pairs), :] = (
            t[b * N_HEADS:(b + 1) * N_HEADS])

  def project_out(s, lo):
    y = _dot(_lane_blocks(wot_v, (), lo, QC)[:, :d_model],
             _lane_blocks(ob_v, (opaque_zero(s, 19),), 0, d_model))
    results.append(y[:SUBLANES, :LANES])
    rows = pl.ds(lo, QC)
    x1_v[s, rows, :] = xt_v[s, rows, :].astype(F32) + mod(2, lo, QC, NB) * y

  def norm2_stats(s, b, chains=2):
    if len(results) >= GATE and chains == 2:
      x1_v[n_tiles, pl.ds(0, SUBLANES), pl.ds(0, LANES)] = results[-GATE]
    cols = pl.ds(b * LANES, LANES)
    moments(lambda k: x1_v[s + opaque_zero(s, 40 + k), :, cols], 1, s, b, chains)

  def norm2(s, b, r):
    cols = pl.ds(b * LANES, LANES), pl.ds(half + b * LANES, LANES)

    def h2(side, row, size):
      return normalize(x1_v[s, pl.ds(row, size), cols[side]], 1, s,
                       b + side * NB // 2, row)

    outs = list(_strassen_rhs(h2(0, r, MR), h2(1, r, MR), h2(0, KH + r, MR),
                              h2(1, KH + r, MR)))
    for j in range(7):
      hb_v[j, b, pl.ds(r, MR), :] = outs[j]
    if r == 0:
      for side in range(2):
        hr_v[b + side * NB // 2] = h2(side, 2 * KH, d_model - 2 * KH).astype(BF16)

  def transpose_weights(w_v, wt_v, a, b):
    for k in range(0, d_model, LANES):
      size = min(LANES, d_model - k)
      t = w_v[pl.ds(k, size), pl.ds(a, b - a)].T
      if size < LANES:
        t = jnp.concatenate([t, jnp.zeros((b - a, LANES - size), BF16)], axis=1)
      wt_v[k // LANES, pl.ds(a, b - a), :] = t

  def transpose_wo():
    transpose_weights(wo_v, wot_v, 0, d_model)

  def run(steps):
    for n, (fn, *args) in enumerate(steps):
      nxt = [f for f, *_ in steps[n + 1:] if f in (project_qkv, project_out)]
      target[0] = (None if not nxt else h1_v if nxt[0] is project_qkv else ob_v)
      fn(*args)
    target[0] = None
    results.clear()

  def stats_steps(fn, s):
    return [(fn, s, b) for b in range(NB)]

  def norm1_steps(s, n=1):
    return [(norm1, s, b, i, n) for b in range(NB) for i in range(n)]

  def token_major_steps(parts):
    return [(to_token_major, part, i) for part in parts for i in range(3)]

  def attention_steps(s, ways):
    return [(attend, s, g, *ways) for g in range(LANES // SUBLANES)]

  zero = lax.fori_loop(0, 2, lambda i, z: z + opaque_zero(i, 1), jnp.int32(0))
  edge_v[...] = jnp.zeros(edge_v.shape, edge_v.dtype)
  x1_v[0] = jnp.zeros(x1_v.shape[1:], F32)
  c_cp.wait()
  cv = c_v[...].astype(F32)
  sc_v[0] = jnp.broadcast_to(cv * jax.nn.sigmoid(cv), (LANES, d_model)).T
  x_cps[0].wait()
  for b in range(NB):
    norm1_stats(zero, b)
  for cp, a, b in zip(wmod_cps[:3], mod_cuts, mod_cuts[1:]):
    cp.wait()
    for j in range(a, b):
      modulation(zero, j, 2)
  for b in range(NB):
    norm1(zero, b)

  waits = dict(zip(DMA_CUTS, wqkv_cps))
  if ONLY_LOOP:
    transpose_wo()
    transpose_weights(wqkv_v, wqkvt_v, 0, 3 * d_model)
  for a, b in zip(Q0_CUTS, Q0_CUTS[1:]) if not ONLY_LOOP else []:
    final = b == 3 * d_model
    if a in waits:
      waits[a].wait()
    if final:
      for cp in (x_cps[1], wo_cp, wmod_cps[3]):
        cp.wait()
    if a in waits:
      transpose_weights(wqkv_v, wqkvt_v, a, DMA_CUTS[DMA_CUTS.index(a) + 1])
    steps = [(project_qkv, zero, lo) for lo in range(a, b, QC)]
    if final:
      n = len(steps)
      P0, P1, P2, P3, P4 = PRO_ORDER or (0, 2, 2, 6, 3)
      steps = _interleave(
          steps,
          ([(modulation, zero, j) for j in range(mod_cuts[3], mod_cuts[4])], P0, P1),
          (stats_steps(norm1_stats, zero + 1), P2, P3),
          (token_major_steps([1]), 0, 3), ([(transpose_wo,)], P4, P4 + 1),
          (token_major_steps([2]), n - 1, n),
          ([(hold_x,)] + norm1_steps(zero + 1, 4), n - 1, n))
    elif a < d_model < b:
      n = (d_model - a) // QC
      steps = _interleave(steps, (token_major_steps([0]), n, n + 3))
    run(steps)
  for cp in x_cps[2:]:
    cp.wait()

  n_q, n_w = 3 * d_model // QC, d_model // QC

  @pl.loop(0, last)
  def _(s):
    s_next = jnp.minimum(s + 2, last)
    pieces = {
        "a": attention_steps(s, (WAY_S, WAY_P)),
        "u": [(to_feature_major, s, i) for i in range(3)],
        "m": stats_steps(norm2_stats, jnp.maximum(s - 1, 0)),
        "l": stats_steps(norm1_stats, s_next),
        "t": token_major_steps(range(3)),

        "L1": norm1_steps(s_next), "L2": norm1_steps(s_next, 2),
        "L4": norm1_steps(s_next, 4),
    }
    place = lambda order: [(pieces[k], lo, hi) for k, lo, hi in order]
    run(_interleave(
        [(project_qkv, s, lo) for lo in range(0, 3 * d_model, QC)],
        *place(X_ORDER)))

    @pl.when(opaque_zero(s, 50) == 0)
    def _():
      run(_interleave(
          [(project_out, s, lo) for lo in range(0, d_model, QC)],
          *place(Y_ORDER)))

  wmod_cps[4].wait()
  s = zero + last
  if not ONLY_LOOP: run([(modulation_mxu, mod_cuts[4], mod_cuts[5])] + stats_steps(norm2_stats, s - 1) + attention_steps(s, TAIL_WAYS)
      + [(to_feature_major, s, i) for i in range(3)]
      + [(project_out, s, lo) for lo in range(0, d_model, QC)]
      + [(norm2_stats, s, b, TAIL_CHAINS) for b in range(NB)])

  for cp in ff_cps:
    cp.wait()

  def out_copy(i):
    cols = pl.ds(pl.multiple_of(i * TILE, TILE), TILE)
    return pltpu.make_async_copy(out_v.at[i], out_hbm.at[:, cols], out_sem.at[i])

  @pl.loop(0, n_tiles)
  def _(i):
    for b in range(NB // 2):
      for r in range(0, KH, MR):
        norm2(i, b, r)
    if SKIP_FFN:
      out_v[i] = (x1_v[i] + hb_v[0, 0, 0:16, :].astype(F32)[0:1, 0:1] + hr_v[0, 0:16, :].astype(F32)[0:1, 0:1] + mod(5, 0, d_model, NB)).astype(BF16)
      out_copy(i).start()
      return

    def project(w_v, j, c0):
      r = _dot_tn(w_v[j, pl.ds(2 * KH, d_model - 2 * KH), pl.ds(c0, FS)],
                  _lane_blocks(hr_v, (), 0, d_model - 2 * KH))
      a = _strassen_lhs(w_v[j, pl.ds(0, KH), pl.ds(c0, fh)],
                        w_v[j, pl.ds(KH, KH), pl.ds(c0, fh)],
                        w_v[j, pl.ds(0, KH), pl.ds(c0 + fh, fh)],
                        w_v[j, pl.ds(KH, KH), pl.ds(c0 + fh, fh)])
      m = {k: _dot_tn(a[k], _lane_blocks(hb_v, (k,), 0, KH)) for k in _ORDER}
      c11, c12, c21, c22 = _strassen_out(*(m[k] for k in range(7)))
      return (c11 + r[:fh, :half], c12 + r[:fh, half:],
              c21 + r[fh:, :half], c22 + r[fh:, half:])

    @pl.loop(0, NC)
    def _(j):
      acc = None
      for c0 in range(0, fc, FS):
        g = project(wg_v, j, c0)
        u = project(wu_v, j, c0)
        b = _strassen_rhs(*(gg * uu for gg, uu in zip(g, u)))
        a = _strassen_lhs(wdt_v[j, pl.ds(0, mh), pl.ds(c0, fh)],
                          wdt_v[j, pl.ds(0, mh), pl.ds(c0 + fh, fh)],
                          wdt_v[j, pl.ds(mh, mh), pl.ds(c0, fh)],
                          wdt_v[j, pl.ds(mh, mh), pl.ds(c0 + fh, fh)])
        m = {k: _dot(a[k], b[k]) for k in _ORDER}
        acc = m if acc is None else {k: acc[k] + m[k] for k in _ORDER}
      for k in _ORDER:
        acc_v[k] = jnp.where(j > 0, acc_v[k], 0.0) + acc[k]

    c11, c12, c21, c22 = _strassen_out(*(acc_v[k] for k in range(7)))
    y = jnp.concatenate([jnp.concatenate([c11, c12], axis=1),
                         jnp.concatenate([c21, c22], axis=1)], axis=0)
    out_v[i] = (x1_v[i] + mod(5, 0, d_model, NB) * y).astype(out_v.dtype)
    out_copy(i).start()

  for i in range(n_tiles):
    out_copy(i).wait()


@jax.jit
def pallas_adaLN_cond__sliding_local_dilated__glu_gated_bilinear__prompt_kernel(
    A_x, A_wqkv, A_wo, B_x, B_w_gate, B_w_up, B_w_down, c, w_mod):
  del B_x
  batch, seq, d_model = A_x.shape
  d_ff = B_w_gate.shape[1]
  dh = d_model // N_HEADS
  n_tiles = seq // TILE
  fc = d_ff // NC
  assert batch == 1 and seq % TILE == 0 and fc % FS == 0 and FS % 256 == 0
  hbm = pl.BlockSpec(memory_space=pltpu.HBM)
  operands = (A_x.reshape(seq, d_model).T, A_wqkv, A_wo, B_w_gate, B_w_up,
              B_w_down.T, c, w_mod)
  like = lambda a: pltpu.VMEM(a.shape, a.dtype)
  out_t = pl.pallas_call(
      _kernel,
      in_specs=[hbm] * len(operands),
      out_specs=hbm,
      out_shape=jax.ShapeDtypeStruct((d_model, seq), A_x.dtype),
      scratch_shapes=[
          pltpu.VMEM((n_tiles + 1, d_model, TILE), A_x.dtype),
          like(A_wqkv), like(A_wo),
          *[pltpu.VMEM((NC, d_model, fc), BF16)] * 3,
          like(c), like(w_mod),
          pltpu.VMEM((2, d_model, LANES), F32),
          pltpu.VMEM((6 * d_model, LANES), F32),
          pltpu.VMEM((2, n_tiles, 2, NB, SUBLANES, LANES), F32),
          pltpu.VMEM((pl.cdiv(d_model, LANES), 3 * d_model, LANES), BF16),
          pltpu.VMEM((pl.cdiv(d_model, LANES), d_model, LANES), BF16),
          pltpu.VMEM((2, NB, d_model, LANES), BF16),
          pltpu.VMEM((2, NB, d_model, LANES), BF16),
          pltpu.VMEM((NB, 3 * d_model, LANES), BF16),
          pltpu.VMEM((2, dh // 2, HALO, LANES), I32),
          pltpu.VMEM((dh, LANES, LANES), F32),
          pltpu.VMEM((dh, HALO + LANES, LANES), F32),
          pltpu.VMEM((dh, HALO + LANES, LANES), F32),
          pltpu.VMEM((dh // 2, 2 * LANES, LANES), F32),
          pltpu.VMEM((dh // 2, 2 * LANES, LANES), BF16),
          pltpu.VMEM((n_tiles + 1, d_model, TILE), F32),
          pltpu.VMEM((7, NB // 2, KH, LANES), BF16),
          pltpu.VMEM((NB, d_model - 2 * KH, LANES), BF16),
          pltpu.VMEM((7, d_model // 2, TILE // 2), F32),
          pltpu.VMEM((n_tiles, d_model, TILE), A_x.dtype),
          pltpu.SemaphoreType.DMA((6 + len(DMA_CUTS) + n_tiles + 3 * NC,)),
          pltpu.SemaphoreType.DMA((n_tiles,)),
      ],
      compiler_params=pltpu.CompilerParams(vmem_limit_bytes=110 * 2**20,
                                           flags=FLAGS),
      name="adaln_window_attn_glu",
  )(*operands)
  return out_t.T.reshape(batch, seq, d_model)
```

```python
import functools

import jax
import jax.numpy as jnp
from jax import lax
import jax.experimental.pallas as pl
import jax.experimental.pallas.tpu as pltpu

N_HEADS = 32
WINDOW = 8
DILATION = 2
LN_EPS = 1e-5
MASK_VALUE = -1000000000.0
LANES = 128
SUBLANES = 8
NB = LANES // N_HEADS
TILE = NB * LANES
HALO = 16

NC = 3
FS = (1536,)
QC = 64
MR = 64
CHAINS = ((2, 2), (2, 2))
TAIL_WAYS = (8, 9)
TAIL_CHAINS = 3
ANCHOR_TW = False
GA_MXU = False
WO_AT = 'x'
FR = 32
NR = 32
FSKIP = 1
NORM_PARTS = ((None, 0), (1,), (2,), (3,), (4,), (5,))
WAY_S = 2
GATE = 2
GATE_M = True
WAY_P = 3
KH = 256
DMA_CUTS = (0, 512, 1728)
Q0_CUTS = (0, 512, 1280, 1728)
X_ORDER = (("a", 1, 17), ("u", 17, 18), ("l", 18, 22), ("m", 22, 26), ("w", 17, 18))
Y_ORDER = (("t", 0, 9), ("L4", 0, 8))
ONLY_LOOP = False
ANCHOR_ST = True
TAIL_ORDER = None
PRO_ORDER = None
ANCHOR_L = False
SKIP_FFN = False
FLAGS = None

F32 = jnp.float32
BF16 = jnp.bfloat16
I32 = jnp.int32
_TN = (((0,), (0,)), ((), ()))


def _dot_tn(a, b):
  return lax.dot_general(a, b, _TN, preferred_element_type=F32)


def _dot(a, b):
  return jnp.dot(a, b, preferred_element_type=F32)


def _load_bf16(ref, lead, lo, size):
  words = ref.bitcast(I32)[(*lead, pl.ds(lo // 2, size // 2), slice(None))]
  return pltpu.bitcast(words, BF16)


def _lane_blocks(ref, lead, lo, size):
  n = ref.shape[len(lead)]
  return jnp.concatenate(
      [_load_bf16(ref, (*lead, b), lo, size) for b in range(n)], axis=1)


def _column_sum(x, chains=2):
  size = chains * SUBLANES
  acc = functools.reduce(jnp.add, [x[i:i + size] for i in range(0, x.shape[0], size)])
  return jnp.sum(acc, axis=0, keepdims=True)


def _after(x, earlier, zero):
  if earlier is None:
    return x
  return pltpu.bitcast(
      pltpu.bitcast(x, I32) | (pltpu.bitcast(earlier, I32) & zero), F32)


def _registers(vals):
  regs = []
  for v in vals:
    v = pltpu.bitcast(v, I32)
    regs += [v[i:i + SUBLANES, k:k + LANES]
             for i in range(0, v.shape[0], SUBLANES)
             for k in range(0, v.shape[1], LANES)]
  return regs


def _strassen_lhs(a11, a12, a21, a22):
  f11, f12, f21, f22 = (a.astype(F32) for a in (a11, a12, a21, a22))
  c = lambda a: a.astype(BF16)
  return (c(f11 + f22), c(f21 + f22), a11, a22, c(f11 + f12), c(f21 - f11),
          c(f12 - f22))


def _strassen_rhs(b11, b12, b21, b22):
  c = lambda b: b.astype(BF16)
  return (c(b11 + b22), c(b11), c(b12 - b22), c(b21 - b11), c(b22),
          c(b11 + b12), c(b21 + b22))


def _strassen_out(m1, m2, m3, m4, m5, m6, m7):
  return m1 + m4 - m5 + m7, m3 + m5, m2 + m4, m1 - m2 + m3 + m6


_ORDER = (2, 3, 0, 4, 6, 1, 5)
ORDER_G = (2, 3, 1, 4, 0, 6, 5)
ORDER_D = (2, 3, 0, 4, 6, 1, 5)
ONLY_FFN = False
FGATE = 1
GROW = 0
_LHS_TERMS = (((1, 0), (1, 3)), ((1, 2), (1, 3)), ((1, 0),), ((1, 3),),
              ((1, 0), (1, 1)), ((1, 2), (-1, 0)), ((1, 1), (-1, 3)))


def _interleave(matmuls, *placed):
  slots = [[m] for m in matmuls]
  for pieces, lo, hi in placed:
    for k, p in enumerate(pieces):
      slots[lo + k * (hi - lo) // len(pieces)].append(p)
  return [p for slot in slots for p in slot]


def _kernel(xt_hbm, wqkv_hbm, wo_hbm, wg_hbm, wu_hbm, wdt_hbm, c_hbm, wmod_hbm,
            out_hbm,
            xt_v, wqkv_v, wo_v, wg_v, wu_v, wdt_v, c_v, wmod_v,
            sc_v, mod_v, stat_v, wqkvt_v, wot_v, h1_v, ob_v, qkv_v, edge_v, qt_v, kt_v,
            vt_v, ot_v, op_v, x1_v, hb_v, hr_v, lead_v, acc_v, out_v, in_sem, out_sem):
  d_model, seq = xt_hbm.shape
  d_ff = wg_hbm.shape[1]
  dh = d_model // N_HEADS
  pairs = dh // 2
  n_tiles = seq // TILE
  last = n_tiles - 1
  fc = d_ff // NC
  mh = d_model // 2
  half = TILE // 2

  sems = iter(range(in_sem.shape[0]))
  copy = lambda src, dst: pltpu.make_async_copy(src, dst, in_sem.at[next(sems)])

  def col_copies(src, dst, cuts):
    return [copy(src.at[:, pl.ds(a, b - a)], dst.at[:, pl.ds(a, b - a)])
            for a, b in zip(cuts, cuts[1:])]

  mod_cuts = (0, 3, 6, 9, 14, 6 * d_model // LANES)
  c_cp = copy(c_hbm, c_v)
  wmod_cps = col_copies(wmod_hbm, wmod_v, [j * LANES for j in mod_cuts])
  wqkv_cps = col_copies(wqkv_hbm, wqkv_v, DMA_CUTS)
  wo_cp = copy(wo_hbm, wo_v)
  x_cps = [copy(xt_hbm.at[:, pl.ds(i * TILE, TILE)], xt_v.at[i])
           for i in range(n_tiles)]
  ff_cps = [copy(w_hbm.at[:, pl.ds(j * fc, fc)], w_v.at[j])
            for j in range(NC)
            for w_hbm, w_v in ((wg_hbm, wg_v), (wu_hbm, wu_v), (wdt_hbm, wdt_v))]
  for cp in (c_cp, x_cps[0], *wmod_cps[:3], *wqkv_cps, x_cps[1], wo_cp,
             wmod_cps[3], *x_cps[2:], wmod_cps[4], *ff_cps):
    cp.start()

  def opaque_zero(s, k):
    return lax.shift_right_logical(s + k, 16)

  target = [None]
  newest = [None]
  results = []

  def anchor(vals):
    if target[0] is None:
      return
    target[0].bitcast(I32)[1, 0, pl.ds(0, SUBLANES), :] = functools.reduce(
        jnp.bitwise_or, _registers(vals))

  def modulation(s, j, chains=1):
    if len(results) >= GATE:
      sc_v[1, pl.ds(0, SUBLANES), :] = results[-GATE]
    cols = pl.ds(j * LANES, LANES)
    row = _column_sum(wmod_v[:, cols].astype(F32) * sc_v[opaque_zero(s, 60)],
                      chains)
    anchor([jnp.broadcast_to(row, (SUBLANES, LANES))])
    store_modulation(j, row)

  def store_modulation(j, row):
    part = (j * LANES + lax.broadcasted_iota(I32, (1, LANES), 1)) // d_model
    row = jnp.where((part == 1) | (part == 4), row + 1.0, row)
    mod_v[pl.ds(j * LANES, LANES), :] = jnp.broadcast_to(row, (LANES, LANES)).T

  def modulation_mxu(lo, hi):
    cv = c_v[...].astype(F32)
    sc = jnp.broadcast_to(cv * jax.nn.sigmoid(cv), (2 * SUBLANES, d_model))
    rows = _dot(sc.astype(BF16), wmod_v[:, pl.ds(lo * LANES, (hi - lo) * LANES)])
    for j in range(lo, hi):
      store_modulation(j, rows[:1, (j - lo) * LANES:(j - lo + 1) * LANES])

  def mod(part, lo, size, n=1):
    col = mod_v[pl.ds(part * d_model + lo, size), :]
    return col if n == 1 else jnp.concatenate([col] * n, axis=1)

  def moments(load, which, s, b, chains):
    inv_d = 1.0 / d_model
    mean = _column_sum(load(0), chains) * inv_d
    xc = load(1) - mean
    var = _column_sum(xc * xc, chains) * inv_d
    for k, v in enumerate((mean, lax.rsqrt(var + LN_EPS))):
      stat_v[which, s, k, b] = v = jnp.broadcast_to(v, (SUBLANES, LANES))
    if ANCHOR_ST is True or ANCHOR_ST == which:
      anchor([v])

  def normalize(x, which, s, b, lo):
    size = x.shape[0]
    mean, rstd = (jnp.tile(stat_v[which, s, k, b], (size // SUBLANES, 1))
                  for k in range(2))
    return ((x - mean) * rstd * mod(3 * which + 1, lo, size)
            + mod(3 * which, lo, size))

  def norm1_stats(s, b):
    if len(results) >= GATE:
      xt_v[n_tiles, pl.ds(0, 2 * SUBLANES), pl.ds(0, LANES)] = pltpu.bitcast(
          results[-GATE], BF16)
    cols = pl.ds(b * LANES, LANES)
    moments(lambda k: xt_v[s + opaque_zero(s, 32 + k), :, cols].astype(F32),
            0, s, b, 2)

  def hold_x():
    xt_v[n_tiles, pl.ds(0, 2 * SUBLANES), pl.ds(0, LANES)] = pltpu.bitcast(
        newest[0], BF16)

  def norm1(s, b, i=0, n=1):
    size = d_model // n
    rows = pl.ds(i * size, size)
    x = xt_v[s + opaque_zero(s, 34), rows, pl.ds(b * LANES, LANES)]
    h1_v[0, b, rows, :] = normalize(x.astype(F32), 0, s, b, i * size).astype(BF16)
    if ANCHOR_L:
      anchor([h1_v.bitcast(I32)[opaque_zero(s, 35), b, pl.ds(0, SUBLANES), :]])

  def project_qkv(s, lo, size=QC):
    qkv = _dot(_lane_blocks(wqkvt_v, (), lo, size)[:, :d_model],
               _lane_blocks(h1_v, (opaque_zero(s, 17),), 0, d_model))
    results.append(qkv[:SUBLANES, :LANES])
    newest[0] = qkv[-SUBLANES:, -LANES:]
    for b in range(NB):
      qkv_v[b, pl.ds(lo, size), :] = qkv[:, b * LANES:(b + 1) * LANES].astype(BF16)

  def to_token_major(part, i, n=3):
    buf = (qt_v, kt_v, vt_v)[part]
    for j in range(i * pairs // n, (i + 1) * pairs // n):
      rows = pl.ds(part * mh + j, N_HEADS, stride=pairs)
      t = jnp.concatenate(
          [qkv_v.bitcast(I32)[b, rows, :] for b in range(NB)], axis=0).T
      if part:
        tail = jnp.where(
            lax.broadcasted_iota(I32, (HALO, LANES), 1) < LANES - N_HEADS,
            t[LANES - HALO:], edge_v[part - 1, j])
        edge_v[part - 1, j] = t[LANES - HALO:]
        t = jnp.concatenate([pltpu.roll(tail, N_HEADS, 1), t], axis=0)
      buf[2 * j] = pltpu.bitcast(t << 16, F32)
      buf[2 * j + 1] = pltpu.bitcast(t & -65536, F32)

  def attend(s, g, way_s, way_p):
    r0 = g * SUBLANES
    z = opaque_zero(s, g)
    window = lambda w: pl.ds(HALO + r0 - DILATION * w, SUBLANES)

    q = [qt_v[z + d, pl.ds(r0, SUBLANES), :] for d in range(dh)]
    logits = []
    for w in range(WINDOW):
      acc = None
      for d in range(dh):
        qd = q[d] if d else _after(q[d], logits[w - way_s] if w >= way_s else None, z)
        t = qd * kt_v[z + d, window(w), :]
        acc = t if d == 0 else acc + t
      logits.append(acc)
    for w in range(WINDOW):
      logits[w] = logits[w] * dh ** -0.5
      if r0 < DILATION * w:
        shape = (SUBLANES, LANES)
        pos = (s * TILE + r0 + lax.broadcasted_iota(I32, shape, 0)
               + lax.broadcasted_iota(I32, shape, 1) // N_HEADS * LANES)
        logits[w] = jnp.where(pos >= DILATION * w, logits[w], MASK_VALUE)
    m = functools.reduce(jnp.maximum, logits)
    e = [jnp.exp(l - m) for l in logits]
    inv = 1.0 / functools.reduce(jnp.add, e)
    p = [x * inv for x in e]
    outs = []
    for d in range(dh):
      o = None
      for w in range(WINDOW):
        pw = p[w] if w else _after(p[w], outs[d - way_p] if d >= way_p else None, z)
        t = pw * vt_v[z + d, window(w), :]
        o = t if o is None else o + t
      ot_v[d // 2, pl.ds(2 * r0 + d % 2, SUBLANES, stride=2), :] = o
      outs.append(o)
    if way_p < dh:
      anchor(outs[-way_p:])

  def to_feature_major(s, i, n=3):
    for j in range(i * pairs // n, (i + 1) * pairs // n):
      op_v[j] = ot_v[opaque_zero(s, 18) + j].astype(BF16)
      t = op_v.bitcast(I32)[j].T
      for b in range(NB):
        ob_v.bitcast(I32)[0, b, pl.ds(j, N_HEADS, stride=pairs), :] = (
            t[b * N_HEADS:(b + 1) * N_HEADS])

  def project_out(s, lo):
    y = _dot(_lane_blocks(wot_v, (), lo, QC)[:, :d_model],
             _lane_blocks(ob_v, (opaque_zero(s, 19),), 0, d_model))
    results.append(y[:SUBLANES, :LANES])
    rows = pl.ds(lo, QC)
    x1_v[s, rows, :] = xt_v[s, rows, :].astype(F32) + mod(2, lo, QC, NB) * y

  def norm2_stats(s, b, chains=2):
    if len(results) >= GATE and chains == 2:
      x1_v[n_tiles, pl.ds(0, SUBLANES), pl.ds(0, LANES)] = results[-GATE]
    cols = pl.ds(b * LANES, LANES)
    moments(lambda k: x1_v[s + opaque_zero(s, 40 + k), :, cols], 1, s, b, chains)

  def norm2(s, slot, b, r, size):
    def h2(side, row):
      blk = b + side * NB // 2
      return normalize(x1_v[s, pl.ds(row, size), pl.ds(blk * LANES, LANES)],
                       1, s, blk, row)

    outs = _strassen_rhs(h2(0, r), h2(1, r), h2(0, r + KH), h2(1, r + KH))
    for k in range(7):
      hb_v[slot, k, b, pl.ds(r, size), :] = outs[k]
    return outs

  def norm2_rest(s, slot):
    rows = pl.ds(2 * KH, d_model - 2 * KH)
    outs = [normalize(x1_v[s, rows, pl.ds(b * LANES, LANES)], 1, s, b,
                      2 * KH).astype(BF16) for b in range(NB)]
    for b in range(NB):
      hr_v[slot, b] = outs[b]
    return outs

  def transpose_weights(w_v, wt_v, a, b, ks=range(0, d_model, LANES)):
    for k in ks:
      size = min(LANES, d_model - k)
      t = w_v[pl.ds(k, size), pl.ds(a, b - a)].T
      if size < LANES:
        t = jnp.concatenate([t, jnp.zeros((b - a, LANES - size), BF16)], axis=1)
      wt_v[k // LANES, pl.ds(a, b - a), :] = t
      if ANCHOR_TW:
        anchor([t[-2 * SUBLANES:]])

  def transpose_leads():
    for j in range(NC):
      t = wg_v[j, pl.ds(2 * KH, d_model - 2 * KH), pl.ds(0, FS[0])].T
      lead_v[j] = jnp.concatenate([t, jnp.zeros_like(t)], axis=1)

  def transpose_wo(*ks):
    transpose_weights(wo_v, wot_v, 0, d_model, ks or range(0, d_model, LANES))

  def run(steps):
    for n, (fn, *args) in enumerate(steps):
      nxt = [f for f, *_ in steps[n + 1:] if f in (project_qkv, project_out)]
      target[0] = (None if not nxt else h1_v if nxt[0] is project_qkv else ob_v)
      fn(*args)
    target[0] = None
    results.clear()

  def stats_steps(fn, s):
    return [(fn, s, b) for b in range(NB)]

  def norm1_steps(s, n=1):
    return [(norm1, s, b, i, n) for b in range(NB) for i in range(n)]

  def token_major_steps(parts):
    return [(to_token_major, part, i) for part in parts for i in range(3)]

  def attention_steps(s, ways):
    return [(attend, s, g, *ways) for g in range(LANES // SUBLANES)]

  zero = lax.fori_loop(0, 2, lambda i, z: z + opaque_zero(i, 1), jnp.int32(0))
  edge_v[...] = jnp.zeros(edge_v.shape, edge_v.dtype)
  x1_v[0] = jnp.zeros(x1_v.shape[1:], F32)
  c_cp.wait()
  cv = c_v[...].astype(F32)
  sc_v[0] = jnp.broadcast_to(cv * jax.nn.sigmoid(cv), (LANES, d_model)).T
  x_cps[0].wait()
  for b in range(NB):
    norm1_stats(zero, b)
  for cp, a, b in zip(wmod_cps[:3], mod_cuts, mod_cuts[1:]):
    cp.wait()
    for j in range(a, b):
      modulation(zero, j, 2)
  for b in range(NB):
    norm1(zero, b)

  waits = dict(zip(DMA_CUTS, wqkv_cps))
  if ONLY_LOOP:
    transpose_wo()
    transpose_weights(wqkv_v, wqkvt_v, 0, 3 * d_model)
  for a, b in zip(Q0_CUTS, Q0_CUTS[1:]) if not ONLY_LOOP else []:
    final = b == 3 * d_model
    if a in waits:
      waits[a].wait()
    if final:
      for cp in (x_cps[1], wo_cp, wmod_cps[3]):
        cp.wait()
    if a in waits:
      transpose_weights(wqkv_v, wqkvt_v, a, DMA_CUTS[DMA_CUTS.index(a) + 1])
    steps = [(project_qkv, zero, lo) for lo in range(a, b, QC)]
    if final:
      n = len(steps)
      P0, P1, P2, P3, P4, P5 = PRO_ORDER or (0, 2, 2, 6, 1, 6)
      steps = _interleave(
          steps,
          ([(modulation_mxu, mod_cuts[3], mod_cuts[4])] if GA_MXU else [(modulation, zero, j) for j in range(mod_cuts[3], mod_cuts[4])], P0, P1),
          (stats_steps(norm1_stats, zero + 1), P2, P3),
          (token_major_steps([1]), 0, 3), ([(transpose_wo, k) for k in range(0, d_model, LANES)] if WO_AT == 'pro' else [(lambda: None,)], P4, P5),
          (token_major_steps([2]), n - 1, n),
          ([(hold_x,)] + norm1_steps(zero + 1, 4), n - 1, n))
    elif a < d_model < b:
      n = (d_model - a) // QC
      steps = _interleave(steps, (token_major_steps([0]), n, n + 3))
    run(steps)
  for cp in x_cps[2:]:
    cp.wait()

  n_q, n_w = 3 * d_model // QC, d_model // QC

  @pl.loop(0, 0 if ONLY_FFN else last)
  def _(s):
    s_next = jnp.minimum(s + 2, last)
    pieces = {
        "a": attention_steps(s, (WAY_S, WAY_P)),
        "u": [(to_feature_major, s, i) for i in range(3)],
        "m": stats_steps(norm2_stats, jnp.maximum(s - 1, 0)),
        "l": stats_steps(norm1_stats, s_next),
        "t": token_major_steps(range(3)),
        "w": [(transpose_wo, k) for k in range(0, d_model, LANES)],

        "L1": norm1_steps(s_next), "L2": norm1_steps(s_next, 2),
        "L4": norm1_steps(s_next, 4),
    }
    place = lambda order: [(pieces[k], lo, hi) for k, lo, hi in order]
    run(_interleave(
        [(project_qkv, s, lo) for lo in range(0, 3 * d_model, QC)],
        *place(X_ORDER)))

    if WO_AT == 'mid':
      pl.when(s == 0)(transpose_wo)

    @pl.when(opaque_zero(s, 50) == 0)
    def _():
      run(_interleave(
          [(project_out, s, lo) for lo in range(0, d_model, QC)],
          *place(Y_ORDER)))

  for cp in (wmod_cps[4], *ff_cps):
    cp.wait()
  s = zero + last
  if not ONLY_LOOP: run([(modulation_mxu, mod_cuts[4], mod_cuts[5])] + stats_steps(norm2_stats, s - 1) + attention_steps(s, TAIL_WAYS)
      + [(to_feature_major, s, i) for i in range(3)]
      + [(project_out, s, lo) for lo in range(0, d_model, QC)]
      + [(transpose_leads,)]
      + [(norm2_stats, s, b, TAIL_CHAINS) for b in range(NB)])

  def out_copy(i):
    cols = pl.ds(i * TILE if isinstance(i, int)
                 else pl.multiple_of(i * TILE, TILE), TILE)
    return pltpu.make_async_copy(out_v.at[i], out_hbm.at[:, cols], out_sem.at[i])

  def finish(i, r, size):
    c11, c12, c21, c22 = _strassen_out(
        *(acc_v[i % 2, k, pl.ds(r, size), :] for k in range(7)))
    outs = []
    for lo, y in ((r, (c11, c12)), (r + mh, (c21, c22))):
      rows = pl.ds(lo, size)
      outs.append((x1_v[i, rows, :] + mod(5, lo, size, NB)
                   * jnp.concatenate(y, axis=1)).astype(out_v.dtype))
      out_v[i, rows, :] = outs[-1]
    return outs

  for b in range(NB // 2):
    for r in range(0, KH, MR):
      norm2(0, 0, b, r, MR)
  norm2_rest(0, 0)

  @pl.loop(0, n_tiles * NC)
  def _(step):
    i, j = lax.div(step, NC), lax.rem(step, NC)
    slot = i % 2

    def hold(w_v, v):
      w_v[NC, pl.ds(0, 2 * SUBLANES), pl.ds(0, LANES)] = pltpu.bitcast(v, BF16)

    def products(w_v, blocks, dot, rhs, order, extra=None, side_work=()):
      out = {}
      side_work, started = list(side_work), []
      for k in order:
        if results:
          hold(w_v, functools.reduce(jnp.bitwise_or,
                                     _registers([results[-1], *started])))
          started = side_work.pop(0)(results[-1]) if side_work else []
        terms = [(sign, w_v[(j, *blocks[q])]) for sign, q in _LHS_TERMS[k]]
        if len(terms) == 1:
          lhs = terms[0][1]
        else:
          (_, x), (sign, y) = terms
          x, y = x.astype(F32), y.astype(F32)
          lhs = (x + y if sign > 0 else x - y).astype(BF16)
        if extra and k in extra:
          lhs = jnp.concatenate([lhs, w_v[(j, *extra[k])]], axis=0)
        out[k] = dot(lhs, rhs[k])
        results.append(out[k][:SUBLANES, :LANES])
      return out

    def project(w_v, lead=False, side_work=()):
      fh = fc // 2
      top, bottom = pl.ds(0, KH), pl.ds(KH, KH)
      rest = pl.ds(2 * KH, d_model - 2 * KH)
      first, second = pl.ds(0, fh), pl.ds(fh, fh)
      b = [_lane_blocks(hb_v, (slot, k), 0, KH) for k in range(7)]
      hr = _lane_blocks(hr_v, (slot,), 0, d_model - 2 * KH)
      if lead:
        r12 = _dot(_load_bf16(lead_v, (j,), 0, fh)[:, :d_model - 2 * KH],
                   hr[:, half:])
        r21 = _dot(_load_bf16(lead_v, (j,), fh, fh)[:, :d_model - 2 * KH],
                   hr[:, :half])
      else:
        r12 = _dot_tn(w_v[j, rest, first], hr[:, half:])
        r21 = _dot_tn(w_v[j, rest, second], hr[:, :half])
      results.append(r21[:SUBLANES, :LANES])
      b[6] = jnp.concatenate([b[6], hr[:, :half]], axis=0)
      b[5] = jnp.concatenate([b[5], hr[:, half:]], axis=0)
      m = products(w_v, ((top, first), (bottom, first), (top, second),
                         (bottom, second)), _dot_tn, b, ORDER_G,
                   {6: (rest, first), 5: (rest, second)}, side_work)
      c11, c12, c21, c22 = _strassen_out(*(m[k] for k in range(7)))
      return c11, c12 + r12, c21 + r21, c22

    def finish_share(n, gate):
      acc_v[2, 0, pl.ds(0, SUBLANES), pl.ds(0, LANES)] = gate
      r = pl.multiple_of(j * (mh // NC) + n * FR, 2 * SUBLANES)
      return finish(jnp.maximum(i - 1, 0), r, FR)

    def norm2_share(n, gate):
      x1_v[n_tiles, pl.ds(0, SUBLANES), pl.ds(0, LANES)] = gate
      nxt = jnp.minimum(i + 1, last)
      outs = []
      for m in n:
        if m is None:
          outs += norm2_rest(nxt, 1 - slot)
          continue
        r = pl.multiple_of(jnp.minimum(j * 96, KH - 96) + m // 2 * NR,
                           2 * SUBLANES)
        outs += norm2(nxt, 1 - slot, m % 2, r, NR)
      return outs

    idle = [lambda gate: []]
    g = project(wg_v, lead=True, side_work=idle * FSKIP + [
        functools.partial(finish_share, n) for n in range(mh // NC // FR)])
    u = project(wu_v)
    b = _strassen_rhs(*(gg * uu for gg, uu in zip(g, u)))
    fh = fc // 2
    top, bottom = pl.ds(0, mh), pl.ds(mh, mh)
    first, second = pl.ds(0, fh), pl.ds(fh, fh)
    m = products(wdt_v, ((top, first), (top, second), (bottom, first),
                         (bottom, second)), _dot, b, ORDER_D,
                 side_work=[functools.partial(norm2_share, n)
                            for n in NORM_PARTS])
    for k in ORDER_D:
      acc_v[slot, k] = jnp.where(j > 0, acc_v[slot, k], 0.0) + m[k]
    results.clear()

    @pl.when((j == NC - 1) & (i > 0))
    def _():
      out_copy(i - 1).start()

  finish(last, 0, mh)
  out_copy(last).start()
  for i in range(n_tiles):
    out_copy(i).wait()


@jax.jit
def pallas_adaLN_cond__sliding_local_dilated__glu_gated_bilinear__prompt_kernel(
    A_x, A_wqkv, A_wo, B_x, B_w_gate, B_w_up, B_w_down, c, w_mod):
  del B_x
  batch, seq, d_model = A_x.shape
  d_ff = B_w_gate.shape[1]
  dh = d_model // N_HEADS
  n_tiles = seq // TILE
  fc = d_ff // NC
  assert batch == 1 and seq % TILE == 0 and sum(FS) == fc
  hbm = pl.BlockSpec(memory_space=pltpu.HBM)
  operands = (A_x.reshape(seq, d_model).T, A_wqkv, A_wo, B_w_gate, B_w_up,
              B_w_down.T, c, w_mod)
  like = lambda a: pltpu.VMEM(a.shape, a.dtype)
  out_t = pl.pallas_call(
      _kernel,
      in_specs=[hbm] * len(operands),
      out_specs=hbm,
      out_shape=jax.ShapeDtypeStruct((d_model, seq), A_x.dtype),
      scratch_shapes=[
          pltpu.VMEM((n_tiles + 1, d_model, TILE), A_x.dtype),
          like(A_wqkv), like(A_wo),
          *[pltpu.VMEM((NC + 1, d_model, fc), BF16)] * 3,
          like(c), like(w_mod),
          pltpu.VMEM((2, d_model, LANES), F32),
          pltpu.VMEM((6 * d_model, LANES), F32),
          pltpu.VMEM((2, n_tiles, 2, NB, SUBLANES, LANES), F32),
          pltpu.VMEM((pl.cdiv(d_model, LANES), 3 * d_model, LANES), BF16),
          pltpu.VMEM((pl.cdiv(d_model, LANES), d_model, LANES), BF16),
          pltpu.VMEM((2, NB, d_model, LANES), BF16),
          pltpu.VMEM((2, NB, d_model, LANES), BF16),
          pltpu.VMEM((NB, 3 * d_model, LANES), BF16),
          pltpu.VMEM((2, dh // 2, HALO, LANES), I32),
          pltpu.VMEM((dh, LANES, LANES), F32),
          pltpu.VMEM((dh, HALO + LANES, LANES), F32),
          pltpu.VMEM((dh, HALO + LANES, LANES), F32),
          pltpu.VMEM((dh // 2, 2 * LANES, LANES), F32),
          pltpu.VMEM((dh // 2, 2 * LANES, LANES), BF16),
          pltpu.VMEM((n_tiles + 1, d_model, TILE), F32),
          pltpu.VMEM((2, 7, NB // 2, KH, LANES), BF16),
          pltpu.VMEM((2, NB, d_model - 2 * KH, LANES), BF16),
          pltpu.VMEM((NC, FS[0], LANES), BF16),
          pltpu.VMEM((3, 7, d_model // 2, TILE // 2), F32),
          pltpu.VMEM((n_tiles, d_model, TILE), A_x.dtype),
          pltpu.SemaphoreType.DMA((6 + len(DMA_CUTS) + n_tiles + 3 * NC,)),
          pltpu.SemaphoreType.DMA((n_tiles,)),
      ],
      compiler_params=pltpu.CompilerParams(vmem_limit_bytes=110 * 2**20,
                                           flags=FLAGS),
      name="adaln_window_attn_glu",
  )(*operands)
  return out_t.T.reshape(batch, seq, d_model)
```

```python
import functools

import jax
import jax.numpy as jnp
from jax import lax
import jax.experimental.pallas as pl
import jax.experimental.pallas.tpu as pltpu

N_HEADS = 32
WINDOW = 8
DILATION = 2
LN_EPS = 1e-5
MASK_VALUE = -1000000000.0

LANES = 128
SUBLANES = 8
NB = LANES // N_HEADS
TILE = NB * LANES
HALO = 16
KH = 256
N_CHUNKS = 3
ROWS = 64
SHARE = 32

F32 = jnp.float32
BF16 = jnp.bfloat16
I32 = jnp.int32

_LHS_TERMS = (((1, 0), (1, 3)), ((1, 2), (1, 3)), ((1, 0),), ((1, 3),),
              ((1, 0), (1, 1)), ((1, 2), (-1, 0)), ((1, 1), (-1, 3)))


def _strassen_rhs(b11, b12, b21, b22):
  return tuple(b.astype(BF16) for b in (
      b11 + b22, b11, b12 - b22, b21 - b11, b22, b11 + b12, b21 + b22))


def _strassen_out(m1, m2, m3, m4, m5, m6, m7):
  return m1 + m4 - m5 + m7, m3 + m5, m2 + m4, m1 - m2 + m3 + m6


def _dot(a, b):
  return jnp.dot(a, b, preferred_element_type=F32)


def _dot_tn(a, b):
  return lax.dot_general(a, b, (((0,), (0,)), ((), ())),
                         preferred_element_type=F32)


def _load_bf16(ref, lead, lo, size):
  words = ref.bitcast(I32)[(*lead, pl.ds(lo // 2, size // 2), slice(None))]
  return pltpu.bitcast(words, BF16)


def _lane_blocks(ref, lead, lo, size):
  return jnp.concatenate([_load_bf16(ref, (*lead, b), lo, size)
                          for b in range(ref.shape[len(lead)])], axis=1)


def _column_sum(x, chains):
  size = chains * SUBLANES
  acc = functools.reduce(
      jnp.add, [x[i:i + size] for i in range(0, x.shape[0], size)])
  return jnp.sum(acc, axis=0, keepdims=True)


def _after(x, earlier, zero):
  return pltpu.bitcast(
      pltpu.bitcast(x, I32) | (pltpu.bitcast(earlier, I32) & zero), F32)


def _token(vals):
  regs = []
  for v in vals:
    v = pltpu.bitcast(v, I32)
    regs += [v[i:i + SUBLANES, k:k + LANES]
             for i in range(0, v.shape[0], SUBLANES)
             for k in range(0, v.shape[1], LANES)]
  return functools.reduce(jnp.bitwise_or, regs)


def _interleave(matmuls, *placed):
  slots = [[m] for m in matmuls]
  for pieces, lo, hi in placed:
    for k, piece in enumerate(pieces):
      slots[lo + k * (hi - lo) // len(pieces)].append(piece)
  return [piece for slot in slots for piece in slot]


def _kernel(xt_hbm, wqkv_hbm, wo_hbm, wg_hbm, wu_hbm, wdt_hbm, c_hbm, wmod_hbm,
            out_hbm,
            xt_v, wqkv_v, wo_v, wg_v, wu_v, wdt_v, c_v, wmod_v,
            sc_v, mod_v, stat_v, wqkvt_v, wot_v, h1_v, qkv_v, edge_v,
            qt_v, kt_v, vt_v, ot_v, op_v, ob_v, x1_v, hb_v, hr_v, lead_v,
            acc_v, out_v, in_sem, out_sem):
  d_model, seq = xt_hbm.shape
  dh = d_model // N_HEADS
  pairs = dh // 2
  n_tiles = seq // TILE
  last = n_tiles - 1
  fc = wg_hbm.shape[1] // N_CHUNKS
  mh = d_model // 2
  half = TILE // 2
  n_rest = d_model - 2 * KH
  spare = (pl.ds(0, SUBLANES), pl.ds(0, LANES))
  spare_bf16 = (pl.ds(0, 2 * SUBLANES), pl.ds(0, LANES))

  sems = iter(range(in_sem.shape[0]))
  copy = lambda src, dst: pltpu.make_async_copy(src, dst, in_sem.at[next(sems)])

  def col_copies(src, dst, cuts):
    return [copy(src.at[:, pl.ds(a, b - a)], dst.at[:, pl.ds(a, b - a)])
            for a, b in zip(cuts, cuts[1:])]

  mod_cuts = (0, 3, 6, 9, 14, 6 * d_model // LANES)
  qkv_cuts = (0, 512, 1280, 3 * d_model)
  c_cp = copy(c_hbm, c_v)
  wmod_cps = col_copies(wmod_hbm, wmod_v, [j * LANES for j in mod_cuts])
  wqkv_cps = col_copies(wqkv_hbm, wqkv_v, (0, qkv_cuts[1], 3 * d_model))
  wo_cp = copy(wo_hbm, wo_v)
  x_cps = [copy(xt_hbm.at[:, pl.ds(i * TILE, TILE)], xt_v.at[i])
           for i in range(n_tiles)]
  ff_cps = [copy(w_hbm.at[:, pl.ds(j * fc, fc)], w_v.at[j])
            for j in range(N_CHUNKS)
            for w_hbm, w_v in ((wg_hbm, wg_v), (wu_hbm, wu_v), (wdt_hbm, wdt_v))]
  for cp in (c_cp, x_cps[0], *wmod_cps[:3], *wqkv_cps, x_cps[1], wo_cp,
             wmod_cps[3], *x_cps[2:], wmod_cps[4], *ff_cps):
    cp.start()

  def out_copy(i):
    start = i * TILE if isinstance(i, int) else pl.multiple_of(i * TILE, TILE)
    return pltpu.make_async_copy(
        out_v.at[i], out_hbm.at[:, pl.ds(start, TILE)], out_sem.at[i])

  def opaque_zero(s, k):
    return lax.shift_right_logical(s + k, 16)

  next_operand = [None]
  results = []
  newest = [None]
  normalized = []

  def pin(*vals):
    if next_operand[0] is not None:
      next_operand[0].bitcast(I32)[1, 0, pl.ds(0, SUBLANES), :] = _token(vals)

  def run(steps):
    for n, (fn, *args) in enumerate(steps):
      later = [f for f, *_ in steps[n + 1:] if f in (project_qkv, project_out)]
      next_operand[0] = (None if not later
                         else h1_v if later[0] is project_qkv else ob_v)
      fn(*args)
    next_operand[0] = None
    results.clear()
    normalized.clear()

  def silu_c(rows):
    cv = c_v[...].astype(F32)
    return jnp.broadcast_to(cv * jax.nn.sigmoid(cv), (rows, d_model))

  def store_modulation(j, row):
    part = (j * LANES + lax.broadcasted_iota(I32, (1, LANES), 1)) // d_model
    row = jnp.where((part == 1) | (part == 4), row + 1.0, row)
    mod_v[pl.ds(j * LANES, LANES), :] = jnp.broadcast_to(row, (LANES, LANES)).T

  def modulation(s, j, chains):
    w = wmod_v[:, pl.ds(j * LANES, LANES)].astype(F32)
    row = _column_sum(w * sc_v[opaque_zero(s, 60)], chains)
    pin(jnp.broadcast_to(row, (SUBLANES, LANES)))
    store_modulation(j, row)

  def modulation_mxu(lo, hi):
    rows = _dot(silu_c(2 * SUBLANES).astype(BF16),
                wmod_v[:, pl.ds(lo * LANES, (hi - lo) * LANES)])
    for j in range(lo, hi):
      store_modulation(j, rows[:1, (j - lo) * LANES:(j - lo + 1) * LANES])

  def mod(part, lo, size, n=1):
    col = mod_v[pl.ds(part * d_model + lo, size), :]
    return col if n == 1 else jnp.concatenate([col] * n, axis=1)

  def moments(load, which, s, b, chains):
    inv_d = 1.0 / d_model
    mean = _column_sum(load(0), chains) * inv_d
    xc = load(1) - mean
    var = _column_sum(xc * xc, chains) * inv_d
    for k, v in enumerate((mean, lax.rsqrt(var + LN_EPS))):
      stat_v[which, s, k, b] = v = jnp.broadcast_to(v, (SUBLANES, LANES))
    pin(v)

  def normalize(x, which, s, b, lo, serial=False):
    size = x.shape[0]
    mean, rstd = stat_v[which, s, 0, b], stat_v[which, s, 1, b]
    if serial and normalized:
      mean = _after(mean, normalized[-1], opaque_zero(s, 36))
    mean, rstd = (jnp.tile(v, (size // SUBLANES, 1)) for v in (mean, rstd))
    y = ((x - mean) * rstd * mod(3 * which + 1, lo, size)
         + mod(3 * which, lo, size))
    normalized.append(y[:SUBLANES])
    return y

  def hold_x(v):
    xt_v[(n_tiles, *spare_bf16)] = pltpu.bitcast(v, BF16)

  def norm1_stats(s, b):
    if len(results) >= 2:
      hold_x(results[-2])
    cols = pl.ds(b * LANES, LANES)
    moments(lambda k: xt_v[s + opaque_zero(s, 32 + k), :, cols].astype(F32),
            0, s, b, 2)

  def norm1(s, b, i, n):
    size = d_model // n
    rows = pl.ds(i * size, size)
    x = xt_v[s + opaque_zero(s, 34), rows, pl.ds(b * LANES, LANES)]
    h1_v[0, b, rows, :] = normalize(x.astype(F32), 0, s, b, i * size).astype(BF16)

  def norm2_stats(s, b, chains=2):
    if len(results) >= 2 and next_operand[0] is not None:
      x1_v[(n_tiles, *spare)] = results[-2]
    cols = pl.ds(b * LANES, LANES)
    moments(lambda k: x1_v[s + opaque_zero(s, 40 + k), :, cols], 1, s, b, chains)

  def norm2(s, tile, slot, b, r, serial=False):
    def h(side, row):
      blk = b + side * NB // 2
      x = x1_v[tile, pl.ds(row, SHARE), pl.ds(blk * LANES, LANES)]
      return normalize(x, 1, s, blk, row, serial)

    outs = _strassen_rhs(h(0, r), h(1, r), h(0, r + KH), h(1, r + KH))
    for k in range(7):
      hb_v[slot, k, b, pl.ds(r, SHARE), :] = outs[k]
    return list(outs)

  def norm2_rest(s, tile, slot):
    rows = pl.ds(2 * KH, n_rest)
    outs = [normalize(x1_v[tile, rows, pl.ds(b * LANES, LANES)], 1, s, b,
                      2 * KH).astype(BF16) for b in range(NB)]
    for b in range(NB):
      hr_v[slot, b] = outs[b]
    return outs

  def transpose_weights(w_v, wt_v, a, b, ks):
    for k in ks:
      size = min(LANES, d_model - k)
      t = w_v[pl.ds(k, size), pl.ds(a, b - a)].T
      if size < LANES:
        t = jnp.concatenate([t, jnp.zeros((b - a, LANES - size), BF16)], axis=1)
      wt_v[k // LANES, pl.ds(a, b - a), :] = t

  def project_qkv(s, lo):
    qkv = _dot(_lane_blocks(wqkvt_v, (), lo, ROWS)[:, :d_model],
               _lane_blocks(h1_v, (opaque_zero(s, 17),), 0, d_model))
    results.append(qkv[:SUBLANES, :LANES])
    newest[0] = qkv[-SUBLANES:, -LANES:]
    for b in range(NB):
      qkv_v[b, pl.ds(lo, ROWS), :] = (
          qkv[:, b * LANES:(b + 1) * LANES].astype(BF16))

  def to_token_major(part, js):
    buf = (qt_v, kt_v, vt_v)[part]
    for j in js:
      rows = pl.ds(part * mh + j, N_HEADS, stride=pairs)
      t = jnp.concatenate(
          [qkv_v.bitcast(I32)[b, rows, :] for b in range(NB)], axis=0).T
      if part:
        lane = lax.broadcasted_iota(I32, (HALO, LANES), 1)
        before = jnp.where(lane < LANES - N_HEADS, t[-HALO:], edge_v[part - 1, j])
        edge_v[part - 1, j] = t[-HALO:]
        t = jnp.concatenate([pltpu.roll(before, N_HEADS, 1), t], axis=0)
      buf[2 * j] = pltpu.bitcast(t << 16, F32)
      buf[2 * j + 1] = pltpu.bitcast(t & -65536, F32)

  def attend(s, g, ways_qk, ways_pv):
    r0 = g * SUBLANES
    z = opaque_zero(s, g)
    window = lambda w: pl.ds(HALO + r0 - DILATION * w, SUBLANES)
    q = [qt_v[z + d, pl.ds(r0, SUBLANES), :] for d in range(dh)]
    logits = []
    for w in range(WINDOW):
      q0 = q[0] if w < ways_qk else _after(q[0], logits[w - ways_qk], z)
      logits.append(functools.reduce(jnp.add, [
          qd * kt_v[z + d, window(w), :] for d, qd in enumerate([q0, *q[1:]])]))
    for w in range(WINDOW):
      logits[w] = logits[w] * dh ** -0.5
      if r0 < DILATION * w:
        shape = (SUBLANES, LANES)
        pos = (s * TILE + r0 + lax.broadcasted_iota(I32, shape, 0)
               + lax.broadcasted_iota(I32, shape, 1) // N_HEADS * LANES)
        logits[w] = jnp.where(pos >= DILATION * w, logits[w], MASK_VALUE)
    m = functools.reduce(jnp.maximum, logits)
    e = [jnp.exp(l - m) for l in logits]
    inv = 1.0 / functools.reduce(jnp.add, e)
    p = [x * inv for x in e]
    outs = []
    for d in range(dh):
      p0 = p[0] if d < ways_pv else _after(p[0], outs[d - ways_pv], z)
      outs.append(functools.reduce(jnp.add, [
          pw * vt_v[z + d, window(w), :] for w, pw in enumerate([p0, *p[1:]])]))
      ot_v[d // 2, pl.ds(2 * r0 + d % 2, SUBLANES, stride=2), :] = outs[-1]
    pin(*outs[-ways_pv:])

  def to_feature_major(s):
    for j in range(pairs):
      op_v[j] = ot_v[opaque_zero(s, 18) + j].astype(BF16)
      t = op_v.bitcast(I32)[j].T
      for b in range(NB):
        ob_v.bitcast(I32)[0, b, pl.ds(j, N_HEADS, stride=pairs), :] = (
            t[b * N_HEADS:(b + 1) * N_HEADS])

  def project_out(s, tile, lo):
    y = _dot(_lane_blocks(wot_v, (), lo, ROWS)[:, :d_model],
             _lane_blocks(ob_v, (opaque_zero(s, 19),), 0, d_model))
    results.append(y[:SUBLANES, :LANES])
    rows = pl.ds(lo, ROWS)
    x1_v[tile, rows, :] = (xt_v[tile, rows, :].astype(F32)
                           + mod(2, lo, ROWS, NB) * y)

  per_block = lambda fn, s: [(fn, s, b) for b in range(NB)]
  norm1_steps = lambda s: [(norm1, s, b, i, 4)
                           for b in range(NB) for i in range(4)]
  qkv_steps = lambda s, a, b: [(project_qkv, s, lo) for lo in range(a, b, ROWS)]
  out_steps = lambda s, tile: [(project_out, s, tile, lo)
                               for lo in range(0, d_model, ROWS)]
  token_steps = lambda part: [(to_token_major, part, range(j, j + 3))
                              for j in range(0, pairs, 3)]
  attend_steps = lambda s, *ways: [(attend, s, g, *ways)
                                   for g in range(LANES // SUBLANES)]
  all_k = range(0, d_model, LANES)

  zero = lax.fori_loop(0, 2, lambda i, z: z + opaque_zero(i, 1), jnp.int32(0))
  edge_v[...] = jnp.zeros(edge_v.shape, edge_v.dtype)
  x1_v[0] = jnp.zeros(x1_v.shape[1:], F32)
  c_cp.wait()
  sc_v[0] = silu_c(LANES).T
  x_cps[0].wait()
  run(per_block(norm1_stats, zero))
  for cp, a, b in zip(wmod_cps[:3], mod_cuts, mod_cuts[1:]):
    cp.wait()
    for j in range(a, b):
      modulation(zero, j, 2)
  run([(norm1, zero, b, 0, 1) for b in range(NB)])

  wqkv_cps[0].wait()
  transpose_weights(wqkv_v, wqkvt_v, 0, qkv_cuts[1], all_k)
  run(qkv_steps(zero, 0, qkv_cuts[1]))
  wqkv_cps[1].wait()
  transpose_weights(wqkv_v, wqkvt_v, qkv_cuts[1], 3 * d_model, all_k)
  run(_interleave(qkv_steps(zero, *qkv_cuts[1:3]), (token_steps(0), 1, 4)))
  for cp in (x_cps[1], wo_cp, wmod_cps[3]):
    cp.wait()
  steps = qkv_steps(zero, *qkv_cuts[2:])
  n = len(steps)
  run(_interleave(
      steps,
      ([(modulation, zero, j, 1) for j in range(*mod_cuts[3:5])], 0, 2),
      (per_block(norm1_stats, zero + 1), 2, n - 1),
      (token_steps(1), 0, 3),
      (token_steps(2) + [(lambda: hold_x(newest[0]),)] + norm1_steps(zero + 1),
       n - 1, n)))
  for cp in x_cps[2:]:
    cp.wait()

  @pl.loop(0, last)
  def _(s):
    ahead = jnp.minimum(s + 2, last)
    run(_interleave(
        qkv_steps(s, 0, 3 * d_model),
        (attend_steps(s, 2, 3), 1, 17),
        ([(to_feature_major, s)], 17, 18),
        (per_block(norm1_stats, ahead), 18, 22),
        (per_block(norm2_stats, jnp.maximum(s - 1, 0)), 22, 26),
        ([(transpose_weights, wo_v, wot_v, 0, d_model, all_k)], 17, 18)))

    @pl.when(opaque_zero(s, 50) == 0)
    def _():
      steps = out_steps(s, s)
      run(_interleave(
          steps,
          (token_steps(0) + token_steps(1) + token_steps(2), 0, len(steps)),
          (norm1_steps(ahead), 0, len(steps) - 1)))

  def first_norm2(b, r):
    if len(results) >= 2:
      stat_v[1, n_tiles, 0, 0] = results[-2]
    if r is None:
      pin(*norm2_rest(zero, 0, 0))
    else:
      pin(*norm2(zero, 0, 0, b, r, True), *norm2(zero, 0, 0, b, r + SHARE, True))

  def transpose_leads():
    for j in range(N_CHUNKS):
      t = wg_v[j, pl.ds(2 * KH, n_rest), :].T
      lead_v[j] = jnp.concatenate(
          [t, jnp.zeros((fc, LANES - n_rest), BF16)], axis=1)

  for cp in (wmod_cps[4], *ff_cps):
    cp.wait()
  s = zero + last
  steps = out_steps(s, last)
  run([(modulation_mxu, *mod_cuts[4:])] + per_block(norm2_stats, s - 1)
      + attend_steps(s, WINDOW, pairs) + [(to_feature_major, s)]
      + _interleave(steps, (
          [(first_norm2, 0, None)] + [(first_norm2, b, r)
                                      for b in range(NB // 2)
                                      for r in range(0, KH, 2 * SHARE)],
          0, len(steps) - 1))
      + [(transpose_leads,)] + [(norm2_stats, s, b, 3) for b in range(NB)])

  def finish(i, r, size):
    c11, c12, c21, c22 = _strassen_out(
        *(acc_v[i & 1, k, pl.ds(r, size), :] for k in range(7)))
    outs = []
    for lo, y in ((r, (c11, c12)), (r + mh, (c21, c22))):
      rows = pl.ds(lo, size)
      outs.append((x1_v[i, rows, :] + mod(5, lo, size, NB)
                   * jnp.concatenate(y, axis=1)).astype(out_v.dtype))
      out_v[i, rows, :] = outs[-1]
    return outs

  @pl.loop(0, n_tiles * N_CHUNKS)
  def _(step):
    i, j = lax.div(step, N_CHUNKS), lax.rem(step, N_CHUNKS)
    slot = i & 1
    first, second = pl.ds(0, fc // 2), pl.ds(fc // 2, fc // 2)

    def products(w_v, blocks, dot, rhs, order, extra, side_work):
      out = {}
      side_work, started = list(side_work), []
      for k in order:
        if results:
          w_v[(N_CHUNKS, *spare_bf16)] = pltpu.bitcast(
              _token([results[-1], *started]), BF16)
          started = side_work.pop(0)(results[-1]) if side_work else []
        terms = [w_v[(j, *blocks[q])] for _, q in _LHS_TERMS[k]]
        lhs = terms[0]
        if len(terms) == 2:
          x, y = (t.astype(F32) for t in terms)
          lhs = (x + y if _LHS_TERMS[k][1][0] > 0 else x - y).astype(BF16)
        if k in extra:
          lhs = jnp.concatenate([lhs, w_v[(j, *extra[k])]], axis=0)
        out[k] = dot(lhs, rhs[k])
        results.append(out[k][:SUBLANES, :LANES])
      return out

    def project(w_v, lead, side_work):
      top, bottom, rest = pl.ds(0, KH), pl.ds(KH, KH), pl.ds(2 * KH, n_rest)
      rhs = [_lane_blocks(hb_v, (slot, k), 0, KH) for k in range(7)]
      hr = _lane_blocks(hr_v, (slot,), 0, n_rest)
      if lead:
        r12, r21 = (
            _dot(_load_bf16(lead_v, (j,), lo, fc // 2)[:, :n_rest], h)
            for lo, h in ((0, hr[:, half:]), (fc // 2, hr[:, :half])))
      else:
        r12 = _dot_tn(w_v[j, rest, first], hr[:, half:])
        r21 = _dot_tn(w_v[j, rest, second], hr[:, :half])
      results.append(r21[:SUBLANES, :LANES])
      rhs[5] = jnp.concatenate([rhs[5], hr[:, half:]], axis=0)
      rhs[6] = jnp.concatenate([rhs[6], hr[:, :half]], axis=0)
      m = products(
          w_v, ((top, first), (bottom, first), (top, second), (bottom, second)),
          _dot_tn, rhs, (2, 3, 1, 4, 0, 6, 5),
          {5: (rest, second), 6: (rest, first)}, side_work)
      c11, c12, c21, c22 = _strassen_out(*(m[k] for k in range(7)))
      return c11, c12 + r12, c21 + r21, c22

    def finish_share(n, after):
      acc_v[(2, 0, *spare)] = after
      r = pl.multiple_of(j * (mh // N_CHUNKS) + n * SHARE, 2 * SUBLANES)
      return finish(jnp.maximum(i - 1, 0), r, SHARE)

    def norm2_share(parts, after):
      x1_v[(n_tiles, *spare)] = after
      nxt = jnp.minimum(i + 1, last)
      outs = []
      for n in parts:
        if n is None:
          outs += norm2_rest(nxt, nxt, 1 - slot)
        else:
          r = jnp.minimum(j * 3 * SHARE, KH - 3 * SHARE) + n // 2 * SHARE
          outs += norm2(nxt, nxt, 1 - slot, n % 2,
                        pl.multiple_of(r, 2 * SUBLANES))
      return outs

    idle = lambda after: []
    g = project(wg_v, True, [idle] + [
        functools.partial(finish_share, n)
        for n in range(mh // N_CHUNKS // SHARE)])
    u = project(wu_v, False, [])
    top, bottom = pl.ds(0, mh), pl.ds(mh, mh)
    order = (2, 3, 0, 4, 6, 1, 5)
    m = products(
        wdt_v, ((top, first), (top, second), (bottom, first), (bottom, second)),
        _dot, _strassen_rhs(*(a * b for a, b in zip(g, u))), order, {},
        [functools.partial(norm2_share, parts)
         for parts in ((None, 0), (1,), (2,), (3,), (4,), (5,))])
    for k in order:
      acc_v[slot, k] = jnp.where(j > 0, acc_v[slot, k], 0.0) + m[k]
    results.clear()
    normalized.clear()

    @pl.when((j == N_CHUNKS - 1) & (i > 0))
    def _():
      out_copy(i - 1).start()

  finish(last, 0, mh)
  out_copy(last).start()
  for i in range(n_tiles):
    out_copy(i).wait()


@jax.jit
def pallas_adaLN_cond__sliding_local_dilated__glu_gated_bilinear__prompt_kernel(
    A_x: jax.Array,
    A_wqkv: jax.Array,
    A_wo: jax.Array,
    B_x: jax.Array,
    B_w_gate: jax.Array,
    B_w_up: jax.Array,
    B_w_down: jax.Array,
    c: jax.Array,
    w_mod: jax.Array,
):
  del B_x
  batch, seq, d_model = A_x.shape
  d_ff = B_w_gate.shape[1]
  assert (batch, d_model, d_ff) == (1, 576, 4608) and seq % TILE == 0
  dh = d_model // N_HEADS
  n_tiles = seq // TILE
  fc = d_ff // N_CHUNKS
  k_blocks = pl.cdiv(d_model, LANES)
  operands = (A_x.reshape(seq, d_model).T, A_wqkv, A_wo, B_w_gate, B_w_up,
              B_w_down.T, c, w_mod)
  hbm = pl.BlockSpec(memory_space=pltpu.HBM)
  vmem = pltpu.VMEM
  out_t = pl.pallas_call(
      _kernel,
      in_specs=[hbm] * len(operands),
      out_specs=hbm,
      out_shape=jax.ShapeDtypeStruct((d_model, seq), A_x.dtype),
      scratch_shapes=[
          vmem((n_tiles + 1, d_model, TILE), BF16),
          vmem(A_wqkv.shape, BF16),
          vmem(A_wo.shape, BF16),
          *[vmem((N_CHUNKS + 1, d_model, fc), BF16)] * 3,
          vmem(c.shape, BF16),
          vmem(w_mod.shape, BF16),
          vmem((1, d_model, LANES), F32),
          vmem((6 * d_model, LANES), F32),
          vmem((2, n_tiles + 1, 2, NB, SUBLANES, LANES), F32),
          vmem((k_blocks, 3 * d_model, LANES), BF16),
          vmem((k_blocks, d_model, LANES), BF16),
          vmem((2, NB, d_model, LANES), BF16),
          vmem((NB, 3 * d_model, LANES), BF16),
          vmem((2, dh // 2, HALO, LANES), I32),
          vmem((dh, LANES, LANES), F32),
          vmem((dh, HALO + LANES, LANES), F32),
          vmem((dh, HALO + LANES, LANES), F32),
          vmem((dh // 2, 2 * LANES, LANES), F32),
          vmem((dh // 2, 2 * LANES, LANES), BF16),
          vmem((2, NB, d_model, LANES), BF16),
          vmem((n_tiles + 1, d_model, TILE), F32),
          vmem((2, 7, NB // 2, KH, LANES), BF16),
          vmem((2, NB, d_model - 2 * KH, LANES), BF16),
          vmem((N_CHUNKS, fc, LANES), BF16),
          vmem((3, 7, d_model // 2, TILE // 2), F32),
          vmem((n_tiles, d_model, TILE), A_x.dtype),
          pltpu.SemaphoreType.DMA((9 + n_tiles + 3 * N_CHUNKS,)),
          pltpu.SemaphoreType.DMA((n_tiles,)),
      ],
      compiler_params=pltpu.CompilerParams(vmem_limit_bytes=100 * 2**20),
      name="adaln_window_attn_glu",
  )(*operands)
  return out_t.T.reshape(batch, seq, d_model)
```

```python
import functools

import jax
import jax.numpy as jnp
from jax import lax
import jax.experimental.pallas as pl
import jax.experimental.pallas.tpu as pltpu

N_HEADS = 32
WINDOW = 8
DILATION = 2
LN_EPS = 1e-5
MASK_VALUE = -1000000000.0

LANES = 128
SUBLANES = 8
NB = LANES // N_HEADS
TILE = NB * LANES
HALO = 16
KH = 256
N_CHUNKS = 3
ROWS = 64
SHARE = 32

F32 = jnp.float32
BF16 = jnp.bfloat16
I32 = jnp.int32

_LHS_TERMS = (((1, 0), (1, 3)), ((1, 2), (1, 3)), ((1, 0),), ((1, 3),),
              ((1, 0), (1, 1)), ((1, 2), (-1, 0)), ((1, 1), (-1, 3)))


def _strassen_rhs(b11, b12, b21, b22):
  return tuple(b.astype(BF16) for b in (
      b11 + b22, b11, b12 - b22, b21 - b11, b22, b11 + b12, b21 + b22))


def _strassen_out(m1, m2, m3, m4, m5, m6, m7):
  return m1 + m4 - m5 + m7, m3 + m5, m2 + m4, m1 - m2 + m3 + m6


def _dot(a, b):
  return jnp.dot(a, b, preferred_element_type=F32)


def _dot_tn(a, b):
  return lax.dot_general(a, b, (((0,), (0,)), ((), ())),
                         preferred_element_type=F32)


def _load_bf16(ref, lead, lo, size):
  words = ref.bitcast(I32)[(*lead, pl.ds(lo // 2, size // 2), slice(None))]
  return pltpu.bitcast(words, BF16)


def _lane_blocks(ref, lead, lo, size):
  return jnp.concatenate([_load_bf16(ref, (*lead, b), lo, size)
                          for b in range(ref.shape[len(lead)])], axis=1)


def _column_sum(x, chains):
  size = chains * SUBLANES
  acc = functools.reduce(
      jnp.add, [x[i:i + size] for i in range(0, x.shape[0], size)])
  return jnp.sum(acc, axis=0, keepdims=True)


def _after(x, earlier, zero):
  return pltpu.bitcast(
      pltpu.bitcast(x, I32) | (pltpu.bitcast(earlier, I32) & zero), F32)


def _token(vals):
  regs = []
  for v in vals:
    v = pltpu.bitcast(v, I32)
    regs += [v[i:i + SUBLANES, k:k + LANES]
             for i in range(0, v.shape[0], SUBLANES)
             for k in range(0, v.shape[1], LANES)]
  return functools.reduce(jnp.bitwise_or, regs)


def _interleave(matmuls, *placed):
  slots = [[m] for m in matmuls]
  for pieces, lo, hi in placed:
    for k, piece in enumerate(pieces):
      slots[lo + k * (hi - lo) // len(pieces)].append(piece)
  return [piece for slot in slots for piece in slot]


def _kernel(xt_hbm, wqkv_hbm, wo_hbm, wg_hbm, wu_hbm, wdt_hbm, c_hbm, wmod_hbm,
            out_hbm,
            xt_v, wqkv_v, wo_v, wg_v, wu_v, wdt_v, c_v, wmod_v,
            sc_v, mod_v, stat_v, wqkvt_v, wot_v, h1_v, qkv_v, edge_v,
            qt_v, kt_v, vt_v, ot_v, op_v, ob_v, x1_v, hb_v, hr_v, lead_v,
            acc_v, out_v, in_sem, out_sem):
  d_model, seq = xt_hbm.shape
  dh = d_model // N_HEADS
  pairs = dh // 2
  n_tiles = seq // TILE
  last = n_tiles - 1
  fc = wg_hbm.shape[1] // N_CHUNKS
  mh = d_model // 2
  half = TILE // 2
  n_rest = d_model - 2 * KH
  spare = (pl.ds(0, SUBLANES), pl.ds(0, LANES))
  spare_bf16 = (pl.ds(0, 2 * SUBLANES), pl.ds(0, LANES))

  sems = iter(range(in_sem.shape[0]))
  copy = lambda src, dst: pltpu.make_async_copy(src, dst, in_sem.at[next(sems)])

  def col_copies(src, dst, cuts):
    return [copy(src.at[:, pl.ds(a, b - a)], dst.at[:, pl.ds(a, b - a)])
            for a, b in zip(cuts, cuts[1:])]

  mod_cuts = (0, 3, 6, 9, 14, 6 * d_model // LANES)
  qkv_cuts = (0, 512, 1280, 3 * d_model)
  c_cp = copy(c_hbm, c_v)
  wmod_cps = col_copies(wmod_hbm, wmod_v, [j * LANES for j in mod_cuts])
  wqkv_cps = col_copies(wqkv_hbm, wqkv_v, (0, qkv_cuts[1], 3 * d_model))
  wo_cp = copy(wo_hbm, wo_v)
  x_cps = [copy(xt_hbm.at[:, pl.ds(i * TILE, TILE)], xt_v.at[i])
           for i in range(n_tiles)]
  ff_cps = [copy(w_hbm.at[:, pl.ds(j * fc, fc)], w_v.at[j])
            for j in range(N_CHUNKS)
            for w_hbm, w_v in ((wg_hbm, wg_v), (wu_hbm, wu_v), (wdt_hbm, wdt_v))]
  for cp in (c_cp, x_cps[0], *wmod_cps[:3], *wqkv_cps, x_cps[1], wo_cp,
             wmod_cps[3], *x_cps[2:], wmod_cps[4], *ff_cps):
    cp.start()

  def out_copy(i):
    start = i * TILE if isinstance(i, int) else pl.multiple_of(i * TILE, TILE)
    return pltpu.make_async_copy(
        out_v.at[i], out_hbm.at[:, pl.ds(start, TILE)], out_sem.at[i])

  def opaque_zero(s, k):
    return lax.shift_right_logical(s + k, 16)

  next_operand = [None]
  results = []
  newest = [None]
  normalized = []

  def pin(*vals):
    if next_operand[0] is not None:
      next_operand[0].bitcast(I32)[1, 0, pl.ds(0, SUBLANES), :] = _token(vals)

  def run(steps):
    for n, (fn, *args) in enumerate(steps):
      later = [f for f, *_ in steps[n + 1:] if f in (project_qkv, project_out)]
      next_operand[0] = (None if not later
                         else h1_v if later[0] is project_qkv else ob_v)
      fn(*args)
    next_operand[0] = None
    results.clear()
    normalized.clear()

  def silu_c(rows):
    cv = c_v[...].astype(F32)
    return jnp.broadcast_to(cv * jax.nn.sigmoid(cv), (rows, d_model))

  def store_modulation(j, row):
    part = (j * LANES + lax.broadcasted_iota(I32, (1, LANES), 1)) // d_model
    row = jnp.where((part == 1) | (part == 4), row + 1.0, row)
    mod_v[pl.ds(j * LANES, LANES), :] = jnp.broadcast_to(row, (LANES, LANES)).T

  def modulation(s, j, chains):
    w = wmod_v[:, pl.ds(j * LANES, LANES)].astype(F32)
    row = _column_sum(w * sc_v[opaque_zero(s, 60)], chains)
    pin(jnp.broadcast_to(row, (SUBLANES, LANES)))
    store_modulation(j, row)

  def modulation_mxu(lo, hi):
    rows = _dot(silu_c(2 * SUBLANES).astype(BF16),
                wmod_v[:, pl.ds(lo * LANES, (hi - lo) * LANES)])
    for j in range(lo, hi):
      store_modulation(j, rows[:1, (j - lo) * LANES:(j - lo + 1) * LANES])

  def mod(part, lo, size, n=1):
    col = mod_v[pl.ds(part * d_model + lo, size), :]
    return col if n == 1 else jnp.concatenate([col] * n, axis=1)

  def moments(load, which, s, b, chains):
    inv_d = 1.0 / d_model
    mean = _column_sum(load(0), chains) * inv_d
    xc = load(1) - mean
    var = _column_sum(xc * xc, chains) * inv_d
    for k, v in enumerate((mean, lax.rsqrt(var + LN_EPS))):
      stat_v[which, s, k, b] = v = jnp.broadcast_to(v, (SUBLANES, LANES))
    pin(v)

  def normalize(x, which, s, b, lo, serial=False):
    size = x.shape[0]
    mean, rstd = stat_v[which, s, 0, b], stat_v[which, s, 1, b]
    if serial and normalized:
      mean = _after(mean, normalized[-1], opaque_zero(s, 36))
    mean, rstd = (jnp.tile(v, (size // SUBLANES, 1)) for v in (mean, rstd))
    y = ((x - mean) * rstd * mod(3 * which + 1, lo, size)
         + mod(3 * which, lo, size))
    normalized.append(y[:SUBLANES])
    return y

  def hold_x(v):
    xt_v[(n_tiles, *spare_bf16)] = pltpu.bitcast(v, BF16)

  def norm1_stats(s, b):
    if len(results) >= 2:
      hold_x(results[-2])
    cols = pl.ds(b * LANES, LANES)
    moments(lambda k: xt_v[s + opaque_zero(s, 32 + k), :, cols].astype(F32),
            0, s, b, 2)

  def norm1(s, b, i, n):
    size = d_model // n
    rows = pl.ds(i * size, size)
    x = xt_v[s + opaque_zero(s, 34), rows, pl.ds(b * LANES, LANES)]
    h1_v[0, b, rows, :] = normalize(x.astype(F32), 0, s, b, i * size).astype(BF16)

  def norm2_stats(s, b, chains=2):
    if len(results) >= 2 and next_operand[0] is not None:
      x1_v[(n_tiles, *spare)] = results[-2]
    cols = pl.ds(b * LANES, LANES)
    moments(lambda k: x1_v[s + opaque_zero(s, 40 + k), :, cols], 1, s, b, chains)

  def norm2(s, tile, slot, b, r, serial=False):
    def h(side, row):
      blk = b + side * NB // 2
      x = x1_v[tile, pl.ds(row, SHARE), pl.ds(blk * LANES, LANES)]
      return normalize(x, 1, s, blk, row, serial)

    outs = _strassen_rhs(h(0, r), h(1, r), h(0, r + KH), h(1, r + KH))
    for k in range(7):
      hb_v[slot, k, b, pl.ds(r, SHARE), :] = outs[k]
    return list(outs)

  def norm2_rest(s, tile, slot):
    rows = pl.ds(2 * KH, n_rest)
    outs = [normalize(x1_v[tile, rows, pl.ds(b * LANES, LANES)], 1, s, b,
                      2 * KH).astype(BF16) for b in range(NB)]
    for b in range(NB):
      hr_v[slot, b] = outs[b]
    return outs

  def transpose_weights(w_v, wt_v, a, b):
    for k in range(0, d_model, LANES):
      size = min(LANES, d_model - k)
      t = w_v[pl.ds(k, size), pl.ds(a, b - a)].T
      if size < LANES:
        t = jnp.concatenate([t, jnp.zeros((b - a, LANES - size), BF16)], axis=1)
      wt_v[k // LANES, pl.ds(a, b - a), :] = t

  def project_qkv(s, lo):
    qkv = _dot(_lane_blocks(wqkvt_v, (), lo, ROWS)[:, :d_model],
               _lane_blocks(h1_v, (opaque_zero(s, 17),), 0, d_model))
    results.append(qkv[:SUBLANES, :LANES])
    newest[0] = qkv[-SUBLANES:, -LANES:]
    for b in range(NB):
      qkv_v[b, pl.ds(lo, ROWS), :] = (
          qkv[:, b * LANES:(b + 1) * LANES].astype(BF16))

  def to_token_major(part, js):
    buf = (qt_v, kt_v, vt_v)[part]
    for j in js:
      rows = pl.ds(part * mh + j, N_HEADS, stride=pairs)
      t = jnp.concatenate(
          [qkv_v.bitcast(I32)[b, rows, :] for b in range(NB)], axis=0).T
      if part:
        lane = lax.broadcasted_iota(I32, (HALO, LANES), 1)
        before = jnp.where(lane < LANES - N_HEADS, t[-HALO:], edge_v[part - 1, j])
        edge_v[part - 1, j] = t[-HALO:]
        t = jnp.concatenate([pltpu.roll(before, N_HEADS, 1), t], axis=0)
      buf[2 * j] = pltpu.bitcast(t << 16, F32)
      buf[2 * j + 1] = pltpu.bitcast(t & -65536, F32)

  def attend(s, g, ways_qk, ways_pv):
    r0 = g * SUBLANES
    z = opaque_zero(s, g)
    window = lambda w: pl.ds(HALO + r0 - DILATION * w, SUBLANES)
    q = [qt_v[z + d, pl.ds(r0, SUBLANES), :] for d in range(dh)]
    logits = []
    for w in range(WINDOW):
      q0 = q[0] if w < ways_qk else _after(q[0], logits[w - ways_qk], z)
      logits.append(functools.reduce(jnp.add, [
          qd * kt_v[z + d, window(w), :] for d, qd in enumerate([q0, *q[1:]])]))
    for w in range(WINDOW):
      logits[w] = logits[w] * dh ** -0.5
      if r0 < DILATION * w:
        shape = (SUBLANES, LANES)
        pos = (s * TILE + r0 + lax.broadcasted_iota(I32, shape, 0)
               + lax.broadcasted_iota(I32, shape, 1) // N_HEADS * LANES)
        logits[w] = jnp.where(pos >= DILATION * w, logits[w], MASK_VALUE)
    m = functools.reduce(jnp.maximum, logits)
    e = [jnp.exp(l - m) for l in logits]
    inv = 1.0 / functools.reduce(jnp.add, e)
    p = [x * inv for x in e]
    outs = []
    for d in range(dh):
      p0 = p[0] if d < ways_pv else _after(p[0], outs[d - ways_pv], z)
      outs.append(functools.reduce(jnp.add, [
          pw * vt_v[z + d, window(w), :] for w, pw in enumerate([p0, *p[1:]])]))
      ot_v[d // 2, pl.ds(2 * r0 + d % 2, SUBLANES, stride=2), :] = outs[-1]
    pin(*outs[-ways_pv:])

  def to_feature_major(s):
    for j in range(pairs):
      op_v[j] = ot_v[opaque_zero(s, 18) + j].astype(BF16)
      t = op_v.bitcast(I32)[j].T
      for b in range(NB):
        ob_v.bitcast(I32)[0, b, pl.ds(j, N_HEADS, stride=pairs), :] = (
            t[b * N_HEADS:(b + 1) * N_HEADS])

  def project_out(s, tile, lo):
    y = _dot(_lane_blocks(wot_v, (), lo, ROWS)[:, :d_model],
             _lane_blocks(ob_v, (opaque_zero(s, 19),), 0, d_model))
    results.append(y[:SUBLANES, :LANES])
    rows = pl.ds(lo, ROWS)
    x1_v[tile, rows, :] = (xt_v[tile, rows, :].astype(F32)
                           + mod(2, lo, ROWS, NB) * y)

  per_block = lambda fn, s: [(fn, s, b) for b in range(NB)]
  norm1_steps = lambda s: [(norm1, s, b, i, 4)
                           for b in range(NB) for i in range(4)]
  qkv_steps = lambda s, a, b: [(project_qkv, s, lo) for lo in range(a, b, ROWS)]
  out_steps = lambda s, tile: [(project_out, s, tile, lo)
                               for lo in range(0, d_model, ROWS)]
  token_steps = lambda part: [(to_token_major, part, range(j, j + 3))
                              for j in range(0, pairs, 3)]
  attend_steps = lambda s, *ways: [(attend, s, g, *ways)
                                   for g in range(LANES // SUBLANES)]

  zero = lax.fori_loop(0, 2, lambda i, z: z + opaque_zero(i, 1), jnp.int32(0))
  edge_v[...] = jnp.zeros(edge_v.shape, edge_v.dtype)
  x1_v[0] = jnp.zeros(x1_v.shape[1:], F32)
  c_cp.wait()
  sc_v[0] = silu_c(LANES).T
  x_cps[0].wait()
  run(per_block(norm1_stats, zero))
  for cp, a, b in zip(wmod_cps[:3], mod_cuts, mod_cuts[1:]):
    cp.wait()
    for j in range(a, b):
      modulation(zero, j, 2)
  run([(norm1, zero, b, 0, 1) for b in range(NB)])

  wqkv_cps[0].wait()
  transpose_weights(wqkv_v, wqkvt_v, 0, qkv_cuts[1])
  run(qkv_steps(zero, 0, qkv_cuts[1]))
  wqkv_cps[1].wait()
  transpose_weights(wqkv_v, wqkvt_v, qkv_cuts[1], 3 * d_model)
  run(_interleave(qkv_steps(zero, *qkv_cuts[1:3]), (token_steps(0), 1, 4)))
  for cp in (x_cps[1], wo_cp, wmod_cps[3]):
    cp.wait()
  steps = qkv_steps(zero, *qkv_cuts[2:])
  n = len(steps)
  run(_interleave(
      steps,
      ([(modulation, zero, j, 1) for j in range(*mod_cuts[3:5])], 0, 2),
      (per_block(norm1_stats, zero + 1), 2, n - 1),
      ([(transpose_weights, wo_v, wot_v, 0, d_model)], 1, 2),
      (token_steps(1), 0, 1),
      (token_steps(2) + [(lambda: hold_x(newest[0]),)] + norm1_steps(zero + 1),
       n - 1, n)))
  for cp in x_cps[2:]:
    cp.wait()

  @pl.loop(0, last)
  def _(s):
    ahead = jnp.minimum(s + 2, last)
    run(_interleave(
        qkv_steps(s, 0, 3 * d_model),
        (attend_steps(s, 2, 3), 1, 17),
        ([(to_feature_major, s)], 17, 18),
        (per_block(norm1_stats, ahead), 18, 22),
        (per_block(norm2_stats, jnp.maximum(s - 1, 0)), 22, 26)))

    @pl.when(opaque_zero(s, 50) == 0)
    def _():
      steps = out_steps(s, s)
      run(_interleave(
          steps,
          (token_steps(0) + token_steps(1) + token_steps(2), 0, len(steps)),
          (norm1_steps(ahead), 0, len(steps) - 1)))

  def first_norm2(b, r):
    if len(results) >= 2:
      stat_v[1, n_tiles, 0, 0] = results[-2]
    if r is None:
      pin(*norm2_rest(zero, 0, 0))
    else:
      pin(*norm2(zero, 0, 0, b, r, True), *norm2(zero, 0, 0, b, r + SHARE, True))

  def transpose_leads():
    for j in range(N_CHUNKS):
      t = wg_v[j, pl.ds(2 * KH, n_rest), :].T
      lead_v[j] = jnp.concatenate(
          [t, jnp.zeros((fc, LANES - n_rest), BF16)], axis=1)

  for cp in (wmod_cps[4], *ff_cps):
    cp.wait()
  s = zero + last
  steps = out_steps(s, last)
  run([(modulation_mxu, *mod_cuts[4:])] + per_block(norm2_stats, s - 1)
      + attend_steps(s, WINDOW, dh) + [(to_feature_major, s)]
      + _interleave(steps, (
          [(first_norm2, 0, None)] + [(first_norm2, b, r)
                                      for b in range(NB // 2)
                                      for r in range(0, KH, 2 * SHARE)],
          0, len(steps) - 1))
      + [(transpose_leads,)] + [(norm2_stats, s, b, 3) for b in range(NB)])

  def finish(i, r, size):
    c11, c12, c21, c22 = _strassen_out(
        *(acc_v[i & 1, k, pl.ds(r, size), :] for k in range(7)))
    outs = []
    for lo, y in ((r, (c11, c12)), (r + mh, (c21, c22))):
      rows = pl.ds(lo, size)
      outs.append((x1_v[i, rows, :] + mod(5, lo, size, NB)
                   * jnp.concatenate(y, axis=1)).astype(out_v.dtype))
      out_v[i, rows, :] = outs[-1]
    return outs

  @pl.loop(0, n_tiles * N_CHUNKS)
  def _(step):
    i, j = lax.div(step, N_CHUNKS), lax.rem(step, N_CHUNKS)
    slot = i & 1
    first, second = pl.ds(0, fc // 2), pl.ds(fc // 2, fc // 2)

    def products(w_v, blocks, dot, rhs, order, extra, side_work):
      out = {}
      side_work, started = list(side_work), []
      for k in order:
        if results:
          w_v[(N_CHUNKS, *spare_bf16)] = pltpu.bitcast(
              _token([results[-1], *started]), BF16)
          started = side_work.pop(0)(results[-1]) if side_work else []
        terms = [w_v[(j, *blocks[q])] for _, q in _LHS_TERMS[k]]
        lhs = terms[0]
        if len(terms) == 2:
          x, y = (t.astype(F32) for t in terms)
          lhs = (x + y if _LHS_TERMS[k][1][0] > 0 else x - y).astype(BF16)
        if k in extra:
          lhs = jnp.concatenate([lhs, w_v[(j, *extra[k])]], axis=0)
        out[k] = dot(lhs, rhs[k])
        results.append(out[k][:SUBLANES, :LANES])
      return out

    def project(w_v, lead, side_work):
      top, bottom, rest = pl.ds(0, KH), pl.ds(KH, KH), pl.ds(2 * KH, n_rest)
      rhs = [_lane_blocks(hb_v, (slot, k), 0, KH) for k in range(7)]
      hr = _lane_blocks(hr_v, (slot,), 0, n_rest)
      if lead:
        r12, r21 = (
            _dot(_load_bf16(lead_v, (j,), lo, fc // 2)[:, :n_rest], h)
            for lo, h in ((0, hr[:, half:]), (fc // 2, hr[:, :half])))
      else:
        r12 = _dot_tn(w_v[j, rest, first], hr[:, half:])
        r21 = _dot_tn(w_v[j, rest, second], hr[:, :half])
      results.append(r21[:SUBLANES, :LANES])
      rhs[5] = jnp.concatenate([rhs[5], hr[:, half:]], axis=0)
      rhs[6] = jnp.concatenate([rhs[6], hr[:, :half]], axis=0)
      m = products(
          w_v, ((top, first), (bottom, first), (top, second), (bottom, second)),
          _dot_tn, rhs, (2, 3, 1, 4, 0, 6, 5),
          {5: (rest, second), 6: (rest, first)}, side_work)
      c11, c12, c21, c22 = _strassen_out(*(m[k] for k in range(7)))
      return c11, c12 + r12, c21 + r21, c22

    def finish_share(n, after):
      acc_v[(2, 0, *spare)] = after
      r = pl.multiple_of(j * (mh // N_CHUNKS) + n * SHARE, 2 * SUBLANES)
      return finish(jnp.maximum(i - 1, 0), r, SHARE)

    def norm2_share(n, after):
      x1_v[(n_tiles, *spare)] = after
      nxt = jnp.minimum(i + 1, last)
      if n is None:
        return norm2_rest(nxt, nxt, 1 - slot)
      r = jnp.minimum(j * 3 * SHARE, KH - 3 * SHARE) + n // 2 * SHARE
      return norm2(nxt, nxt, 1 - slot, n % 2, pl.multiple_of(r, 2 * SUBLANES))

    idle = lambda after: []
    norm2_shares = [functools.partial(norm2_share, n)
                    for n in (None, *range(6))]
    g = project(wg_v, True, [idle] * 3 + [
        functools.partial(finish_share, n)
        for n in range(mh // N_CHUNKS // SHARE)])
    u = project(wu_v, False, norm2_shares[:-1])
    top, bottom = pl.ds(0, mh), pl.ds(mh, mh)
    order = (2, 3, 0, 4, 6, 1, 5)
    m = products(
        wdt_v, ((top, first), (top, second), (bottom, first), (bottom, second)),
        _dot, _strassen_rhs(*(a * b for a, b in zip(g, u))), order, {},
        norm2_shares[-1:])
    for k in order:
      acc_v[slot, k] = jnp.where(j > 0, acc_v[slot, k], 0.0) + m[k]
    results.clear()
    normalized.clear()

    @pl.when((j == N_CHUNKS - 1) & (i > 0))
    def _():
      out_copy(i - 1).start()

  last_cps = []
  for r in range(0, mh, mh // 3):
    finish(last, r, mh // 3)
    for lo in (r, r + mh):
      rows = pl.ds(lo, mh // 3)
      last_cps.append(pltpu.make_async_copy(
          out_v.at[last, rows], out_hbm.at[rows, pl.ds(last * TILE, TILE)],
          out_sem.at[last + len(last_cps)]))
      last_cps[-1].start()
  for cp in (*map(out_copy, range(last)), *last_cps):
    cp.wait()


@jax.jit
def pallas_adaLN_cond__sliding_local_dilated__glu_gated_bilinear__prompt_kernel(
    A_x: jax.Array,
    A_wqkv: jax.Array,
    A_wo: jax.Array,
    B_x: jax.Array,
    B_w_gate: jax.Array,
    B_w_up: jax.Array,
    B_w_down: jax.Array,
    c: jax.Array,
    w_mod: jax.Array,
):
  del B_x
  batch, seq, d_model = A_x.shape
  d_ff = B_w_gate.shape[1]
  assert (batch, d_model, d_ff) == (1, 576, 4608) and seq % TILE == 0
  dh = d_model // N_HEADS
  n_tiles = seq // TILE
  fc = d_ff // N_CHUNKS
  k_blocks = pl.cdiv(d_model, LANES)
  operands = (A_x.reshape(seq, d_model).T, A_wqkv, A_wo, B_w_gate, B_w_up,
              B_w_down.T, c, w_mod)
  hbm = pl.BlockSpec(memory_space=pltpu.HBM)
  vmem = pltpu.VMEM
  out_t = pl.pallas_call(
      _kernel,
      in_specs=[hbm] * len(operands),
      out_specs=hbm,
      out_shape=jax.ShapeDtypeStruct((d_model, seq), A_x.dtype),
      scratch_shapes=[
          vmem((n_tiles + 1, d_model, TILE), BF16),
          vmem(A_wqkv.shape, BF16),
          vmem(A_wo.shape, BF16),
          *[vmem((N_CHUNKS + 1, d_model, fc), BF16)] * 3,
          vmem(c.shape, BF16),
          vmem(w_mod.shape, BF16),
          vmem((1, d_model, LANES), F32),
          vmem((6 * d_model, LANES), F32),
          vmem((2, n_tiles + 1, 2, NB, SUBLANES, LANES), F32),
          vmem((k_blocks, 3 * d_model, LANES), BF16),
          vmem((k_blocks, d_model, LANES), BF16),
          vmem((2, NB, d_model, LANES), BF16),
          vmem((NB, 3 * d_model, LANES), BF16),
          vmem((2, dh // 2, HALO, LANES), I32),
          vmem((dh, LANES, LANES), F32),
          vmem((dh, HALO + LANES, LANES), F32),
          vmem((dh, HALO + LANES, LANES), F32),
          vmem((dh // 2, 2 * LANES, LANES), F32),
          vmem((dh // 2, 2 * LANES, LANES), BF16),
          vmem((2, NB, d_model, LANES), BF16),
          vmem((n_tiles + 1, d_model, TILE), F32),
          vmem((2, 7, NB // 2, KH, LANES), BF16),
          vmem((2, NB, d_model - 2 * KH, LANES), BF16),
          vmem((N_CHUNKS, fc, LANES), BF16),
          vmem((3, 7, d_model // 2, TILE // 2), F32),
          vmem((n_tiles, d_model, TILE), A_x.dtype),
          pltpu.SemaphoreType.DMA((9 + n_tiles + 3 * N_CHUNKS,)),
          pltpu.SemaphoreType.DMA((n_tiles + 5,)),
      ],
      compiler_params=pltpu.CompilerParams(vmem_limit_bytes=100 * 2**20),
      name="adaln_window_attn_glu",
  )(*operands)
  return out_t.T.reshape(batch, seq, d_model)
```

```python
import functools

import jax
import jax.numpy as jnp
from jax import lax
import jax.experimental.pallas as pl
import jax.experimental.pallas.tpu as pltpu

N_HEADS = 32
WINDOW = 8
DILATION = 2
LN_EPS = 1e-5
MASK_VALUE = -1000000000.0

LANES = 128
SUBLANES = 8
NB = LANES // N_HEADS
TILE = NB * LANES
HALO = 16
KH = 256
N_CHUNKS = 3
ROWS = 64
SHARE = 32

F32 = jnp.float32
BF16 = jnp.bfloat16
I32 = jnp.int32

_LHS_TERMS = (((1, 0), (1, 3)), ((1, 2), (1, 3)), ((1, 0),), ((1, 3),),
              ((1, 0), (1, 1)), ((1, 2), (-1, 0)), ((1, 1), (-1, 3)))


def _strassen_rhs(b11, b12, b21, b22):
  return tuple(b.astype(BF16) for b in (
      b11 + b22, b11, b12 - b22, b21 - b11, b22, b11 + b12, b21 + b22))


def _strassen_out(m1, m2, m3, m4, m5, m6, m7):
  return m1 + m4 - m5 + m7, m3 + m5, m2 + m4, m1 - m2 + m3 + m6


def _dot(a, b):
  return jnp.dot(a, b, preferred_element_type=F32)


def _dot_tn(a, b):
  return lax.dot_general(a, b, (((0,), (0,)), ((), ())),
                         preferred_element_type=F32)


def _load_bf16(ref, lead, lo, size):
  words = ref.bitcast(I32)[(*lead, pl.ds(lo // 2, size // 2), slice(None))]
  return pltpu.bitcast(words, BF16)


def _lane_blocks(ref, lead, lo, size):
  return jnp.concatenate([_load_bf16(ref, (*lead, b), lo, size)
                          for b in range(ref.shape[len(lead)])], axis=1)


def _column_sum(x, chains):
  size = chains * SUBLANES
  acc = functools.reduce(
      jnp.add, [x[i:i + size] for i in range(0, x.shape[0], size)])
  return jnp.sum(acc, axis=0, keepdims=True)


def _after(x, earlier, zero):
  return pltpu.bitcast(
      pltpu.bitcast(x, I32) | (pltpu.bitcast(earlier, I32) & zero), F32)


def _token(vals):
  regs = []
  for v in vals:
    v = pltpu.bitcast(v, I32)
    regs += [v[i:i + SUBLANES, k:k + LANES]
             for i in range(0, v.shape[0], SUBLANES)
             for k in range(0, v.shape[1], LANES)]
  return functools.reduce(jnp.bitwise_or, regs)


def _interleave(matmuls, *placed):
  slots = [[m] for m in matmuls]
  for pieces, lo, hi in placed:
    for k, piece in enumerate(pieces):
      slots[lo + k * (hi - lo) // len(pieces)].append(piece)
  return [piece for slot in slots for piece in slot]


def _kernel(xt_hbm, wqkv_hbm, wo_hbm, wg_hbm, wu_hbm, wdt_hbm, c_hbm, wmod_hbm,
            out_hbm,
            xt_v, wqkv_v, wo_v, wg_v, wu_v, wdt_v, c_v, wmod_v,
            sc_v, mod_v, stat_v, wqkvt_v, wot_v, h1_v, qkv_v, edge_v,
            qt_v, kt_v, vt_v, ot_v, op_v, ob_v, x1_v, hb_v, hr_v, lead_v,
            acc_v, out_v, in_sem, out_sem):
  d_model, seq = xt_hbm.shape
  dh = d_model // N_HEADS
  pairs = dh // 2
  n_tiles = seq // TILE
  last = n_tiles - 1
  fc = wg_hbm.shape[1] // N_CHUNKS
  mh = d_model // 2
  half = TILE // 2
  n_rest = d_model - 2 * KH
  spare = (pl.ds(0, SUBLANES), pl.ds(0, LANES))
  spare_bf16 = (pl.ds(0, 2 * SUBLANES), pl.ds(0, LANES))

  sems = iter(range(in_sem.shape[0]))
  copy = lambda src, dst: pltpu.make_async_copy(src, dst, in_sem.at[next(sems)])

  def col_copies(src, dst, cuts):
    return [copy(src.at[:, pl.ds(a, b - a)], dst.at[:, pl.ds(a, b - a)])
            for a, b in zip(cuts, cuts[1:])]

  mod_cuts = (0, 3, 6, 9, 14, 6 * d_model // LANES)
  qkv_cuts = (0, 512, 1280, 3 * d_model)
  c_cp = copy(c_hbm, c_v)
  wmod_cps = col_copies(wmod_hbm, wmod_v, [j * LANES for j in mod_cuts])
  wqkv_cps = col_copies(wqkv_hbm, wqkv_v, (0, qkv_cuts[1], 3 * d_model))
  wo_cp = copy(wo_hbm, wo_v)
  x_cps = [copy(xt_hbm.at[:, pl.ds(i * TILE, TILE)], xt_v.at[i])
           for i in range(n_tiles)]
  ff_cps = [copy(w_hbm.at[:, pl.ds(j * fc, fc)], w_v.at[j])
            for j in range(N_CHUNKS)
            for w_hbm, w_v in ((wg_hbm, wg_v), (wu_hbm, wu_v), (wdt_hbm, wdt_v))]
  for cp in (c_cp, x_cps[0], *wmod_cps[:3], *wqkv_cps, x_cps[1], wo_cp,
             wmod_cps[3], *x_cps[2:], wmod_cps[4], *ff_cps):
    cp.start()

  def out_copy(i):
    start = i * TILE if isinstance(i, int) else pl.multiple_of(i * TILE, TILE)
    return pltpu.make_async_copy(
        out_v.at[i], out_hbm.at[:, pl.ds(start, TILE)], out_sem.at[i])

  def opaque_zero(s, k):
    return lax.shift_right_logical(s + k, 16)

  next_operand = [None]
  results = []
  newest = [None]
  normalized = []

  def pin(*vals):
    if next_operand[0] is not None:
      next_operand[0].bitcast(I32)[1, 0, pl.ds(0, SUBLANES), :] = _token(vals)

  def run(steps):
    for n, (fn, *args) in enumerate(steps):
      later = [f for f, *_ in steps[n + 1:] if f in (project_qkv, project_out)]
      next_operand[0] = (None if not later
                         else h1_v if later[0] is project_qkv else ob_v)
      fn(*args)
    next_operand[0] = None
    results.clear()
    normalized.clear()

  def silu_c(rows):
    cv = c_v[...].astype(F32)
    return jnp.broadcast_to(cv * jax.nn.sigmoid(cv), (rows, d_model))

  def store_modulation(j, row):
    part = (j * LANES + lax.broadcasted_iota(I32, (1, LANES), 1)) // d_model
    row = jnp.where((part == 1) | (part == 4), row + 1.0, row)
    mod_v[pl.ds(j * LANES, LANES), :] = jnp.broadcast_to(row, (LANES, LANES)).T

  def modulation(s, j, chains):
    w = wmod_v[:, pl.ds(j * LANES, LANES)].astype(F32)
    row = _column_sum(w * sc_v[opaque_zero(s, 60)], chains)
    pin(jnp.broadcast_to(row, (SUBLANES, LANES)))
    store_modulation(j, row)

  def modulation_mxu(lo, hi):
    rows = _dot(silu_c(2 * SUBLANES).astype(BF16),
                wmod_v[:, pl.ds(lo * LANES, (hi - lo) * LANES)])
    for j in range(lo, hi):
      store_modulation(j, rows[:1, (j - lo) * LANES:(j - lo + 1) * LANES])

  def mod(part, lo, size, n=1):
    col = mod_v[pl.ds(part * d_model + lo, size), :]
    return col if n == 1 else jnp.concatenate([col] * n, axis=1)

  def moments(load, which, s, b, chains):
    inv_d = 1.0 / d_model
    mean = _column_sum(load(0), chains) * inv_d
    xc = load(1) - mean
    var = _column_sum(xc * xc, chains) * inv_d
    for k, v in enumerate((mean, lax.rsqrt(var + LN_EPS))):
      stat_v[which, s, k, b] = v = jnp.broadcast_to(v, (SUBLANES, LANES))
    pin(v)

  def normalize(x, which, s, b, lo, serial=False):
    size = x.shape[0]
    mean, rstd = stat_v[which, s, 0, b], stat_v[which, s, 1, b]
    if serial and normalized:
      mean = _after(mean, normalized[-1], opaque_zero(s, 36))
    mean, rstd = (jnp.tile(v, (size // SUBLANES, 1)) for v in (mean, rstd))
    y = ((x - mean) * rstd * mod(3 * which + 1, lo, size)
         + mod(3 * which, lo, size))
    normalized.append(y[:SUBLANES])
    return y

  def hold_x(v):
    xt_v[(n_tiles, *spare_bf16)] = pltpu.bitcast(v, BF16)

  def norm1_stats(s, b):
    if len(results) >= 2:
      hold_x(results[-2])
    cols = pl.ds(b * LANES, LANES)
    moments(lambda k: xt_v[s + opaque_zero(s, 32 + k), :, cols].astype(F32),
            0, s, b, 2)

  def norm1(s, b, i, n):
    size = d_model // n
    rows = pl.ds(i * size, size)
    x = xt_v[s + opaque_zero(s, 34), rows, pl.ds(b * LANES, LANES)]
    h1_v[0, b, rows, :] = normalize(x.astype(F32), 0, s, b, i * size).astype(BF16)

  def norm2_stats(s, b, chains=2):
    if len(results) >= 2 and next_operand[0] is not None:
      x1_v[(n_tiles, *spare)] = results[-2]
    cols = pl.ds(b * LANES, LANES)
    moments(lambda k: x1_v[s + opaque_zero(s, 40 + k), :, cols], 1, s, b, chains)

  def norm2(s, tile, slot, b, r, serial=False):
    def h(side, row):
      blk = b + side * NB // 2
      x = x1_v[tile, pl.ds(row, SHARE), pl.ds(blk * LANES, LANES)]
      return normalize(x, 1, s, blk, row, serial)

    outs = _strassen_rhs(h(0, r), h(1, r), h(0, r + KH), h(1, r + KH))
    for k in range(7):
      hb_v[slot, k, b, pl.ds(r, SHARE), :] = outs[k]
    return list(outs)

  def norm2_rest(s, tile, slot):
    rows = pl.ds(2 * KH, n_rest)
    outs = [normalize(x1_v[tile, rows, pl.ds(b * LANES, LANES)], 1, s, b,
                      2 * KH).astype(BF16) for b in range(NB)]
    for b in range(NB):
      hr_v[slot, b] = outs[b]
    return outs

  def transpose_weights(w_v, wt_v, a, b):
    for k in range(0, d_model, LANES):
      size = min(LANES, d_model - k)
      t = w_v[pl.ds(k, size), pl.ds(a, b - a)].T
      if size < LANES:
        t = jnp.concatenate([t, jnp.zeros((b - a, LANES - size), BF16)], axis=1)
      wt_v[k // LANES, pl.ds(a, b - a), :] = t

  def project_qkv(s, lo):
    qkv = _dot(_lane_blocks(wqkvt_v, (), lo, ROWS)[:, :d_model],
               _lane_blocks(h1_v, (opaque_zero(s, 17),), 0, d_model))
    results.append(qkv[:SUBLANES, :LANES])
    newest[0] = qkv[-SUBLANES:, -LANES:]
    for b in range(NB):
      qkv_v[b, pl.ds(lo, ROWS), :] = (
          qkv[:, b * LANES:(b + 1) * LANES].astype(BF16))

  def to_token_major(part, js):
    buf = (qt_v, kt_v, vt_v)[part]
    for j in js:
      rows = pl.ds(part * mh + j, N_HEADS, stride=pairs)
      t = jnp.concatenate(
          [qkv_v.bitcast(I32)[b, rows, :] for b in range(NB)], axis=0).T
      if part:
        lane = lax.broadcasted_iota(I32, (HALO, LANES), 1)
        before = jnp.where(lane < LANES - N_HEADS, t[-HALO:], edge_v[part - 1, j])
        edge_v[part - 1, j] = t[-HALO:]
        t = jnp.concatenate([pltpu.roll(before, N_HEADS, 1), t], axis=0)
      buf[2 * j] = pltpu.bitcast(t << 16, F32)
      buf[2 * j + 1] = pltpu.bitcast(t & -65536, F32)

  probs = {}

  def window(g, w):
    return pl.ds(HALO + g * SUBLANES - DILATION * w, SUBLANES)

  def scores(s, g, ways):
    r0 = g * SUBLANES
    z = opaque_zero(s, g)
    q = [qt_v[z + d, pl.ds(r0, SUBLANES), :] for d in range(dh)]
    logits = []
    for w in range(WINDOW):
      q0 = q[0] if w < ways else _after(q[0], logits[w - ways], z)
      logits.append(functools.reduce(jnp.add, [
          qd * kt_v[z + d, window(g, w), :]
          for d, qd in enumerate([q0, *q[1:]])]))
    for w in range(WINDOW):
      logits[w] = logits[w] * dh ** -0.5
      if r0 < DILATION * w:
        shape = (SUBLANES, LANES)
        pos = (s * TILE + r0 + lax.broadcasted_iota(I32, shape, 0)
               + lax.broadcasted_iota(I32, shape, 1) // N_HEADS * LANES)
        logits[w] = jnp.where(pos >= DILATION * w, logits[w], MASK_VALUE)
    m = functools.reduce(jnp.maximum, logits)
    e = [jnp.exp(l - m) for l in logits]
    inv = 1.0 / functools.reduce(jnp.add, e)
    probs[g] = [x * inv for x in e]
    return [inv]

  def mix(s, g, ways):
    z = opaque_zero(s, g)
    p = probs.pop(g)
    outs = []
    for d in range(dh):
      p0 = p[0] if d < ways else _after(p[0], outs[d - ways], z)
      outs.append(functools.reduce(jnp.add, [
          pw * vt_v[z + d, window(g, w), :]
          for w, pw in enumerate([p0, *p[1:]])]))
      rows = pl.ds(2 * g * SUBLANES + d % 2, SUBLANES, stride=2)
      ot_v[d // 2, rows, :] = outs[-1]
    return outs[-ways:]

  def attend(s, g, ways_qk, ways_pv):
    pin(*(scores(s, g, ways_qk) if g < LANES // SUBLANES else []),
        *(mix(s, g - 1, ways_pv) if g else []))

  def to_feature_major(s):
    for j in range(pairs):
      op_v[j] = ot_v[opaque_zero(s, 18) + j].astype(BF16)
      t = op_v.bitcast(I32)[j].T
      for b in range(NB):
        ob_v.bitcast(I32)[0, b, pl.ds(j, N_HEADS, stride=pairs), :] = (
            t[b * N_HEADS:(b + 1) * N_HEADS])

  def project_out(s, tile, lo):
    y = _dot(_lane_blocks(wot_v, (), lo, ROWS)[:, :d_model],
             _lane_blocks(ob_v, (opaque_zero(s, 19),), 0, d_model))
    results.append(y[:SUBLANES, :LANES])
    rows = pl.ds(lo, ROWS)
    x1_v[tile, rows, :] = (xt_v[tile, rows, :].astype(F32)
                           + mod(2, lo, ROWS, NB) * y)

  per_block = lambda fn, s: [(fn, s, b) for b in range(NB)]
  norm1_steps = lambda s: [(norm1, s, b, i, 4)
                           for b in range(NB) for i in range(4)]
  qkv_steps = lambda s, a, b: [(project_qkv, s, lo) for lo in range(a, b, ROWS)]
  out_steps = lambda s, tile: [(project_out, s, tile, lo)
                               for lo in range(0, d_model, ROWS)]
  token_steps = lambda part: [(to_token_major, part, range(j, j + 3))
                              for j in range(0, pairs, 3)]
  attend_steps = lambda s, *ways: [(attend, s, g, *ways)
                                   for g in range(LANES // SUBLANES + 1)]

  zero = lax.fori_loop(0, 2, lambda i, z: z + opaque_zero(i, 1), jnp.int32(0))
  edge_v[...] = jnp.zeros(edge_v.shape, edge_v.dtype)
  x1_v[0] = jnp.zeros(x1_v.shape[1:], F32)
  c_cp.wait()
  sc_v[0] = silu_c(LANES).T
  x_cps[0].wait()
  run(per_block(norm1_stats, zero))
  for cp, a, b in zip(wmod_cps[:3], mod_cuts, mod_cuts[1:]):
    cp.wait()
    for j in range(a, b):
      modulation(zero, j, 2)
  run([(norm1, zero, b, 0, 1) for b in range(NB)])

  wqkv_cps[0].wait()
  transpose_weights(wqkv_v, wqkvt_v, 0, qkv_cuts[1])
  run(qkv_steps(zero, 0, qkv_cuts[1]))
  wqkv_cps[1].wait()
  transpose_weights(wqkv_v, wqkvt_v, qkv_cuts[1], 3 * d_model)
  run(_interleave(qkv_steps(zero, *qkv_cuts[1:3]), (token_steps(0), 1, 4)))
  for cp in (x_cps[1], wo_cp, wmod_cps[3]):
    cp.wait()
  steps = qkv_steps(zero, *qkv_cuts[2:])
  n = len(steps)
  run(_interleave(
      steps,
      ([(modulation, zero, j, 1) for j in range(*mod_cuts[3:5])], 0, 2),
      (per_block(norm1_stats, zero + 1), 2, n - 1),
      ([(transpose_weights, wo_v, wot_v, 0, d_model)], 1, 2),
      (token_steps(1), 0, 1),
      (token_steps(2) + [(lambda: hold_x(newest[0]),)] + norm1_steps(zero + 1),
       n - 1, n)))
  for cp in x_cps[2:]:
    cp.wait()

  @pl.loop(0, last)
  def _(s):
    ahead = jnp.minimum(s + 2, last)
    run(_interleave(
        qkv_steps(s, 0, 3 * d_model),
        (attend_steps(s, 2, 2), 1, 18),
        ([(to_feature_major, s)], 18, 19),
        (per_block(norm1_stats, ahead), 18, 22),
        (per_block(norm2_stats, jnp.maximum(s - 1, 0)), 22, 26)))

    @pl.when(opaque_zero(s, 50) == 0)
    def _():
      steps = out_steps(s, s)
      run(_interleave(
          steps,
          (token_steps(0) + token_steps(1) + token_steps(2), 0, len(steps)),
          (norm1_steps(ahead), 0, len(steps) - 1)))

  def first_norm2(b, r):
    if len(results) >= 2:
      stat_v[1, n_tiles, 0, 0] = results[-2]
    if r is None:
      pin(*norm2_rest(zero, 0, 0))
    else:
      pin(*norm2(zero, 0, 0, b, r, True), *norm2(zero, 0, 0, b, r + SHARE, True))

  def transpose_leads():
    for j in range(N_CHUNKS):
      t = wg_v[j, pl.ds(2 * KH, n_rest), :].T
      lead_v[j] = jnp.concatenate(
          [t, jnp.zeros((fc, LANES - n_rest), BF16)], axis=1)

  for cp in (wmod_cps[4], *ff_cps):
    cp.wait()
  s = zero + last
  steps = out_steps(s, last)
  run([(modulation_mxu, *mod_cuts[4:])] + per_block(norm2_stats, s - 1)
      + attend_steps(s, WINDOW, dh) + [(to_feature_major, s)]
      + _interleave(steps, (
          [(first_norm2, 0, None)] + [(first_norm2, b, r)
                                      for b in range(NB // 2)
                                      for r in range(0, KH, 2 * SHARE)],
          0, len(steps) - 1))
      + [(transpose_leads,)] + [(norm2_stats, s, b, 3) for b in range(NB)])

  def finish(i, r, size):
    c11, c12, c21, c22 = _strassen_out(
        *(acc_v[i & 1, k, pl.ds(r, size), :] for k in range(7)))
    outs = []
    for lo, y in ((r, (c11, c12)), (r + mh, (c21, c22))):
      rows = pl.ds(lo, size)
      outs.append((x1_v[i, rows, :] + mod(5, lo, size, NB)
                   * jnp.concatenate(y, axis=1)).astype(out_v.dtype))
      out_v[i, rows, :] = outs[-1]
    return outs

  @pl.loop(0, n_tiles * N_CHUNKS)
  def _(step):
    i, j = lax.div(step, N_CHUNKS), lax.rem(step, N_CHUNKS)
    slot = i & 1
    first, second = pl.ds(0, fc // 2), pl.ds(fc // 2, fc // 2)

    def products(w_v, blocks, dot, rhs, order, extra, side_work):
      out = {}
      side_work, started = list(side_work), []
      for k in order:
        if results:
          w_v[(N_CHUNKS, *spare_bf16)] = pltpu.bitcast(
              _token([results[-1], *started]), BF16)
          started = side_work.pop(0)(results[-1]) if side_work else []
        terms = [w_v[(j, *blocks[q])] for _, q in _LHS_TERMS[k]]
        lhs = terms[0]
        if len(terms) == 2:
          x, y = (t.astype(F32) for t in terms)
          lhs = (x + y if _LHS_TERMS[k][1][0] > 0 else x - y).astype(BF16)
        if k in extra:
          lhs = jnp.concatenate([lhs, w_v[(j, *extra[k])]], axis=0)
        out[k] = dot(lhs, rhs[k])
        results.append(out[k][:SUBLANES, :LANES])
      return out

    def project(w_v, lead, side_work):
      top, bottom, rest = pl.ds(0, KH), pl.ds(KH, KH), pl.ds(2 * KH, n_rest)
      rhs = [_lane_blocks(hb_v, (slot, k), 0, KH) for k in range(7)]
      hr = _lane_blocks(hr_v, (slot,), 0, n_rest)
      if lead:
        r12, r21 = (
            _dot(_load_bf16(lead_v, (j,), lo, fc // 2)[:, :n_rest], h)
            for lo, h in ((0, hr[:, half:]), (fc // 2, hr[:, :half])))
      else:
        r12 = _dot_tn(w_v[j, rest, first], hr[:, half:])
        r21 = _dot_tn(w_v[j, rest, second], hr[:, :half])
      results.append(r21[:SUBLANES, :LANES])
      rhs[5] = jnp.concatenate([rhs[5], hr[:, half:]], axis=0)
      rhs[6] = jnp.concatenate([rhs[6], hr[:, :half]], axis=0)
      m = products(
          w_v, ((top, first), (bottom, first), (top, second), (bottom, second)),
          _dot_tn, rhs, (2, 3, 1, 4, 0, 6, 5),
          {5: (rest, second), 6: (rest, first)}, side_work)
      c11, c12, c21, c22 = _strassen_out(*(m[k] for k in range(7)))
      return c11, c12 + r12, c21 + r21, c22

    def finish_share(n, after):
      acc_v[(2, 0, *spare)] = after
      r = pl.multiple_of(j * (mh // N_CHUNKS) + n * SHARE, 2 * SUBLANES)
      return finish(jnp.maximum(i - 1, 0), r, SHARE)

    def norm2_share(n, after):
      x1_v[(n_tiles, *spare)] = after
      nxt = jnp.minimum(i + 1, last)
      if n is None:
        return norm2_rest(nxt, nxt, 1 - slot)
      r = jnp.minimum(j * 3 * SHARE, KH - 3 * SHARE) + n // 2 * SHARE
      return norm2(nxt, nxt, 1 - slot, n % 2, pl.multiple_of(r, 2 * SUBLANES))

    idle = lambda after: []
    norm2_shares = [functools.partial(norm2_share, n)
                    for n in (None, *range(6))]
    g = project(wg_v, True, [idle] * 3 + [
        functools.partial(finish_share, n)
        for n in range(mh // N_CHUNKS // SHARE)])
    u = project(wu_v, False, norm2_shares[:-1])
    top, bottom = pl.ds(0, mh), pl.ds(mh, mh)
    order = (2, 3, 0, 4, 6, 1, 5)
    m = products(
        wdt_v, ((top, first), (top, second), (bottom, first), (bottom, second)),
        _dot, _strassen_rhs(*(a * b for a, b in zip(g, u))), order, {},
        norm2_shares[-1:])
    for k in order:
      acc_v[slot, k] = jnp.where(j > 0, acc_v[slot, k], 0.0) + m[k]
    results.clear()
    normalized.clear()

    @pl.when((j == N_CHUNKS - 1) & (i > 0))
    def _():
      out_copy(i - 1).start()

  last_cps = []
  for r in range(0, mh, mh // 3):
    finish(last, r, mh // 3)
    for lo in (r, r + mh):
      rows = pl.ds(lo, mh // 3)
      last_cps.append(pltpu.make_async_copy(
          out_v.at[last, rows], out_hbm.at[rows, pl.ds(last * TILE, TILE)],
          out_sem.at[last + len(last_cps)]))
      last_cps[-1].start()
  for cp in (*map(out_copy, range(last)), *last_cps):
    cp.wait()


@jax.jit
def pallas_adaLN_cond__sliding_local_dilated__glu_gated_bilinear__prompt_kernel(
    A_x: jax.Array,
    A_wqkv: jax.Array,
    A_wo: jax.Array,
    B_x: jax.Array,
    B_w_gate: jax.Array,
    B_w_up: jax.Array,
    B_w_down: jax.Array,
    c: jax.Array,
    w_mod: jax.Array,
):
  del B_x
  batch, seq, d_model = A_x.shape
  d_ff = B_w_gate.shape[1]
  assert (batch, d_model, d_ff) == (1, 576, 4608) and seq % TILE == 0
  dh = d_model // N_HEADS
  n_tiles = seq // TILE
  fc = d_ff // N_CHUNKS
  k_blocks = pl.cdiv(d_model, LANES)
  operands = (A_x.reshape(seq, d_model).T, A_wqkv, A_wo, B_w_gate, B_w_up,
              B_w_down.T, c, w_mod)
  hbm = pl.BlockSpec(memory_space=pltpu.HBM)
  vmem = pltpu.VMEM
  out_t = pl.pallas_call(
      _kernel,
      in_specs=[hbm] * len(operands),
      out_specs=hbm,
      out_shape=jax.ShapeDtypeStruct((d_model, seq), A_x.dtype),
      scratch_shapes=[
          vmem((n_tiles + 1, d_model, TILE), BF16),
          vmem(A_wqkv.shape, BF16),
          vmem(A_wo.shape, BF16),
          *[vmem((N_CHUNKS + 1, d_model, fc), BF16)] * 3,
          vmem(c.shape, BF16),
          vmem(w_mod.shape, BF16),
          vmem((1, d_model, LANES), F32),
          vmem((6 * d_model, LANES), F32),
          vmem((2, n_tiles + 1, 2, NB, SUBLANES, LANES), F32),
          vmem((k_blocks, 3 * d_model, LANES), BF16),
          vmem((k_blocks, d_model, LANES), BF16),
          vmem((2, NB, d_model, LANES), BF16),
          vmem((NB, 3 * d_model, LANES), BF16),
          vmem((2, dh // 2, HALO, LANES), I32),
          vmem((dh, LANES, LANES), F32),
          vmem((dh, HALO + LANES, LANES), F32),
          vmem((dh, HALO + LANES, LANES), F32),
          vmem((dh // 2, 2 * LANES, LANES), F32),
          vmem((dh // 2, 2 * LANES, LANES), BF16),
          vmem((2, NB, d_model, LANES), BF16),
          vmem((n_tiles + 1, d_model, TILE), F32),
          vmem((2, 7, NB // 2, KH, LANES), BF16),
          vmem((2, NB, d_model - 2 * KH, LANES), BF16),
          vmem((N_CHUNKS, fc, LANES), BF16),
          vmem((3, 7, d_model // 2, TILE // 2), F32),
          vmem((n_tiles, d_model, TILE), A_x.dtype),
          pltpu.SemaphoreType.DMA((9 + n_tiles + 3 * N_CHUNKS,)),
          pltpu.SemaphoreType.DMA((n_tiles + 5,)),
      ],
      compiler_params=pltpu.CompilerParams(vmem_limit_bytes=100 * 2**20),
      name="adaln_window_attn_glu",
  )(*operands)
  return out_t.T.reshape(batch, seq, d_model)
```

```python
import functools

import jax
import jax.numpy as jnp
from jax import lax
import jax.experimental.pallas as pl
import jax.experimental.pallas.tpu as pltpu

N_HEADS = 32
WINDOW = 8
DILATION = 2
LN_EPS = 1e-5
MASK_VALUE = -1000000000.0

LANES = 128
SUBLANES = 8
NB = LANES // N_HEADS
TILE = NB * LANES
HALO = 16
KH = 256
N_CHUNKS = 3
ROWS = 64
SHARE = 32

F32 = jnp.float32
BF16 = jnp.bfloat16
I32 = jnp.int32

_LHS_TERMS = (((1, 0), (1, 3)), ((1, 2), (1, 3)), ((1, 0),), ((1, 3),),
              ((1, 0), (1, 1)), ((1, 2), (-1, 0)), ((1, 1), (-1, 3)))


def _strassen_rhs(b11, b12, b21, b22):
  return tuple(b.astype(BF16) for b in (
      b11 + b22, b11, b12 - b22, b21 - b11, b22, b11 + b12, b21 + b22))


def _strassen_out(m1, m2, m3, m4, m5, m6, m7):
  return m1 + m4 - m5 + m7, m3 + m5, m2 + m4, m1 - m2 + m3 + m6


def _dot(a, b):
  return jnp.dot(a, b, preferred_element_type=F32)


def _dot_tn(a, b):
  return lax.dot_general(a, b, (((0,), (0,)), ((), ())),
                         preferred_element_type=F32)


def _load_bf16(ref, lead, lo, size):
  words = ref.bitcast(I32)[(*lead, pl.ds(lo // 2, size // 2), slice(None))]
  return pltpu.bitcast(words, BF16)


def _lane_blocks(ref, lead, lo, size):
  return jnp.concatenate([_load_bf16(ref, (*lead, b), lo, size)
                          for b in range(ref.shape[len(lead)])], axis=1)


def _column_sum(x, chains):
  size = chains * SUBLANES
  acc = functools.reduce(
      jnp.add, [x[i:i + size] for i in range(0, x.shape[0], size)])
  return jnp.sum(acc, axis=0, keepdims=True)


def _after(x, earlier, zero):
  return pltpu.bitcast(
      pltpu.bitcast(x, I32) | (pltpu.bitcast(earlier, I32) & zero), F32)


def _token(vals):
  regs = []
  for v in vals:
    v = pltpu.bitcast(v, I32)
    regs += [v[i:i + SUBLANES, k:k + LANES]
             for i in range(0, v.shape[0], SUBLANES)
             for k in range(0, v.shape[1], LANES)]
  return functools.reduce(jnp.bitwise_or, regs)


def _interleave(matmuls, *placed):
  slots = [[m] for m in matmuls]
  for pieces, lo, hi in placed:
    for k, piece in enumerate(pieces):
      slots[lo + k * (hi - lo) // len(pieces)].append(piece)
  return [piece for slot in slots for piece in slot]


def _kernel(xt_hbm, wqkv_hbm, wo_hbm, wg_hbm, wu_hbm, wdt_hbm, c_hbm, wmod_hbm,
            out_hbm,
            xt_v, wqkv_v, wo_v, wg_v, wu_v, wdt_v, c_v, wmod_v,
            sc_v, mod_v, stat_v, wqkvt_v, wot_v, h1_v, qkv_v, edge_v,
            qt_v, kt_v, vt_v, ot_v, op_v, ob_v, x1_v, hb_v, hr_v, lead_v,
            acc_v, out_v, in_sem, out_sem):
  d_model, seq = xt_hbm.shape
  dh = d_model // N_HEADS
  pairs = dh // 2
  n_tiles = seq // TILE
  last = n_tiles - 1
  fc = wg_hbm.shape[1] // N_CHUNKS
  mh = d_model // 2
  half = TILE // 2
  n_rest = d_model - 2 * KH
  spare = (pl.ds(0, SUBLANES), pl.ds(0, LANES))
  spare_bf16 = (pl.ds(0, 2 * SUBLANES), pl.ds(0, LANES))

  sems = iter(range(in_sem.shape[0]))
  copy = lambda src, dst: pltpu.make_async_copy(src, dst, in_sem.at[next(sems)])

  def col_copies(src, dst, cuts):
    return [copy(src.at[:, pl.ds(a, b - a)], dst.at[:, pl.ds(a, b - a)])
            for a, b in zip(cuts, cuts[1:])]

  mod_cuts = (0, 3, 6, 9, 14, 6 * d_model // LANES)
  qkv_cut = 512
  c_cp = copy(c_hbm, c_v)
  wmod_cps = col_copies(wmod_hbm, wmod_v, [j * LANES for j in mod_cuts])
  wqkv_cps = col_copies(wqkv_hbm, wqkv_v, (0, qkv_cut, 3 * d_model))
  wo_cp = copy(wo_hbm, wo_v)
  x_cps = [copy(xt_hbm.at[:, pl.ds(i * TILE, TILE)], xt_v.at[i])
           for i in range(n_tiles)]
  ff_cps = [copy(w_hbm.at[:, pl.ds(j * fc, fc)], w_v.at[j])
            for j in range(N_CHUNKS)
            for w_hbm, w_v in ((wg_hbm, wg_v), (wu_hbm, wu_v), (wdt_hbm, wdt_v))]
  for cp in (c_cp, x_cps[0], *wmod_cps[:3], *wqkv_cps, x_cps[1], wo_cp,
             wmod_cps[3], *x_cps[2:], wmod_cps[4], *ff_cps):
    cp.start()

  def out_copy(i):
    start = i * TILE if isinstance(i, int) else pl.multiple_of(i * TILE, TILE)
    return pltpu.make_async_copy(
        out_v.at[i], out_hbm.at[:, pl.ds(start, TILE)], out_sem.at[i])

  def opaque_zero(s, k):
    return lax.shift_right_logical(s + k, 16)

  next_operand = [None]
  results = []
  normalized = []

  def pin(*vals):
    if next_operand[0] is not None:
      ref = next_operand[0]
      ref.bitcast(I32)[(ref.shape[0] - 1, 0, *spare)] = _token(vals)

  def run(steps):
    for n, (fn, *args) in enumerate(steps):
      later = [f for f, *_ in steps[n + 1:] if f in (project_qkv, project_out)]
      next_operand[0] = (None if not later
                         else h1_v if later[0] is project_qkv else ob_v)
      fn(*args)
    next_operand[0] = None
    results.clear()
    normalized.clear()

  def silu_c(rows):
    cv = c_v[...].astype(F32)
    return jnp.broadcast_to(cv * jax.nn.sigmoid(cv), (rows, d_model))

  def store_modulation(j, row):
    part = (j * LANES + lax.broadcasted_iota(I32, (1, LANES), 1)) // d_model
    row = jnp.where((part == 1) | (part == 4), row + 1.0, row)
    mod_v[pl.ds(j * LANES, LANES), :] = jnp.broadcast_to(row, (LANES, LANES)).T

  def modulation(s, j):
    w = wmod_v[:, pl.ds(j * LANES, LANES)].astype(F32)
    row = _column_sum(w * sc_v[opaque_zero(s, 60)], 2)
    store_modulation(j, row)

  def modulation_mxu(lo, hi):
    rows = _dot(silu_c(2 * SUBLANES).astype(BF16),
                wmod_v[:, pl.ds(lo * LANES, (hi - lo) * LANES)])
    for j in range(lo, hi):
      store_modulation(j, rows[:1, (j - lo) * LANES:(j - lo + 1) * LANES])

  def mod(part, lo, size, n=1):
    col = mod_v[pl.ds(part * d_model + lo, size), :]
    return col if n == 1 else jnp.concatenate([col] * n, axis=1)

  def moments(load, which, s, b, chains):
    inv_d = 1.0 / d_model
    mean = _column_sum(load(0), chains) * inv_d
    xc = load(1) - mean
    var = _column_sum(xc * xc, chains) * inv_d
    for k, v in enumerate((mean, lax.rsqrt(var + LN_EPS))):
      stat_v[which, s, k, b] = v = jnp.broadcast_to(v, (SUBLANES, LANES))
    pin(v)
    return [v]

  def normalize(x, which, s, b, lo, serial=False):
    size = x.shape[0]
    mean, rstd = stat_v[which, s, 0, b], stat_v[which, s, 1, b]
    if serial and normalized:
      mean = _after(mean, normalized[-1], opaque_zero(s, 36))
    mean, rstd = (jnp.tile(v, (size // SUBLANES, 1)) for v in (mean, rstd))
    y = ((x - mean) * rstd * mod(3 * which + 1, lo, size)
         + mod(3 * which, lo, size))
    normalized.append(y[:SUBLANES])
    return y

  def norm1_stats(s, b):
    if len(results) >= 2:
      xt_v[(n_tiles, *spare_bf16)] = pltpu.bitcast(results[-2], BF16)
    cols = pl.ds(b * LANES, LANES)
    moments(lambda k: xt_v[s + opaque_zero(s, 32 + k), :, cols].astype(F32),
            0, s, b, 2)

  def norm1(s, slot, b, i, n):
    size = d_model // n
    rows = pl.ds(i * size, size)
    x = xt_v[s + opaque_zero(s, 34), rows, pl.ds(b * LANES, LANES)]
    h1_v[slot, b, rows, :] = normalize(
        x.astype(F32), 0, s, b, i * size).astype(BF16)

  def norm2_stats(s, b):
    if len(results) >= 2:
      x1_v[(n_tiles, *spare)] = results[-2]
    cols = pl.ds(b * LANES, LANES)
    moments(lambda k: x1_v[s + opaque_zero(s, 40 + k), :, cols], 1, s, b, 2)

  def norm2(s, tile, slot, b, r, serial=False):
    def h(side, row):
      blk = b + side * NB // 2
      x = x1_v[tile, pl.ds(row, SHARE), pl.ds(blk * LANES, LANES)]
      return normalize(x, 1, s, blk, row, serial)

    outs = _strassen_rhs(h(0, r), h(1, r), h(0, r + KH), h(1, r + KH))
    for k in range(7):
      hb_v[slot, k, b, pl.ds(r, SHARE), :] = outs[k]
    return list(outs)

  def norm2_rest(s, tile, slot):
    rows = pl.ds(2 * KH, n_rest)
    outs = [normalize(x1_v[tile, rows, pl.ds(b * LANES, LANES)], 1, s, b,
                      2 * KH).astype(BF16) for b in range(NB)]
    for b in range(NB):
      hr_v[slot, b] = outs[b]
    return outs

  def transpose_weights(w_v, wt_v, a, b):
    for k in range(0, d_model, LANES):
      size = min(LANES, d_model - k)
      t = w_v[pl.ds(k, size), pl.ds(a, b - a)].T
      if size < LANES:
        t = jnp.concatenate([t, jnp.zeros((b - a, LANES - size), BF16)], axis=1)
      wt_v[k // LANES, pl.ds(a, b - a), :] = t

  def project_qkv(s, lo, size):
    qkv = _dot(_lane_blocks(wqkvt_v, (), lo, size)[:, :d_model],
               _lane_blocks(h1_v, ((s & 1) + opaque_zero(s, 17),), 0, d_model))
    results.append(qkv[:SUBLANES, :LANES])
    for b in range(NB):
      qkv_v[b, pl.ds(lo, size), :] = (
          qkv[:, b * LANES:(b + 1) * LANES].astype(BF16))

  def to_token_major(part, js):
    buf = (qt_v, kt_v, vt_v)[part]
    for j in js:
      rows = pl.ds(part * mh + j, N_HEADS, stride=pairs)
      t = jnp.concatenate(
          [qkv_v.bitcast(I32)[b, rows, :] for b in range(NB)], axis=0).T
      if part:
        lane = lax.broadcasted_iota(I32, (HALO, LANES), 1)
        before = jnp.where(lane < LANES - N_HEADS, t[-HALO:], edge_v[part - 1, j])
        edge_v[part - 1, j] = t[-HALO:]
        t = jnp.concatenate([pltpu.roll(before, N_HEADS, 1), t], axis=0)
      buf[2 * j] = pltpu.bitcast(t << 16, F32)
      buf[2 * j + 1] = pltpu.bitcast(t & -65536, F32)

  probs = {}

  def window(g, w):
    return pl.ds(HALO + g * SUBLANES - DILATION * w, SUBLANES)

  def scores(s, g, ways):
    r0 = g * SUBLANES
    z = opaque_zero(s, g)
    q = [qt_v[z + d, pl.ds(r0, SUBLANES), :] for d in range(dh)]
    logits = []
    for w in range(WINDOW):
      q0 = q[0] if w < ways else _after(q[0], logits[w - ways], z)
      logits.append(functools.reduce(jnp.add, [
          qd * kt_v[z + d, window(g, w), :]
          for d, qd in enumerate([q0, *q[1:]])]))
    for w in range(WINDOW):
      logits[w] = logits[w] * dh ** -0.5
      if r0 < DILATION * w:
        shape = (SUBLANES, LANES)
        pos = (s * TILE + r0 + lax.broadcasted_iota(I32, shape, 0)
               + lax.broadcasted_iota(I32, shape, 1) // N_HEADS * LANES)
        logits[w] = jnp.where(pos >= DILATION * w, logits[w], MASK_VALUE)
    m = functools.reduce(jnp.maximum, logits)
    e = [jnp.exp(l - m) for l in logits]
    inv = 1.0 / functools.reduce(jnp.add, e)
    probs[g] = [x * inv for x in e]
    return [inv]

  def mix(s, g, ways):
    z = opaque_zero(s, g)
    p = probs.pop(g)
    outs = []
    for d in range(dh):
      p0 = p[0] if d < ways else _after(p[0], outs[d - ways], z)
      outs.append(functools.reduce(jnp.add, [
          pw * vt_v[z + d, window(g, w), :]
          for w, pw in enumerate([p0, *p[1:]])]))
      rows = pl.ds(2 * g * SUBLANES + d % 2, SUBLANES, stride=2)
      ot_v[d // 2, rows, :] = outs[-1]
    return outs[-ways:]

  def attend(s, g, ways_qk, ways_pv):
    pin(*(scores(s, g, ways_qk) if g < LANES // SUBLANES else []),
        *(mix(s, g - 1, ways_pv) if g else []))

  def to_feature_major(s):
    for j in range(pairs):
      op_v[j] = ot_v[opaque_zero(s, 18) + j].astype(BF16)
      t = op_v.bitcast(I32)[j].T
      for b in range(NB):
        ob_v.bitcast(I32)[0, b, pl.ds(j, N_HEADS, stride=pairs), :] = (
            t[b * N_HEADS:(b + 1) * N_HEADS])

  def project_out(s, tile, lo, size):
    y = _dot(_lane_blocks(wot_v, (), lo, size)[:, :d_model],
             _lane_blocks(ob_v, (opaque_zero(s, 19),), 0, d_model))
    results.append(y[:SUBLANES, :LANES])
    rows = pl.ds(lo, size)
    x1_v[tile, rows, :] = (xt_v[tile, rows, :].astype(F32)
                           + mod(2, lo, size, NB) * y)

  per_block = lambda fn, s: [(fn, s, b) for b in range(NB)]
  norm1_steps = lambda s, slot: [(norm1, s, slot, b, i, 4)
                                 for b in range(NB) for i in range(4)]
  qkv_steps = lambda s, a, b: [(project_qkv, s, lo, ROWS)
                               for lo in range(a, b, ROWS)]
  token_steps = lambda part: [(to_token_major, part, range(j, j + 3))
                              for j in range(0, pairs, 3)]
  attend_steps = lambda s, *ways: [(attend, s, g, *ways)
                                   for g in range(LANES // SUBLANES + 1)]

  zero = lax.fori_loop(0, 2, lambda i, z: z + opaque_zero(i, 1), jnp.int32(0))
  edge_v[...] = jnp.zeros(edge_v.shape, edge_v.dtype)
  x1_v[0] = jnp.zeros(x1_v.shape[1:], F32)
  c_cp.wait()
  sc_v[0] = silu_c(LANES).T
  x_cps[0].wait()
  run(per_block(norm1_stats, zero))
  for cp, a, b in zip(wmod_cps[:3], mod_cuts, mod_cuts[1:]):
    cp.wait()
    for j in range(a, b):
      modulation(zero, j)
  run([(norm1, zero, 0, b, 0, 1) for b in range(NB)])

  wqkv_cps[0].wait()
  transpose_weights(wqkv_v, wqkvt_v, 0, qkv_cut)
  run(qkv_steps(zero, 0, qkv_cut))
  wqkv_cps[1].wait()
  transpose_weights(wqkv_v, wqkvt_v, qkv_cut, 3 * d_model)
  run(qkv_steps(zero, qkv_cut, d_model)
      + [(project_qkv, zero, d_model, d_model)] + token_steps(0))
  for cp in (x_cps[1], wo_cp, wmod_cps[3]):
    cp.wait()
  run([(project_qkv, zero, 2 * d_model, d_model)] + token_steps(1)
      + [(modulation, zero, j) for j in range(*mod_cuts[3:5])]
      + per_block(norm1_stats, zero + 1)
      + [(transpose_weights, wo_v, wot_v, 0, d_model)]
      + norm1_steps(zero + 1, 1) + token_steps(2))
  for cp in x_cps[2:]:
    cp.wait()

  @pl.loop(0, last)
  def _(s):
    ahead = jnp.minimum(s + 2, last)
    run(_interleave(
        qkv_steps(s + 1, 0, 3 * d_model),
        (attend_steps(s, 2, 2), 1, 18),
        ([(to_feature_major, s)], 18, 19),
        (per_block(norm1_stats, ahead), 18, 22),
        (per_block(norm2_stats, jnp.maximum(s - 1, 0)), 22, 26)))

    @pl.when(opaque_zero(s, 50) == 0)
    def _():
      steps = [(project_out, s, s, lo, ROWS // 2)
               for lo in range(0, d_model, ROWS // 2)]
      run(_interleave(
          steps,
          (token_steps(0) + token_steps(1) + token_steps(2), 0, len(steps)),
          (norm1_steps(ahead, s & 1), 0, len(steps))))

  def transpose_lead(j):
    t = wg_v[j, pl.ds(2 * KH, n_rest), :].T
    lead_v[j] = jnp.concatenate(
        [t, jnp.zeros((fc, LANES - n_rest), BF16)], axis=1)

  for cp in (wmod_cps[4], *ff_cps):
    cp.wait()
  run(attend_steps(zero + last, WINDOW, dh)
      + [(modulation_mxu, *mod_cuts[4:]), (to_feature_major, zero + last),
         (project_out, zero + last, last, 0, d_model), (norm2_rest, zero, 0, 0)]
      + [(norm2, zero, 0, 0, b, r, True)
         for b in range(NB // 2) for r in range(0, KH, SHARE)]
      + [(transpose_lead, j) for j in range(N_CHUNKS)])

  def finish(i, r, size):
    c11, c12, c21, c22 = _strassen_out(
        *(acc_v[i & 1, k, pl.ds(r, size), :] for k in range(7)))
    outs = []
    for lo, y in ((r, (c11, c12)), (r + mh, (c21, c22))):
      rows = pl.ds(lo, size)
      outs.append((x1_v[i, rows, :] + mod(5, lo, size, NB)
                   * jnp.concatenate(y, axis=1)).astype(out_v.dtype))
      out_v[i, rows, :] = outs[-1]
    return outs

  @pl.loop(0, n_tiles * N_CHUNKS)
  def _(step):
    i, j = lax.div(step, N_CHUNKS), lax.rem(step, N_CHUNKS)
    slot = i & 1
    first, second = pl.ds(0, fc // 2), pl.ds(fc // 2, fc // 2)

    def products(w_v, blocks, dot, rhs, order, extra, side_work):
      out = {}
      side_work, started = list(side_work), []
      for k in order:
        if results:
          w_v[(N_CHUNKS, *spare_bf16)] = pltpu.bitcast(
              _token([results[-1], *started]), BF16)
          started = side_work.pop(0)(results[-1]) if side_work else []
        terms = [w_v[(j, *blocks[q])] for _, q in _LHS_TERMS[k]]
        lhs = terms[0]
        if len(terms) == 2:
          x, y = (t.astype(F32) for t in terms)
          lhs = (x + y if _LHS_TERMS[k][1][0] > 0 else x - y).astype(BF16)
        if k in extra:
          lhs = jnp.concatenate([lhs, w_v[(j, *extra[k])]], axis=0)
        out[k] = dot(lhs, rhs[k])
        results.append(out[k][:SUBLANES, :LANES])
      return out

    def project(w_v, lead, side_work):
      top, bottom, rest = pl.ds(0, KH), pl.ds(KH, KH), pl.ds(2 * KH, n_rest)
      rhs = [_lane_blocks(hb_v, (slot, k), 0, KH) for k in range(7)]
      hr = _lane_blocks(hr_v, (slot,), 0, n_rest)
      if lead:
        r12, r21 = (
            _dot(_load_bf16(lead_v, (j,), lo, fc // 2)[:, :n_rest], h)
            for lo, h in ((0, hr[:, half:]), (fc // 2, hr[:, :half])))
      else:
        r12 = _dot_tn(w_v[j, rest, first], hr[:, half:])
        r21 = _dot_tn(w_v[j, rest, second], hr[:, :half])
      results.append(r21[:SUBLANES, :LANES])
      rhs[5] = jnp.concatenate([rhs[5], hr[:, half:]], axis=0)
      rhs[6] = jnp.concatenate([rhs[6], hr[:, :half]], axis=0)
      m = products(
          w_v, ((top, first), (bottom, first), (top, second), (bottom, second)),
          _dot_tn, rhs, (2, 3, 1, 4, 0, 6, 5),
          {5: (rest, second), 6: (rest, first)}, side_work)
      c11, c12, c21, c22 = _strassen_out(*(m[k] for k in range(7)))
      return c11, c12 + r12, c21 + r21, c22

    def finish_share(n, after):
      acc_v[(2, 0, *spare)] = after
      r = pl.multiple_of(j * (mh // N_CHUNKS) + n * SHARE, 2 * SUBLANES)
      return finish(jnp.maximum(i - 1, 0), r, SHARE)

    def norm2_share(n, after):
      x1_v[(n_tiles, *spare)] = after
      nxt = jnp.minimum(i + 1, last)
      if n is None:
        return norm2_rest(nxt, nxt, 1 - slot)
      r = jnp.minimum(j * 3 * SHARE, KH - 3 * SHARE) + n // 2 * SHARE
      return norm2(nxt, nxt, 1 - slot, n % 2, pl.multiple_of(r, 2 * SUBLANES))

    def stats_share(n, after):
      x1_v[(n_tiles, *spare)] = after
      k = jnp.minimum(2 * step + n, 2 * NB - 1)
      tile, b = last - 1 + lax.div(k, NB), lax.rem(k, NB)
      cols = pl.ds(pl.multiple_of(b * LANES, LANES), LANES)
      return moments(lambda u: x1_v[tile + opaque_zero(step, 40 + u), :, cols],
                     1, tile, b, 1)

    idle = lambda after: []
    stats = [functools.partial(stats_share, n) for n in range(2)]
    norm2_shares = [functools.partial(norm2_share, n)
                    for n in (None, *range(6))]
    g = project(wg_v, True, stats + [idle] + [
        functools.partial(finish_share, n)
        for n in range(mh // N_CHUNKS // SHARE)])
    u = project(wu_v, False, norm2_shares[:-1])
    top, bottom = pl.ds(0, mh), pl.ds(mh, mh)
    order = (2, 3, 0, 4, 6, 1, 5)
    m = products(
        wdt_v, ((top, first), (top, second), (bottom, first), (bottom, second)),
        _dot, _strassen_rhs(*(a * b for a, b in zip(g, u))), order, {},
        norm2_shares[-1:])
    for k in order:
      acc_v[slot, k] = jnp.where(j > 0, acc_v[slot, k], 0.0) + m[k]
    results.clear()
    normalized.clear()

    @pl.when((j == N_CHUNKS - 1) & (i > 0))
    def _():
      out_copy(i - 1).start()

  last_cps = []
  for r in range(0, mh, mh // 3):
    finish(last, r, mh // 3)
    for lo in (r, r + mh):
      rows = pl.ds(lo, mh // 3)
      last_cps.append(pltpu.make_async_copy(
          out_v.at[last, rows], out_hbm.at[rows, pl.ds(last * TILE, TILE)],
          out_sem.at[last + len(last_cps)]))
      last_cps[-1].start()
  for cp in (*map(out_copy, range(last)), *last_cps):
    cp.wait()


@jax.jit
def pallas_adaLN_cond__sliding_local_dilated__glu_gated_bilinear__prompt_kernel(
    A_x: jax.Array,
    A_wqkv: jax.Array,
    A_wo: jax.Array,
    B_x: jax.Array,
    B_w_gate: jax.Array,
    B_w_up: jax.Array,
    B_w_down: jax.Array,
    c: jax.Array,
    w_mod: jax.Array,
):
  del B_x
  batch, seq, d_model = A_x.shape
  d_ff = B_w_gate.shape[1]
  assert (batch, d_model, d_ff) == (1, 576, 4608)
  assert seq % TILE == 0 and seq >= 4 * TILE
  dh = d_model // N_HEADS
  n_tiles = seq // TILE
  fc = d_ff // N_CHUNKS
  k_blocks = pl.cdiv(d_model, LANES)
  operands = (A_x.reshape(seq, d_model).T, A_wqkv, A_wo, B_w_gate, B_w_up,
              B_w_down.T, c, w_mod)
  hbm = pl.BlockSpec(memory_space=pltpu.HBM)
  vmem = pltpu.VMEM
  out_t = pl.pallas_call(
      _kernel,
      in_specs=[hbm] * len(operands),
      out_specs=hbm,
      out_shape=jax.ShapeDtypeStruct((d_model, seq), A_x.dtype),
      scratch_shapes=[
          vmem((n_tiles + 1, d_model, TILE), BF16),
          vmem(A_wqkv.shape, BF16),
          vmem(A_wo.shape, BF16),
          *[vmem((N_CHUNKS + 1, d_model, fc), BF16)] * 3,
          vmem(c.shape, BF16),
          vmem(w_mod.shape, BF16),
          vmem((1, d_model, LANES), F32),
          vmem((6 * d_model, LANES), F32),
          vmem((2, n_tiles + 1, 2, NB, SUBLANES, LANES), F32),
          vmem((k_blocks, 3 * d_model, LANES), BF16),
          vmem((k_blocks, d_model, LANES), BF16),
          vmem((3, NB, d_model, LANES), BF16),
          vmem((NB, 3 * d_model, LANES), BF16),
          vmem((2, dh // 2, HALO, LANES), I32),
          vmem((dh, LANES, LANES), F32),
          vmem((dh, HALO + LANES, LANES), F32),
          vmem((dh, HALO + LANES, LANES), F32),
          vmem((dh // 2, 2 * LANES, LANES), F32),
          vmem((dh // 2, 2 * LANES, LANES), BF16),
          vmem((2, NB, d_model, LANES), BF16),
          vmem((n_tiles + 1, d_model, TILE), F32),
          vmem((2, 7, NB // 2, KH, LANES), BF16),
          vmem((2, NB, d_model - 2 * KH, LANES), BF16),
          vmem((N_CHUNKS, fc, LANES), BF16),
          vmem((3, 7, d_model // 2, TILE // 2), F32),
          vmem((n_tiles, d_model, TILE), A_x.dtype),
          pltpu.SemaphoreType.DMA((9 + n_tiles + 3 * N_CHUNKS,)),
          pltpu.SemaphoreType.DMA((n_tiles + 5,)),
      ],
      compiler_params=pltpu.CompilerParams(vmem_limit_bytes=100 * 2**20),
      name="adaln_window_attn_glu",
  )(*operands)
  return out_t.T.reshape(batch, seq, d_model)
```
